```python
import jax
import jax.numpy as jnp

def _softmax(x, axis=-1):
    return jax.nn.softmax(x, axis=axis)
def _gelu(x):
    return jax.nn.gelu(x, approximate=True)
def _silu(x):
    return jax.nn.silu(x)
def _sigmoid(x):
    return jax.nn.sigmoid(x)
def _layernorm(x, axis=-1, eps=1e-5):
    m = jnp.mean(x, axis=axis, keepdims=True)
    v = jnp.var(x, axis=axis, keepdims=True)
    return (x - m) / jnp.sqrt(v + eps)
def _scatter_add(tgt, idx, src, axis=0):
    return tgt.at[idx].add(src)
def _segment_sum(src, seg, n):
    return jax.ops.segment_sum(src, seg, n)
class _Rng:
    def __init__(self, key):
        self._k = key
    def _next(self):
        self._k, sub = jax.random.split(self._k)
        return sub
    def normal(self, shape):
        return jax.random.normal(self._next(), shape, dtype=jnp.bfloat16)
    def randint(self, lo, hi, shape):
        return jax.random.randint(self._next(), shape, lo, hi, dtype=jnp.int32)
    def uniform(self, shape, lo=0.0, hi=1.0):
        return jax.random.uniform(self._next(), shape, jnp.bfloat16, lo, hi)
    def permutation(self, n):
        return jax.random.permutation(self._next(), n)


kernel_name = 'parallel_sum__linear_attn_block__moe_arch_mod__prompt'

def setup_inputs():
    _rng = _Rng(jax.random.key(int.from_bytes(__import__("os").urandom(4), "little")))
    _w = (lambda a: (lambda t: t.astype(jnp.bfloat16) if jnp.issubdtype(t.dtype, jnp.floating) else t)(jnp.asarray(a)))
    def _A_setup():
        B, S, D = 1, 2048, 1024
        return {
            "x": _w((lambda *s: _rng.normal(s) * 0.05)(B, S, D)),
            "wqkv": _w((lambda *s: _rng.normal(s) * 0.05)(D, 3 * D)),
            "wo": _w((lambda *s: _rng.normal(s) * 0.05)(D, D)),
        }
    _A_in = _A_setup()

    def _B_setup():
        B, S, D, F, C = 1, 2048, 1024, 3584, 1
        return {
            "x": _w((lambda *s: _rng.normal(s) * 0.05)(B, S, D)),
            "w_r": _w((lambda *s: _rng.normal(s) * 0.05)(D)),
            "w_gate": _w((lambda *s: _rng.normal(s) * 0.05)(D, F)),
            "w_up": _w((lambda *s: _rng.normal(s) * 0.05)(D, F)),
            "w_down": _w((lambda *s: _rng.normal(s) * 0.05)(F, D)),
        }
    _B_in = _B_setup()

    return {
        "A_x": _A_in["x"],
        "A_wqkv": _A_in["wqkv"],
        "A_wo": _A_in["wo"],
        "B_x": _B_in["x"],
        "B_w_r": _B_in["w_r"],
        "B_w_gate": _B_in["w_gate"],
        "B_w_up": _B_in["w_up"],
        "B_w_down": _B_in["w_down"],
    }

def reference(A_x, A_wqkv, A_wo, B_x, B_w_r, B_w_gate, B_w_up, B_w_down):
    def _A_ref(x, wqkv, wo):
        B, S, D = x.shape
        H = 32; Dh = D // H
        qkv = (lambda x, *d: x.transpose(*d))((x @ wqkv).reshape(B, S, 3, H, Dh), 2, 0, 3, 1, 4)
        q, k, v = qkv[0], qkv[1], qkv[2]
        phi = lambda t: jnp.where(t > 0, t + 1, jnp.exp(t)) + 1e-6
        pq, pk = phi(q), phi(k)
        kv = jnp.einsum("bhsd,bhse->bhde", pk, v)
        z = jnp.einsum("bhsd->bhd", pk)
        num = jnp.einsum("bhqd,bhde->bhqe", pq, kv)
        den = jnp.einsum("bhqd,bhd->bhq", pq, z)[..., None] + 1e-6
        o = num / den
        return (lambda x, *d: x.transpose(*d))(o, 0, 2, 1, 3).reshape(B, S, D) @ wo

    def _B_ref(x, w_r, w_gate, w_up, w_down):
        B, S, D = x.shape
        C = 1
        r = x @ w_r
        idx = jnp.argsort(-r, axis=-1)[:, :C]
        idx_e = jnp.repeat(idx.reshape(B, C, 1), D, axis=2)
        x_sel = jnp.take_along_axis(x, idx_e, axis=1)
        g = _silu(x_sel @ w_gate)
        u = x_sel @ w_up
        y = (g * u) @ w_down
        r_sel = _sigmoid(jnp.take_along_axis(r, idx, axis=1))
        y = y * r_sel.reshape(B, C, 1)
        b_off = (jnp.arange(B) * S).reshape(B, 1)
        flat_idx = (idx + b_off).reshape(B * C)
        zero = (x * 0.0).reshape(B * S, D)
        upd = _scatter_add(zero, flat_idx, y.reshape(B * C, D), axis=0)
        return x + upd.reshape(B, S, D)

    x = A_x
    xn = _layernorm(x, axis=-1)
    return x + _A_ref(xn, A_wqkv, A_wo) + _B_ref(xn, B_w_r, B_w_gate, B_w_up, B_w_down)
```

```python
import functools, contextlib
import numpy as np
import jax
import jax.numpy as jnp
from jax import lax
import jax.experimental.pallas as pl
import jax.experimental.pallas.tpu as pltpu

S, D, H, DH, F = 2048, 1024, 32, 32, 3584
L = 128
NB = D // L
f32, bf16, u32 = jnp.float32, jnp.bfloat16, jnp.uint32


def _phi(t):
    return jnp.where(t > 0, t + 1.0, jnp.exp(t)) + 1e-6


def _dot(a, b):
    return jnp.dot(a, b, preferred_element_type=f32)


def _zero(v):
    b = pltpu.bitcast(v, u32)
    return lax.shift_right_logical(lax.shift_right_logical(b, jnp.uint32(31)), jnp.uint32(1))


def _tie(xv, z):
    return pltpu.bitcast(pltpu.bitcast(xv, u32) | z, bf16)


def tied_lhs(load, nrows, nslab, thunks, kk=None):
    n = len(thunks)
    if n == 0:
        return jnp.concatenate([load(slice(0, nrows), k) for k in range(nslab)], axis=1)
    if kk is None:
        kk = [k for k in range(0, nslab, 2)]
    per = -(-n // len(kk))
    npos = 1
    while npos < per * len(kk) and npos < nrows // 16:
        npos *= 2
    step = nrows // npos
    slabs = []
    order = {}
    for p in range(n):
        m, q = divmod(p, per)
        r = (q * npos) // per + (m * npos) // (per * len(kk))
        order.setdefault((kk[m], min(r, npos - 1)), []).append(p)
    zs = {}
    for p in range(n):
        v = thunks[p]()
        zs[p] = None if v is None else _zero(v)
    for k in range(nslab):
        if k not in kk:
            slabs.append(load(slice(0, nrows), k))
            continue
        parts = []
        for r in range(npos):
            ps = [zs[p] for p in order.get((k, r), []) if zs[p] is not None]
            if not ps:
                parts.append(load(slice(r * step, (r + 1) * step), k))
            else:
                z = ps[0]
                for z2 in ps[1:]:
                    z = z | z2
                parts.append(_tie(load(slice(r * step, r * step + 16), k), z))
                if step > 16:
                    parts.append(load(slice(r * step + 16, (r + 1) * step), k))
        slabs.append(jnp.concatenate(parts, axis=0))
    return jnp.concatenate(slabs, axis=1)


def make(R=512, WC=256, scopes=False, recip="nr", flags=None, tie1=True, tie2=True, LNS=16, GS=8, DS=32, tieG=True, tieD=True, tieM=True, kkA=None, kkH=None, dbg='', order='GA_DH', xval=True):
    sc = (lambda n: jax.named_scope(n)) if scopes else (lambda n: contextlib.nullcontext())
    NI = S // R
    NWC = (2 * D) // WC
    FC = F // NI
    FB = FC // L
    QW = 256

    def rcp(x):
        if recip == "approx":
            return pl.reciprocal(x, approx=True)
        if recip == "nr":
            r = pl.reciprocal(x, approx=True)
            return r * (2.0 - x * r)
        return pl.reciprocal(x, approx=False)

    def kernel(x_hbm, wqkv_hbm, wo_hbm, wr_ref, wg_hbm, wu_hbm, wd_hbm, out_hbm,
               x_v, xn_v, wqkv_v, wo_v, wg_v, wu_v, wd_v, out_v, kv_acc, zb_v, m_v, xb_v, pq_v, o_v, acc_v, hb_v, y_v,
               sems):
        HR = R // 2

        def x_dma(i):
            return pltpu.make_async_copy(x_hbm.at[pl.ds(i * R, R)], x_v.at[pl.ds(i * R, R)], sems.at[i])

        def x0_dma(h):
            return pltpu.make_async_copy(x_hbm.at[pl.ds(h * HR, HR)], x_v.at[pl.ds(h * HR, HR)], sems.at[NI + h])

        def w_dma(c):
            cs = pl.ds(D + c * WC, WC)
            return pltpu.make_async_copy(wqkv_hbm.at[:, cs], wqkv_v.at[:, cs], sems.at[NI + 2 + c])

        o0 = NI + 2 + NWC
        wq_dma = pltpu.make_async_copy(wqkv_hbm.at[:, pl.ds(0, D)], wqkv_v.at[:, pl.ds(0, D)], sems.at[o0])
        wo_dma = pltpu.make_async_copy(wo_hbm, wo_v, sems.at[o0 + 1])

        def wg_dma(c):
            return pltpu.make_async_copy(wg_hbm.at[:, pl.ds(c * FC, FC)], wg_v.at[c], sems.at[o0 + 2 + c])

        def wu_dma(c):
            return pltpu.make_async_copy(wu_hbm.at[:, pl.ds(c * FC, FC)], wu_v.at[c], sems.at[o0 + 2 + NI + c])

        def wd_dma(c):
            return pltpu.make_async_copy(wd_hbm.at[pl.ds(c * FC, FC)], wd_v.at[c], sems.at[o0 + 2 + 2 * NI + c])

        def o_dma(b):
            rows = pl.ds(pl.multiple_of(b * R, R), R)
            return pltpu.make_async_copy(out_v.at[rows], out_hbm.at[rows], sems.at[o0 + 2 + 3 * NI + b])

        x0_dma(0).start()
        w_dma(0).start()
        x0_dma(1).start()
        for c in range(1, NWC):
            w_dma(c).start()
        for i in range(1, NI):
            x_dma(i).start()
        wq_dma.start()
        wo_dma.start()
        for c in range(NI):
            wg_dma(c).start()
            wu_dma(c).start()
            wd_dma(c).start()

        wr = wr_ref[...].astype(f32).reshape(1, D)

        def ln(row0, n, st):
            best, bidx = st
            rows = pl.ds(row0, n)
            x = x_v[rows, :].astype(f32)
            m = jnp.mean(x, axis=-1, keepdims=True)
            d = x - m
            v = jnp.mean(d * d, axis=-1, keepdims=True)
            xn = d * lax.rsqrt(v + 1e-5)
            xn_v[rows, :] = xn.astype(bf16)
            r = jnp.sum(xn * wr, axis=-1, keepdims=True)
            bm = jnp.max(r, axis=0, keepdims=True)
            ridx = lax.broadcasted_iota(jnp.int32, (n, 1), 0) + row0
            bi = jnp.min(jnp.where(r == bm, ridx, S), axis=0, keepdims=True)
            better = jnp.logical_or(bm > best, jnp.logical_and(bm == best, bi < bidx))
            st[0] = jnp.where(better, bm, best)
            st[1] = jnp.where(better, bi, bidx)
            return xn[0:8, 0:L]

        kv_acc[...] = jnp.zeros(kv_acc.shape, f32)
        st = [jnp.full((1, 1), -jnp.inf, f32), jnp.full((1, 1), S, jnp.int32)]
        with sc("wait_x0a"):
            x0_dma(0).wait()
        ln(0, HR, st)
        with sc("wait_x0b"):
            x0_dma(1).wait()
        ln(HR, HR, st)
        best, bidx = st

        nck = D // WC

        def kvchunk(pk, vv, c):
            for jj in range(WC // L):
                j = c * (WC // L) + jj
                kv_acc[j] += lax.dot_general(pk[:, jj * L:(jj + 1) * L], vv[:, jj * L:(jj + 1) * L],
                                             (((0,), (0,)), ((), ())), preferred_element_type=f32)

        def p1_iter(i, zacc, best, bidx, first):
            row0 = 0 if first else pl.multiple_of(i * R, R)
            rows = pl.ds(row0, R)
            nxt = R if first else pl.multiple_of(lax.rem(i + 1, NI) * R, R)
            st = [best, bidx]
            pks, vs = [], []
            zs = []

            xn = xn_v[rows, :]

            def load(rs, k):
                return xn[rs, k * L:(k + 1) * L]

            for c in range(nck):
                if first:
                    w_dma(c).wait()
                k = _dot(xn, wqkv_v[:, D + c * WC: D + (c + 1) * WC])
                pk = _phi(k)
                zs.append(jnp.sum(pk.reshape(R // 8, 8, WC), axis=0))
                pks.append(pk.astype(bf16))
            nsub = LNS // nck
            sub = R // LNS
            for c in range(nck):
                if first:
                    w_dma(nck + c).wait()
                    if c == 0:
                        x_dma(1).wait()
                th = [functools.partial(ln, nxt + (c * nsub + p) * sub, sub, st) for p in range(nsub)]
                if tie1:
                    lhs = tied_lhs(load, R, NB, th)
                else:
                    for t in th:
                        t()
                    lhs = xn
                v = _dot(lhs, wqkv_v[:, 2 * D + c * WC: 2 * D + (c + 1) * WC])
                vs.append(v.astype(bf16))
                if c > 0:
                    kvchunk(pks[c - 1], vs[c - 1], c - 1)
            kvchunk(pks[nck - 1], vs[nck - 1], nck - 1)
            zacc = zacc + jnp.concatenate(zs, axis=1)
            return zacc, st[0], st[1]

        zacc = jnp.zeros((8, D), f32)
        with sc("p1_it0"):
            zacc, best, bidx = p1_iter(0, zacc, best, bidx, True)

        def body1(i, carry):
            zacc, best, bidx = carry

            @pl.when(i < NI - 1)
            def _():
                x_dma(jnp.minimum(i + 1, NI - 1)).wait()

            return p1_iter(i, zacc, best, bidx, False)

        with sc("p1_loop"):
            zacc, best, bidx = lax.fori_loop(1, NI, body1, (zacc, best, bidx))

        z = jnp.sum(zacc, axis=0, keepdims=True)
        ri = lax.broadcasted_iota(jnp.int32, (L, L), 0) // DH
        ci = lax.broadcasted_iota(jnp.int32, (L, L), 1) // DH
        mask = ri == ci
        with sc("wait_wq_wo"):
            wq_dma.wait()
            wo_dma.wait()
        kvb_list = []
        for j in range(NB):
            kvb = jnp.where(mask, kv_acc[j], 0.0).astype(bf16)
            zc = jnp.broadcast_to(z[:, j * L:(j + 1) * L], (L, L)).T
            zb_v[j] = jnp.where(mask, zc, 0.0).astype(bf16)
            kvb_list.append(kvb)

        idx = jnp.clip(bidx[0, 0], 0, S - 1)
        g0 = pl.multiple_of((idx // 16) * 16, 16)
        xg = xn_v[pl.ds(g0, 16), :]
        gate = jax.nn.sigmoid(best)
        rr = lax.broadcasted_iota(jnp.int32, (16, 1), 0)
        xsel = jnp.sum(jnp.where(rr == idx - g0, xg.astype(f32), 0.0), axis=0, keepdims=True)
        xb_v[...] = jnp.broadcast_to(xsel, (L, D)).T
        y_v[...] = jnp.zeros((8, D), f32)
        iblk = idx // R

        def split(lst, n):
            k = -(-len(lst) // n) if lst else 0
            return [lst[a * k:(a + 1) * k] for a in range(n)]

        def mk(load, nrows, nslab, th, on, kk=None):
            if on:
                return tied_lhs(load, nrows, nslab, th, kk)
            for t in th:
                t()
            return tied_lhs(load, nrows, nslab, [])

        def g_thunks(c, slot):
            gu = {}
            wg = wg_v.at[c]
            wu = wu_v.at[c]

            def g_sub(jb, s):
                n = D // GS
                rs = slice(s * n, (s + 1) * n)
                cs = slice(jb * L, (jb + 1) * L)
                xb = xb_v[rs, :]
                g = jnp.sum((wg[rs, cs].astype(f32) * xb).reshape(n // 8, 8, L), axis=0)
                u = jnp.sum((wu[rs, cs].astype(f32) * xb).reshape(n // 8, 8, L), axis=0)
                if s > 0:
                    g = g + gu[jb][0]
                    u = u + gu[jb][1]
                gu[jb] = (g, u)
                return pltpu.bitcast(pltpu.bitcast(g, u32) | pltpu.bitcast(u, u32), f32)

            def g_fin(jb):
                g, u = gu[jb]
                g = jnp.sum(g, axis=0, keepdims=True)
                u = jnp.sum(u, axis=0, keepdims=True)
                h = g * jax.nn.sigmoid(g) * u
                hb = jnp.broadcast_to(h, (L, L)).T
                hb_v[slot, jb * L:(jb + 1) * L, :] = hb
                return hb[0:8]

            th = []
            for jb in range(FB):
                for s in range(GS):
                    th.append(functools.partial(g_sub, jb, s))
                th.append(functools.partial(g_fin, jb))
            return th

        def d_thunks(c, slot):
            ya = [None]
            NDS = FC // DS
            wd = wd_v.at[c]

            def d_sub(s):
                rs = slice(s * DS, (s + 1) * DS)
                hb = hb_v[slot, rs, :]
                w = wd[rs, :].astype(f32)
                parts = []
                for jb in range(NB):
                    parts.append(jnp.sum((w[:, jb * L:(jb + 1) * L] * hb).reshape(DS // 8, 8, L), axis=0))
                yy = jnp.concatenate(parts, axis=1)
                yy = yy + (ya[0] if s > 0 else y_v[...])
                ya[0] = yy
                if s == NDS - 1:
                    y_v[...] = yy
                hnd = pltpu.bitcast(yy[:, 0:L], u32)
                for jb in range(1, NB):
                    hnd = hnd | pltpu.bitcast(yy[:, jb * L:(jb + 1) * L], u32)
                return pltpu.bitcast(hnd, f32)

            return [functools.partial(d_sub, s) for s in range(NDS)]

        with sc("wait_ffn0"):
            wg_dma(0).wait(); wu_dma(0).wait()
        gp = split(g_thunks(0, 0), NB)
        for j in range(NB):
            kvb = kvb_list[j]
            lhs = mk(lambda rs, k: kvb[rs, :], L, 1, gp[j], tie2 and tieM)
            m_v[j * L:(j + 1) * L, :] = _dot(lhs, wo_v[j * L:(j + 1) * L, :]).astype(bf16)

        def body2(i, _):
            b = lax.rem(iblk + 1 + i, NI)
            row0 = pl.multiple_of(b * R, R)
            rows = pl.ds(row0, R)
            cn = lax.rem(i + 1, NI)
            with sc("wait_ffn"):
                wd_dma(i).wait()

                @pl.when(i < NI - 1)
                def _():
                    wg_dma(cn).wait(); wu_dma(cn).wait()
            ridx = lax.broadcasted_iota(jnp.int32, (R, 1), 0) + row0
            HK = D // 2
            xnb = xn_v.at[rows]
            xblk = x_v.at[rows]
            oblk = out_v.at[rows]
            slot = lax.rem(i, 2)
            nA, nH, nC = D // QW, D // QW, D // QW
            if order == 'DA_GH':
                aparts = split(d_thunks(i, slot), nA)
                hparts = split(g_thunks(cn, 1 - slot), nH)
                cparts = [[]] * nC
            elif order == 'GA_DH':
                aparts = split(g_thunks(cn, 1 - slot), nA)
                hparts = split(d_thunks(i, slot), nH)
                cparts = [[]] * nC
            elif order == 'DH_GAC':
                gt = g_thunks(cn, 1 - slot)
                na = len(gt) // 2
                aparts = split(gt[:na], nA)
                cparts = split(gt[na:], nC)
                hparts = split(d_thunks(i, slot), nH)
            elif order == 'DA_GHC':
                gt = g_thunks(cn, 1 - slot)
                na = len(gt) // 2
                aparts = split(d_thunks(i, slot), nA)
                hparts = split(gt[:na], nH)
                cparts = split(gt[na:], nC)
            xnval = xnb[...] if xval else None

            def load_xn(rs, k):
                return xnval[rs, k * L:(k + 1) * L] if xval else xnb[rs, k * L:(k + 1) * L]

            def load_o(half):
                return lambda rs, k: o_v[rs, half * HK + k * L: half * HK + (k + 1) * L]

            def A(c):
                cs = slice(c * QW, (c + 1) * QW)
                lhs = mk(load_xn, R, NB, aparts[c], tie2, kkA)
                pq_v[:, cs] = _phi(_dot(lhs, wqkv_v[:, cs])).astype(bf16)

            def B(j):
                cs = slice(j * L, (j + 1) * L)
                pq = pq_v[:, cs]
                den = _dot(pq, zb_v[j]) + 1e-6
                o_v[:, cs] = (pq.astype(f32) * rcp(den)).astype(bf16)

            def Hh(n):
                cs = slice(n * QW, (n + 1) * QW)
                lhs = mk(load_o(0), R, NB // 2, hparts[n], tie2, kkH)
                acc_v[:, cs] = _dot(lhs, m_v[0:HK, cs])

            def C(n):
                cs = slice(n * QW, (n + 1) * QW)
                a = acc_v[:, cs] + _dot(mk(load_o(1), R, NB // 2, cparts[n], tie2, kkH), m_v[HK:D, cs])
                y = jnp.sum(y_v[:, cs], axis=0, keepdims=True) * gate
                res = xblk[:, cs].astype(f32) + xnb[:, cs].astype(f32) + a + jnp.where(ridx == idx, y, 0.0)
                oblk[:, cs] = res.astype(bf16)

            A(0); A(1); B(0); B(1); A(2); B(2); B(3); A(3); B(4); B(5)
            Hh(0); B(6); B(7); Hh(1); Hh(2); Hh(3); C(0); C(1); C(2); C(3)
            o_dma(b).start()
            return None

        with sc("p2_loop"):
            lax.fori_loop(0, NI, body2, None)
        with sc("wait_out"):
            for b in range(NI):
                o_dma(b).wait()

    def fn(A_x, A_wqkv, A_wo, B_x, B_w_r, B_w_gate, B_w_up, B_w_down):
        anyspec = pl.BlockSpec(memory_space=pl.ANY)
        out = pl.pallas_call(
            kernel,
            out_shape=jax.ShapeDtypeStruct((S, D), bf16),
            in_specs=[anyspec, anyspec, anyspec, pl.BlockSpec(memory_space=pltpu.VMEM), anyspec, anyspec, anyspec],
            out_specs=anyspec,
            scratch_shapes=[
                pltpu.VMEM((S, D), bf16), pltpu.VMEM((S, D), bf16), pltpu.VMEM((D, 3 * D), bf16),
                pltpu.VMEM((D, D), bf16),
                pltpu.VMEM((NI, D, FC), bf16), pltpu.VMEM((NI, D, FC), bf16), pltpu.VMEM((NI, FC, D), bf16),
                pltpu.VMEM((S, D), bf16), pltpu.VMEM((NB, L, L), f32),
                pltpu.VMEM((NB, L, L), bf16), pltpu.VMEM((D, D), bf16), pltpu.VMEM((D, L), f32),
                pltpu.VMEM((R, D), bf16), pltpu.VMEM((R, D), bf16), pltpu.VMEM((R, D), f32),
                pltpu.VMEM((2, FC, L), f32), pltpu.VMEM((8, D), f32),
                pltpu.SemaphoreType.DMA((5 * NI + 4 + NWC,)),
            ],
            compiler_params=pltpu.CompilerParams(vmem_limit_bytes=100 * 1024 * 1024, flags=flags),
        )(A_x.reshape(S, D), A_wqkv, A_wo, B_w_r, B_w_gate, B_w_up, B_w_down)
        return out.reshape(1, S, D)
    return fn


_IMPL = make(**dict(tie1=False,order='DH_GAC'))


@jax.jit
def pallas_parallel_sum__linear_attn_block__moe_arch_mod__prompt_kernel(
    A_x: jax.Array,
    A_wqkv: jax.Array,
    A_wo: jax.Array,
    B_x: jax.Array,
    B_w_r: jax.Array,
    B_w_gate: jax.Array,
    B_w_up: jax.Array,
    B_w_down: jax.Array,
):
    return _IMPL(A_x, A_wqkv, A_wo, B_x, B_w_r, B_w_gate, B_w_up, B_w_down)
```

```python
import functools, contextlib
import numpy as np
import jax
import jax.numpy as jnp
from jax import lax
import jax.experimental.pallas as pl
import jax.experimental.pallas.tpu as pltpu

S, D, H, DH, F = 2048, 1024, 32, 32, 3584
L = 128
NB = D // L
f32, bf16, u32 = jnp.float32, jnp.bfloat16, jnp.uint32


def _phi(t):
    return jnp.where(t > 0, t + 1.0, jnp.exp(t)) + 1e-6


def _dot(a, b):
    return jnp.dot(a, b, preferred_element_type=f32)


def _dg(a, b, ca, cb):
    return lax.dot_general(a, b, (((ca,), (cb,)), ((), ())), preferred_element_type=f32)


def _zero(v):
    b = pltpu.bitcast(v, u32)
    return lax.shift_right_logical(lax.shift_right_logical(b, jnp.uint32(31)), jnp.uint32(1))


def _tie(xv, z):
    return pltpu.bitcast(pltpu.bitcast(xv, u32) | z, bf16)


def tied_lhs(load, nrows, nslab, thunks, kk=None):
    n = len(thunks)
    if n == 0:
        return jnp.concatenate([load(slice(0, nrows), k) for k in range(nslab)], axis=1)
    if kk is None:
        kk = [k for k in range(0, nslab, 2)]
    per = -(-n // len(kk))
    npos = 1
    while npos < per * len(kk) and npos < nrows // 16:
        npos *= 2
    step = nrows // npos
    slabs = []
    order = {}
    for p in range(n):
        m, q = divmod(p, per)
        r = (q * npos) // per + (m * npos) // (per * len(kk))
        order.setdefault((kk[m], min(r, npos - 1)), []).append(p)
    zs = {}
    for p in range(n):
        v = thunks[p]()
        zs[p] = None if v is None else _zero(v)
    for k in range(nslab):
        if k not in kk:
            slabs.append(load(slice(0, nrows), k))
            continue
        parts = []
        for r in range(npos):
            ps = [zs[p] for p in order.get((k, r), []) if zs[p] is not None]
            if not ps:
                parts.append(load(slice(r * step, (r + 1) * step), k))
            else:
                z = ps[0]
                for z2 in ps[1:]:
                    z = z | z2
                parts.append(_tie(load(slice(r * step, r * step + 16), k), z))
                if step > 16:
                    parts.append(load(slice(r * step + 16, (r + 1) * step), k))
        slabs.append(jnp.concatenate(parts, axis=0))
    return jnp.concatenate(slabs, axis=1)


def split(lst, n):
    k = -(-len(lst) // n) if lst else 0
    return [lst[a * k:(a + 1) * k] for a in range(n)]


def make(R=512, scopes=False, recip="nr", flags=None, tie2=True, tieM=True, LNS=4, GS=8, DS=32,
         kkQ=None, kkH=None, order='DH_GAC', wgroups=(1, 2, 1), tailsplit=True, finlate=4, nosemchk=False,
         lnpos=(2, 3, 4, 5), opq=True, qw=None, noffn=False, ksplit=True, g2=False, GR=16, wtie=False, lnk=(0, 0, 0, 0), lnp=(0, 0, 0, 0), midsplit=(1, 1), midskew=8, samesplit=(1, 0)):
    sc = (lambda n: jax.named_scope(n)) if scopes else (lambda n: contextlib.nullcontext())
    NI = S // R
    CW = 256
    NC = D // CW
    FC = F // NI
    FB = FC // L

    def rcp(x):
        if recip == "approx":
            return pl.reciprocal(x, approx=True)
        if recip == "nr":
            r = pl.reciprocal(x, approx=True)
            return r * (2.0 - x * r)
        return pl.reciprocal(x, approx=False)

    SX0, SWR, SWK, SX, SWQ, SWV, SWO = 0, 2, 3, 3 + NC, 3 + NC + NI, 4 + NC + NI, 5 + NC + NI
    SWG = SWO + 1
    SWU, SWD, SO = SWG + NI, SWG + 2 * NI, SWG + 3 * NI
    NSEM = SO + NI * (NC if tailsplit else 1)

    def kernel(x_hbm, wqkv_hbm, wo_hbm, wr_hbm, wg_hbm, wu_hbm, wd_hbm, out_hbm,
               x_v, xn_v, wqkv_v, wo_v, wr_v, wg_v, wu_v, wd_v, out_v, pt_v, zc_v, m_v, xb_v, o_v, acc_v, hb_v, y_v,
               sems):
        HR = R // 2

        def x0_dma(h):
            return pltpu.make_async_copy(x_hbm.at[pl.ds(h * HR, HR)], x_v.at[pl.ds(h * HR, HR)], sems.at[SX0 + h])

        wr_dma = pltpu.make_async_copy(wr_hbm, wr_v, sems.at[SWR])

        def wk_dma(c):
            cs = pl.ds(D + c * CW, CW)
            return pltpu.make_async_copy(wqkv_hbm.at[:, cs], wqkv_v.at[:, cs], sems.at[SWK + c])

        def x_dma(i):
            return pltpu.make_async_copy(x_hbm.at[pl.ds(i * R, R)], x_v.at[pl.ds(i * R, R)], sems.at[SX + i])

        wq_dma = pltpu.make_async_copy(wqkv_hbm.at[:, pl.ds(0, D)], wqkv_v.at[:, pl.ds(0, D)], sems.at[SWQ])
        wv_dma = pltpu.make_async_copy(wqkv_hbm.at[:, pl.ds(2 * D, D)], wqkv_v.at[:, pl.ds(2 * D, D)], sems.at[SWV])
        wo_dma = pltpu.make_async_copy(wo_hbm, wo_v, sems.at[SWO])

        def wg_dma(c):
            return pltpu.make_async_copy(wg_hbm.at[:, pl.ds(c * FC, FC)], wg_v.at[c], sems.at[SWG + c])

        def wu_dma(c):
            return pltpu.make_async_copy(wu_hbm.at[:, pl.ds(c * FC, FC)], wu_v.at[c], sems.at[SWU + c])

        def wd_dma(c):
            return pltpu.make_async_copy(wd_hbm.at[pl.ds(c * FC, FC)], wd_v.at[c], sems.at[SWD + c])

        def o_dma(b, n=None):
            rows = pl.ds(pl.multiple_of(b * R, R), R)
            if n is None:
                return pltpu.make_async_copy(out_v.at[rows], out_hbm.at[rows], sems.at[SO + b])
            cs = pl.ds(n * CW, CW)
            return pltpu.make_async_copy(out_v.at[rows, cs], out_hbm.at[rows, cs], sems.at[SO + b * NC + n])

        x0_dma(0).start()
        wr_dma.start()
        wk_dma(0).start()
        x0_dma(1).start()
        for c in range(1, NC):
            wk_dma(c).start()
        for i in range(1, NI):
            x_dma(i).start()
        wq_dma.start()
        wv_dma.start()
        wo_dma.start()
        for c in range(NI):
            wg_dma(c).start()
            wu_dma(c).start()
            wd_dma(c).start()

        def ln(row0, n, st, wr):
            best, bidx = st
            rows = pl.ds(row0, n)
            x = x_v[rows, :].astype(f32)
            m = jnp.mean(x, axis=-1, keepdims=True)
            d = x - m
            v = jnp.mean(d * d, axis=-1, keepdims=True)
            xn = d * lax.rsqrt(v + 1e-5)
            xn_v[rows, :] = xn.astype(bf16)
            r = jnp.sum(xn * wr, axis=-1, keepdims=True)
            bm = jnp.max(r, axis=0, keepdims=True)
            ridx = lax.broadcasted_iota(jnp.int32, (n, 1), 0) + row0
            bi = jnp.min(jnp.where(r == bm, ridx, S), axis=0, keepdims=True)
            better = jnp.logical_or(bm > best, jnp.logical_and(bm == best, bi < bidx))
            st[0] = jnp.where(better, bm, best)
            st[1] = jnp.where(better, bi, bidx)
            hnd = pltpu.bitcast(jnp.broadcast_to(st[0], (8, L)), u32)
            for g in range(n // 8):
                hnd = hnd | pltpu.bitcast(xn[8 * g:8 * g + 8, D - L:D], u32)
            return pltpu.bitcast(hnd, f32)

        st = [jnp.full((1, 1), -jnp.inf, f32), jnp.full((1, 1), S, jnp.int32)]
        with sc("wait_x0a"):
            x0_dma(0).wait()
            wr_dma.wait()
        wr = wr_v[...].astype(f32).reshape(1, D)
        ln(0, HR, st, wr)
        with sc("wait_x0b"):
            x0_dma(1).wait()
        ln(HR, HR, st, wr)
        best, bidx = st

        def p1_iter(i, zacc, best, bidx, first):
            row0 = 0 if first else pl.multiple_of(i * R, R)
            rows = pl.ds(row0, R)
            nxt = R if first else pl.multiple_of(lax.rem(i + 1, NI) * R, R)
            st = [best, bidx]
            wr = wr_v[...].astype(f32).reshape(1, D)
            xn = xn_v[rows, :]
            pks, zs = [], []
            sub = R // LNS
            wstart = set(np.cumsum((0,) + wgroups[:-1]).tolist())
            slot = [0]

            def lnth(n):
                out = []
                for _ in range(n):
                    out.append(LN)
                return out

            def K(c):
                if first and c in wstart:
                    g = wgroups[sorted(wstart).index(c)]
                    for cc in range(c, c + g):
                        wk_dma(cc).wait()
                nl = lnk[c]
                if nl:
                    if first and slot[0] == 0:
                        x_dma(1).wait()
                    w = tied_lhs(lambda rs, k: wqkv_v[rs, D + c * CW + k * L: D + c * CW + (k + 1) * L], D, CW // L,
                                 lnth(nl), [0, 1])
                else:
                    w = wqkv_v[:, D + c * CW: D + (c + 1) * CW]
                k = _dot(xn, w)
                pk = _phi(k)
                zs.append(jnp.sum(pk.reshape(R // 8, 8, CW), axis=0))
                pks.append(pk.astype(bf16))

            def PT(c):
                cs = slice(c * CW, (c + 1) * CW)
                nl = lnp[c]
                if nl:
                    if first and slot[0] == 0:
                        x_dma(1).wait()
                    rhs = tied_lhs(lambda rs, k: pks[c][rs, k * L:(k + 1) * L], R, CW // L, lnth(nl), [0, 1])
                else:
                    rhs = pks[c]
                r = _dg(xn, rhs, 0, 0)
                if first:
                    pt_v[:, cs] = r
                else:
                    pt_v[:, cs] += r

            def LN():
                p = slot[0]
                slot[0] += 1
                if first and p == 0 and not (sum(lnk) + sum(lnp)):
                    x_dma(1).wait()
                return ln(nxt + p * sub, sub, st, wr)

            seq = [lambda: K(0), lambda: K(1), lambda: PT(0), lambda: K(2), lambda: PT(1), lambda: K(3),
                   lambda: PT(2), lambda: PT(3)]
            for pos, f in enumerate(seq):
                f()
                for _ in range(lnpos.count(pos)):
                    LN()
            assert slot[0] == LNS
            zacc = zacc + jnp.concatenate(zs, axis=1)
            return zacc, st[0], st[1]

        zacc = jnp.zeros((8, D), f32)
        with sc("p1_it0"):
            zacc, best, bidx = p1_iter(0, zacc, best, bidx, True)

        def body1(i, carry):
            zacc, best, bidx = carry

            @pl.when(i < NI - 1)
            def _():
                x_dma(jnp.minimum(i + 1, NI - 1)).wait()

            return p1_iter(i, zacc, best, bidx, False)

        with sc("p1_loop"):
            zacc, best, bidx = lax.fori_loop(1, NI, body1, (zacc, best, bidx))

        z = jnp.sum(zacc, axis=0, keepdims=True)
        zc_v[...] = jnp.broadcast_to(z, (L, D)).T
        ri = lax.broadcasted_iota(jnp.int32, (L, L), 0) // DH
        ci = lax.broadcasted_iota(jnp.int32, (L, L), 1) // DH
        mask = ri == ci
        with sc("wait_w"):
            wq_dma.wait()
            wv_dma.wait()
            wo_dma.wait()
            if order != 'same':
                wg_dma(0).wait()
                wu_dma(0).wait()

        idx = jnp.clip(bidx[0, 0], 0, S - 1)
        g0 = pl.multiple_of((idx // 16) * 16, 16)
        xg = xn_v[pl.ds(g0, 16), :]
        gate = jax.nn.sigmoid(best)
        rr = lax.broadcasted_iota(jnp.int32, (16, 1), 0)
        xsel = jnp.sum(jnp.where(rr == idx - g0, xg.astype(f32), 0.0), axis=0, keepdims=True)
        xb_v[0:D, :] = jnp.broadcast_to(xsel, (L, D)).T
        y_v[...] = jnp.zeros((8, D), f32)
        iblk = idx // R

        def mk(load, nrows, nslab, th, on, kk=None):
            if on:
                return tied_lhs(load, nrows, nslab, th, kk)
            for t in th:
                t()
            return tied_lhs(load, nrows, nslab, [])

        def g_thunks(c, slot, zz=None):
            gu = {}
            wg = wg_v.at[c]
            wu = wu_v.at[c]

            def g_sub(jb, s):
                n = D // GS
                rs = slice(s * n, (s + 1) * n)
                cs = slice(jb * L, (jb + 1) * L)
                if zz is None:
                    xb = xb_v[rs, :]
                else:
                    xb = xb_v[pl.ds(pl.multiple_of((zz | (zz << jb)) + rs.start, 8), n), :]
                g = jnp.sum((wg[rs, cs].astype(f32) * xb).reshape(n // 8, 8, L), axis=0)
                u = jnp.sum((wu[rs, cs].astype(f32) * xb).reshape(n // 8, 8, L), axis=0)
                if s > 0:
                    g = g + gu[jb][0]
                    u = u + gu[jb][1]
                gu[jb] = (g, u)
                return pltpu.bitcast(pltpu.bitcast(g, u32) | pltpu.bitcast(u, u32), f32)

            def g_fin(jb):
                g, u = gu[jb]
                g = jnp.sum(g, axis=0, keepdims=True)
                u = jnp.sum(u, axis=0, keepdims=True)
                h = g * jax.nn.sigmoid(g) * u
                hb = jnp.broadcast_to(h, (L, L)).T
                hb_v[slot, jb * L:(jb + 1) * L, :] = hb
                return hb[0:8]

            th = []
            pend = []
            for jb in range(FB):
                for s in range(GS):
                    th.append(functools.partial(g_sub, jb, s))
                    if pend and s == finlate - 1:
                        th.append(pend.pop(0))
                pend.append(functools.partial(g_fin, jb))
                if finlate == 0:
                    th.append(pend.pop(0))
            th.extend(pend)
            return th

        def d_thunks(c, slot):
            ya = [None]
            NDS = FC // DS
            wd = wd_v.at[c]

            def d_sub(s):
                rs = slice(s * DS, (s + 1) * DS)
                hb = hb_v[slot, rs, :]
                w = wd[rs, :].astype(f32)
                parts = []
                for jb in range(NB):
                    parts.append(jnp.sum((w[:, jb * L:(jb + 1) * L] * hb).reshape(DS // 8, 8, L), axis=0))
                yy = jnp.concatenate(parts, axis=1)
                yy = yy + (ya[0] if s > 0 else y_v[...])
                ya[0] = yy
                if s == NDS - 1:
                    y_v[...] = yy
                hnd = pltpu.bitcast(yy[:, 0:L], u32)
                for jb in range(1, NB):
                    hnd = hnd | pltpu.bitcast(yy[:, jb * L:(jb + 1) * L], u32)
                return pltpu.bitcast(hnd, f32)

            return [functools.partial(d_sub, s) for s in range(NDS)]

        def g2_thunks(c, slot, fins_sep=False):
            acc = [None]
            wg = wg_v.at[c]
            wu = wu_v.at[c]
            NG = D // GR

            def sub(s):
                rs = slice(s * GR, (s + 1) * GR)
                xb = xb_v[rs, :]
                parts = []
                for w in (wg, wu):
                    wf = w[rs, :].astype(f32)
                    for jb in range(FB):
                        parts.append(jnp.sum((wf[:, jb * L:(jb + 1) * L] * xb).reshape(GR // 8, 8, L), axis=0))
                a = jnp.concatenate(parts, axis=1)
                if s > 0:
                    a = a + acc[0]
                acc[0] = a
                hnd = pltpu.bitcast(a[:, 0:L], u32)
                for jb in range(1, 2 * FB):
                    hnd = hnd | pltpu.bitcast(a[:, jb * L:(jb + 1) * L], u32)
                return pltpu.bitcast(hnd, f32)

            def fin(jb):
                g = jnp.sum(acc[0][:, jb * L:(jb + 1) * L], axis=0, keepdims=True)
                u = jnp.sum(acc[0][:, (FB + jb) * L:(FB + jb + 1) * L], axis=0, keepdims=True)
                h = g * jax.nn.sigmoid(g) * u
                hb = jnp.broadcast_to(h, (L, L)).T
                hb_v[slot, jb * L:(jb + 1) * L, :] = hb
                return hb[0:8]

            return [functools.partial(sub, s) for s in range(NG)] + [functools.partial(fin, jb) for jb in range(FB)]

        gt0 = [] if order == 'same' else (g2_thunks(0, 0) if g2 else g_thunks(0, 0))
        nk = (len(gt0) * midsplit[0]) // sum(midsplit)
        gpk = split(gt0[:nk], NB)
        gpm = split(gt0[nk:], NB)
        kvbs = []

        def kv_dot(j):
            cs = slice(j * L, (j + 1) * L)
            wv = mk(lambda rs, k: wqkv_v[rs, 2 * D + j * L: 2 * D + (j + 1) * L], D, 1, gpk[j], tie2 and tieM)
            kv = _dg(pt_v[:, cs].astype(bf16), wv, 0, 0)
            kvbs.append(jnp.where(mask, kv, 0.0).astype(bf16))

        def m_dot(j):
            cs = slice(j * L, (j + 1) * L)
            wo = mk(lambda rs, k: wo_v[j * L + rs.start: j * L + rs.stop, k * L:(k + 1) * L], L, NB, gpm[j],
                    tie2 and tieM, list(range(NB)))
            m_v[cs, :] = _dot(kvbs[j], wo).astype(bf16)

        for j in range(NB + midskew):
            if j < NB:
                kv_dot(j)
            if j >= midskew:
                m_dot(j - midskew)

        def body2(i, _):
            b = lax.rem(iblk + 1 + i, NI)
            row0 = pl.multiple_of(b * R, R)
            rows = pl.ds(row0, R)
            cn = lax.rem(i + 1, NI)
            with sc("wait_ffn"):
                wd_dma(i).wait()
                if order == 'same':
                    wg_dma(i).wait(); wu_dma(i).wait()
                else:
                    @pl.when(i < NI - 1)
                    def _():
                        wg_dma(cn).wait(); wu_dma(cn).wait()
            ridx = lax.broadcasted_iota(jnp.int32, (R, 1), 0) + row0
            HK = D // 2
            xnb = xn_v.at[rows]
            xblk = x_v.at[rows]
            oblk = out_v.at[rows]
            slot = lax.rem(i, 2)
            gt = g2_thunks(cn, 1 - slot) if g2 else g_thunks(cn, 1 - slot, (i // NI) * 8 if opq else None)
            dt = d_thunks(i, slot)
            if order == 'same':
                gt = g2_thunks(i, 0) if g2 else g_thunks(i, 0, (i // NI) * 8 if opq else None)
                dt = d_thunks(i, 0)
            if noffn:
                gt, dt = [], []
            if order == 'DH_GAC':
                na = len(gt) // 2
                qparts = split(gt[:na], NC)
                cparts = split(gt[na:], NC)
                hparts = split(dt, NC)
            elif order == 'DH_GQ':
                qparts = split(gt, NC)
                cparts = [[]] * NC
                hparts = split(dt, NC)
            elif order == 'same':
                qparts = split(gt, NC)
                nh = (len(dt) * samesplit[0]) // sum(samesplit)
                hparts = split(dt[:nh], NC)
                cparts = [dt[nh:]] + [[]] * (NC - 1)
            elif order == 'w':
                seq = {'GD': None, 'DG': dt + gt}[qw[0]]
                tot = sum(qw[1:])
                parts, a = [], 0
                for k, w in enumerate(qw[1:]):
                    e = len(seq) if k == len(qw) - 2 else a + (len(seq) * w) // tot
                    parts.append(seq[a:e]); a = e
                qparts, hparts, cparts = parts[0:4], parts[4:8], parts[8:12]
            xn = xnb[...]

            def Q(c):
                cs = slice(c * CW, (c + 1) * CW)
                rhs = mk(lambda rs, k: xn[rs, k * L:(k + 1) * L], R, NB, qparts[c], tie2, kkQ)
                qT = _dg(wqkv_v[:, cs], rhs, 0, 1)
                pq = _phi(qT)
                zc = zc_v[cs, :]
                nh = CW // DH
                for t in range(R // L):
                    p = pq[:, t * L:(t + 1) * L]
                    den = jnp.sum((p * zc).reshape(nh, DH, L), axis=1, keepdims=True) + 1e-6
                    o = (p.reshape(nh, DH, L) * rcp(den)).reshape(CW, L).astype(bf16)
                    o_v[t * L:(t + 1) * L, cs] = o.T

            def load_o(half):
                return lambda rs, k: o_v[rs, half * HK + k * L: half * HK + (k + 1) * L]

            def Hh(n):
                cs = slice(n * CW, (n + 1) * CW)
                if wtie:
                    rhs = mk(lambda rs, k: m_v[rs, n * CW + k * L: n * CW + (k + 1) * L], HK, CW // L, hparts[n], tie2, [0, 1])
                    acc_v[:, cs] = _dot(o_v[:, 0:HK], rhs)
                else:
                    lhs = mk(load_o(0), R, NB // 2, hparts[n], tie2, kkH)
                    acc_v[:, cs] = _dot(lhs, m_v[0:HK, cs])

            def C(n):
                cs = slice(n * CW, (n + 1) * CW)
                if wtie:
                    rhs = mk(lambda rs, k: m_v[HK + rs.start: HK + rs.stop, n * CW + k * L: n * CW + (k + 1) * L], HK, CW // L, cparts[n], tie2, [0, 1])
                    a = acc_v[:, cs] + _dot(o_v[:, HK:D], rhs)
                else:
                    a = acc_v[:, cs] + _dot(mk(load_o(1), R, NB // 2, cparts[n], tie2, kkH), m_v[HK:D, cs])
                y = jnp.sum(y_v[:, cs], axis=0, keepdims=True) * gate
                res = xblk[:, cs].astype(f32) + xnb[:, cs].astype(f32) + a + jnp.where(ridx == idx, y, 0.0)
                oblk[:, cs] = res.astype(bf16)
                if tailsplit:
                    o_dma(b, n).start()

            for c in range(NC):
                Q(c)
            for n in range(NC):
                Hh(n)
            for n in range(NC):
                C(n)
            if not tailsplit:
                o_dma(b).start()
            return None

        with sc("p2_loop"):
            lax.fori_loop(0, NI, body2, None)
        with sc("wait_out"):
            for b in range(NI):
                if tailsplit:
                    for n in range(NC):
                        o_dma(b, n).wait()
                else:
                    o_dma(b).wait()

    def fn(A_x, A_wqkv, A_wo, B_x, B_w_r, B_w_gate, B_w_up, B_w_down):
        anyspec = pl.BlockSpec(memory_space=pl.ANY)
        out = pl.pallas_call(
            kernel,
            out_shape=jax.ShapeDtypeStruct((S, D), bf16),
            in_specs=[anyspec] * 7,
            out_specs=anyspec,
            scratch_shapes=[
                pltpu.VMEM((S, D), bf16), pltpu.VMEM((S, D), bf16), pltpu.VMEM((D, 3 * D), bf16),
                pltpu.VMEM((D, D), bf16), pltpu.VMEM((D,), bf16),
                pltpu.VMEM((NI, D, FC), bf16), pltpu.VMEM((NI, D, FC), bf16), pltpu.VMEM((NI, FC, D), bf16),
                pltpu.VMEM((S, D), bf16), pltpu.VMEM((D, D), f32), pltpu.VMEM((D, L), f32),
                pltpu.VMEM((D, D), bf16), pltpu.VMEM((D + 8 * 128, L), f32),
                pltpu.VMEM((R, D), bf16), pltpu.VMEM((R, D), f32),
                pltpu.VMEM((2, FC, L), f32), pltpu.VMEM((8, D), f32),
                pltpu.SemaphoreType.DMA((NSEM,)),
            ],
            compiler_params=pltpu.CompilerParams(vmem_limit_bytes=100 * 1024 * 1024, flags=flags,
                                                 disable_semaphore_checks=nosemchk),
        )(A_x.reshape(S, D), A_wqkv, A_wo, B_w_r, B_w_gate, B_w_up, B_w_down)
        return out.reshape(1, S, D)
    return fn


_IMPL = make(**dict(order='w',qw=('DG',2,2,2,2,2,2,2,2,2,2,2,2),g2=True,GR=16,DS=16,wtie=True,tieM=False,flags={'XLA_TPU_EVENLY_DISTRIBUTE_CRITICAL_NODES':True}))


@jax.jit
def pallas_parallel_sum__linear_attn_block__moe_arch_mod__prompt_kernel(
    A_x: jax.Array,
    A_wqkv: jax.Array,
    A_wo: jax.Array,
    B_x: jax.Array,
    B_w_r: jax.Array,
    B_w_gate: jax.Array,
    B_w_up: jax.Array,
    B_w_down: jax.Array,
):
    return _IMPL(A_x, A_wqkv, A_wo, B_x, B_w_r, B_w_gate, B_w_up, B_w_down)
```

```python
import functools, contextlib
import numpy as np
import jax
import jax.numpy as jnp
from jax import lax
import jax.experimental.pallas as pl
import jax.experimental.pallas.tpu as pltpu

S, D, H, DH, F = 2048, 1024, 32, 32, 3584
L = 128
NB = D // L
f32, bf16, u32 = jnp.float32, jnp.bfloat16, jnp.uint32


def _phi(t):
    return jnp.where(t > 0, t + 1.0, jnp.exp(t)) + 1e-6


def _dot(a, b):
    return jnp.dot(a, b, preferred_element_type=f32)


def _dg(a, b, ca, cb):
    return lax.dot_general(a, b, (((ca,), (cb,)), ((), ())), preferred_element_type=f32)


def _zero(v):
    b = pltpu.bitcast(v, u32)
    return lax.shift_right_logical(lax.shift_right_logical(b, jnp.uint32(31)), jnp.uint32(1))


def _tie(xv, z):
    return pltpu.bitcast(pltpu.bitcast(xv, u32) | z, bf16)


def tied_lhs(load, nrows, nslab, thunks, kk=None):
    n = len(thunks)
    if n == 0:
        return jnp.concatenate([load(slice(0, nrows), k) for k in range(nslab)], axis=1)
    if kk is None:
        kk = [k for k in range(0, nslab, 2)]
    per = -(-n // len(kk))
    npos = 1
    while npos < per * len(kk) and npos < nrows // 16:
        npos *= 2
    step = nrows // npos
    slabs = []
    order = {}
    for p in range(n):
        m, q = divmod(p, per)
        r = (q * npos) // per + (m * npos) // (per * len(kk))
        order.setdefault((kk[m], min(r, npos - 1)), []).append(p)
    zs = {}
    for p in range(n):
        v = thunks[p]()
        zs[p] = None if v is None else _zero(v)
    for k in range(nslab):
        if k not in kk:
            slabs.append(load(slice(0, nrows), k))
            continue
        parts = []
        for r in range(npos):
            ps = [zs[p] for p in order.get((k, r), []) if zs[p] is not None]
            if not ps:
                parts.append(load(slice(r * step, (r + 1) * step), k))
            else:
                z = ps[0]
                for z2 in ps[1:]:
                    z = z | z2
                parts.append(_tie(load(slice(r * step, r * step + 16), k), z))
                if step > 16:
                    parts.append(load(slice(r * step + 16, (r + 1) * step), k))
        slabs.append(jnp.concatenate(parts, axis=0))
    return jnp.concatenate(slabs, axis=1)


def split(lst, n):
    k = -(-len(lst) // n) if lst else 0
    return [lst[a * k:(a + 1) * k] for a in range(n)]


def make(R=512, scopes=False, recip="nr", flags=None, tie2=True, tieM=True, LNS=4, GS=8, DS=32,
         kkQ=None, kkH=None, order='DH_GAC', x0parts=4, finlate=4, nosemchk=False,
         lnpos=(2, 3, 4, 5), lnpos0=(3, 4, 5, 6), opq=True, qw=None, noffn=False, ksplit=True, g2=False, GR=16, wtie=False, lnk=(0, 0, 0, 0), lnp=(0, 0, 0, 0), midsplit=(1, 1), midskew=8, samesplit=(1, 0)):
    sc = (lambda n: jax.named_scope(n)) if scopes else (lambda n: contextlib.nullcontext())
    NI = S // R
    CW = 256
    NC = D // CW
    FC = F // NI
    FB = FC // L

    def rcp(x):
        if recip == "approx":
            return pl.reciprocal(x, approx=True)
        if recip == "nr":
            r = pl.reciprocal(x, approx=True)
            return r * (2.0 - x * r)
        return pl.reciprocal(x, approx=False)

    NX0 = x0parts
    SX0, SWR, SWK = 0, NX0, NX0 + 1
    SX = SWK + 4
    SW = SX + NI - 1
    SF = SW + 1
    SO = SF + 2
    NSEM = SO + 1

    def kernel(x_hbm, wqkv_hbm, wo_hbm, wr_hbm, wg_hbm, wu_hbm, wd_hbm, out_hbm,
               x_v, xn_v, wqkv_v, wo_v, wr_v, wg_v, wu_v, wd_v, out_v, pt_v, zc_v, m_v, xb_v, o_v, acc_v, hb_v, y_v,
               sems):
        XR = R // NX0

        def x0_dma(h):
            return pltpu.make_async_copy(x_hbm.at[pl.ds(h * XR, XR)], x_v.at[pl.ds(h * XR, XR)], sems.at[SX0 + h])

        wr_dma = pltpu.make_async_copy(wr_hbm, wr_v, sems.at[SWR])
        wk_cols = [(0, L), (L, L), (CW, CW), (2 * CW, 2 * CW)]

        def wk_dma(g):
            cs = pl.ds(D + wk_cols[g][0], wk_cols[g][1])
            return pltpu.make_async_copy(wqkv_hbm.at[:, cs], wqkv_v.at[:, cs], sems.at[SWK + g])

        def x_dma(i):
            return pltpu.make_async_copy(x_hbm.at[pl.ds(i * R, R)], x_v.at[pl.ds(i * R, R)], sems.at[SX + i - 1])

        wq_dma = pltpu.make_async_copy(wqkv_hbm.at[:, pl.ds(0, D)], wqkv_v.at[:, pl.ds(0, D)], sems.at[SW])
        wv_dma = pltpu.make_async_copy(wqkv_hbm.at[:, pl.ds(2 * D, D)], wqkv_v.at[:, pl.ds(2 * D, D)], sems.at[SW])
        wo_dma = pltpu.make_async_copy(wo_hbm, wo_v, sems.at[SW])

        def wg_dma(c):
            return pltpu.make_async_copy(wg_hbm.at[:, pl.ds(c * FC, FC)], wg_v.at[c], sems.at[SF + (c > 0)])

        def wu_dma(c):
            return pltpu.make_async_copy(wu_hbm.at[:, pl.ds(c * FC, FC)], wu_v.at[c], sems.at[SF + (c > 0)])

        def wd_dma(c):
            return pltpu.make_async_copy(wd_hbm.at[pl.ds(c * FC, FC)], wd_v.at[c], sems.at[SF + 1])

        def o_dma(b, n):
            rows = pl.ds(pl.multiple_of(b * R, R), R)
            cs = pl.ds(n * CW, CW)
            return pltpu.make_async_copy(out_v.at[rows, cs], out_hbm.at[rows, cs], sems.at[SO])

        for h in range(NX0):
            x0_dma(h).start()
            if h == 0:
                wr_dma.start()
        for g in range(4):
            wk_dma(g).start()
        for i in range(1, NI):
            x_dma(i).start()
        wq_dma.start()
        wv_dma.start()
        wo_dma.start()
        for c in range(NI):
            wg_dma(c).start()
            wu_dma(c).start()
        for c in range(NI):
            wd_dma(c).start()

        def ln(row0, n, st, wr):
            best, bidx = st
            rows = pl.ds(row0, n)
            x = x_v[rows, :].astype(f32)
            m = jnp.mean(x, axis=-1, keepdims=True)
            d = x - m
            v = jnp.mean(d * d, axis=-1, keepdims=True)
            xn = d * lax.rsqrt(v + 1e-5)
            xn_v[rows, :] = xn.astype(bf16)
            r = jnp.broadcast_to(jnp.sum(xn * wr, axis=-1, keepdims=True), (n, L))
            sub_iota = lax.broadcasted_iota(jnp.int32, (8, L), 0) + row0
            for g in range(n // 8):
                rg = r[8 * g:8 * g + 8]
                better = rg > best
                best = jnp.where(better, rg, best)
                bidx = jnp.where(better, sub_iota + 8 * g, bidx)
            st[0], st[1] = best, bidx
            hnd = pltpu.bitcast(best, u32)
            for g in range(n // 8):
                hnd = hnd | pltpu.bitcast(xn[8 * g:8 * g + 8, D - L:D], u32)
            return pltpu.bitcast(hnd, f32)

        st = [jnp.full((8, L), -jnp.inf, f32), jnp.full((8, L), S, jnp.int32)]
        for h in range(NX0):
            with sc("wait_x0"):
                x0_dma(h).wait()
                if h == 0:
                    wr_dma.wait()
            if h == 0:
                wr0 = wr_v[...].astype(f32).reshape(1, D)
            ln(h * XR, XR, st, wr0)
        best, bidx = st

        def p1_iter(i, zacc, best, bidx, first):
            row0 = 0 if first else pl.multiple_of(i * R, R)
            rows = pl.ds(row0, R)
            nxt = R if first else pl.multiple_of(lax.rem(i + 1, NI) * R, R)
            st = [best, bidx]
            wr = wr_v[...].astype(f32).reshape(1, D)
            if first:
                wk_dma(0).wait()
            xn = xn_v[rows, :]
            pks, zs = [], []
            sub = R // LNS
            slot = [0]

            def lnth(n):
                out = []
                for _ in range(n):
                    out.append(LN)
                return out

            def K(c):
                if first and c == 0:
                    k0 = _dot(xn, wqkv_v[:, D: D + L])
                    wk_dma(1).wait()
                    k1 = _dot(xn, wqkv_v[:, D + L: D + 2 * L])
                    pk = _phi(jnp.concatenate([k0, k1], axis=1))
                    zs.append(jnp.sum(pk.reshape(R // 8, 8, CW), axis=0))
                    pks.append(pk.astype(bf16))
                    return
                if first and c in (1, 2):
                    wk_dma(c + 1).wait()
                    if c == 2:
                        x_dma(1).wait()
                nl = lnk[c]
                if nl:
                    w = tied_lhs(lambda rs, k: wqkv_v[rs, D + c * CW + k * L: D + c * CW + (k + 1) * L], D, CW // L,
                                 lnth(nl), [0, 1])
                else:
                    w = wqkv_v[:, D + c * CW: D + (c + 1) * CW]
                k = _dot(xn, w)
                pk = _phi(k)
                zs.append(jnp.sum(pk.reshape(R // 8, 8, CW), axis=0))
                pks.append(pk.astype(bf16))

            def PT(c):
                cs = slice(c * CW, (c + 1) * CW)
                nl = lnp[c]
                if nl:
                    rhs = tied_lhs(lambda rs, k: pks[c][rs, k * L:(k + 1) * L], R, CW // L, lnth(nl), [0, 1])
                else:
                    rhs = pks[c]
                r = _dg(xn, rhs, 0, 0)
                if first:
                    pt_v[:, cs] = r
                else:
                    pt_v[:, cs] += r

            def LN():
                p = slot[0]
                slot[0] += 1
                return ln(nxt + p * sub, sub, st, wr)

            seq = [lambda: K(0), lambda: K(1), lambda: PT(0), lambda: K(2), lambda: PT(1), lambda: K(3),
                   lambda: PT(2), lambda: PT(3)]
            for pos, f in enumerate(seq):
                f()
                for _ in range((lnpos0 if first else lnpos).count(pos)):
                    LN()
            assert slot[0] == LNS
            zacc = zacc + jnp.concatenate(zs, axis=1)
            return zacc, st[0], st[1]

        zacc = jnp.zeros((8, D), f32)
        with sc("p1_it0"):
            zacc, best, bidx = p1_iter(0, zacc, best, bidx, True)

        def body1(i, carry):
            zacc, best, bidx = carry

            @pl.when(i < NI - 1)
            def _():
                x_dma(jnp.minimum(i + 1, NI - 1)).wait()

            @pl.when(i == NI - 1)
            def _():
                wq_dma.wait()
                wv_dma.wait()
                wo_dma.wait()
                if order != 'same':
                    wg_dma(0).wait()
                    wu_dma(0).wait()

            return p1_iter(i, zacc, best, bidx, False)

        with sc("p1_loop"):
            zacc, best, bidx = lax.fori_loop(1, NI, body1, (zacc, best, bidx))

        z = jnp.sum(zacc, axis=0, keepdims=True)
        zc_v[...] = jnp.broadcast_to(z, (L, D)).T
        ri = lax.broadcasted_iota(jnp.int32, (L, L), 0) // DH
        ci = lax.broadcasted_iota(jnp.int32, (L, L), 1) // DH
        mask = ri == ci
        bmax = jnp.max(best, axis=0, keepdims=True)
        idx = jnp.clip(jnp.min(jnp.where(best == bmax, bidx, S)), 0, S - 1)
        g0 = pl.multiple_of((idx // 16) * 16, 16)
        xg = xn_v[pl.ds(g0, 16), :]
        gate = jax.nn.sigmoid(bmax[:, 0:1])
        rr = lax.broadcasted_iota(jnp.int32, (16, 1), 0)
        xsel = jnp.sum(jnp.where(rr == idx - g0, xg.astype(f32), 0.0), axis=0, keepdims=True)
        xb_v[0:D, :] = jnp.broadcast_to(xsel, (L, D)).T
        y_v[...] = jnp.zeros((8, D), f32)
        iblk = idx // R

        def mk(load, nrows, nslab, th, on, kk=None):
            if on:
                return tied_lhs(load, nrows, nslab, th, kk)
            for t in th:
                t()
            return tied_lhs(load, nrows, nslab, [])

        def g_thunks(c, slot, zz=None):
            gu = {}
            wg = wg_v.at[c]
            wu = wu_v.at[c]

            def g_sub(jb, s):
                n = D // GS
                rs = slice(s * n, (s + 1) * n)
                cs = slice(jb * L, (jb + 1) * L)
                if zz is None:
                    xb = xb_v[rs, :]
                else:
                    xb = xb_v[pl.ds(pl.multiple_of((zz | (zz << jb)) + rs.start, 8), n), :]
                g = jnp.sum((wg[rs, cs].astype(f32) * xb).reshape(n // 8, 8, L), axis=0)
                u = jnp.sum((wu[rs, cs].astype(f32) * xb).reshape(n // 8, 8, L), axis=0)
                if s > 0:
                    g = g + gu[jb][0]
                    u = u + gu[jb][1]
                gu[jb] = (g, u)
                return pltpu.bitcast(pltpu.bitcast(g, u32) | pltpu.bitcast(u, u32), f32)

            def g_fin(jb):
                g, u = gu[jb]
                g = jnp.sum(g, axis=0, keepdims=True)
                u = jnp.sum(u, axis=0, keepdims=True)
                h = g * jax.nn.sigmoid(g) * u
                hb = jnp.broadcast_to(h, (L, L)).T
                hb_v[slot, jb * L:(jb + 1) * L, :] = hb
                return hb[0:8]

            th = []
            pend = []
            for jb in range(FB):
                for s in range(GS):
                    th.append(functools.partial(g_sub, jb, s))
                    if pend and s == finlate - 1:
                        th.append(pend.pop(0))
                pend.append(functools.partial(g_fin, jb))
                if finlate == 0:
                    th.append(pend.pop(0))
            th.extend(pend)
            return th

        def d_thunks(c, slot):
            ya = [None]
            NDS = FC // DS
            wd = wd_v.at[c]

            def d_sub(s):
                rs = slice(s * DS, (s + 1) * DS)
                hb = hb_v[slot, rs, :]
                w = wd[rs, :].astype(f32)
                parts = []
                for jb in range(NB):
                    parts.append(jnp.sum((w[:, jb * L:(jb + 1) * L] * hb).reshape(DS // 8, 8, L), axis=0))
                yy = jnp.concatenate(parts, axis=1)
                yy = yy + (ya[0] if s > 0 else y_v[...])
                ya[0] = yy
                if s == NDS - 1:
                    y_v[...] = yy
                hnd = pltpu.bitcast(yy[:, 0:L], u32)
                for jb in range(1, NB):
                    hnd = hnd | pltpu.bitcast(yy[:, jb * L:(jb + 1) * L], u32)
                return pltpu.bitcast(hnd, f32)

            return [functools.partial(d_sub, s) for s in range(NDS)]

        def g2_thunks(c, slot, fins_sep=False):
            acc = [None]
            wg = wg_v.at[c]
            wu = wu_v.at[c]
            NG = D // GR

            def sub(s):
                rs = slice(s * GR, (s + 1) * GR)
                xb = xb_v[rs, :]
                parts = []
                for w in (wg, wu):
                    wf = w[rs, :].astype(f32)
                    for jb in range(FB):
                        parts.append(jnp.sum((wf[:, jb * L:(jb + 1) * L] * xb).reshape(GR // 8, 8, L), axis=0))
                a = jnp.concatenate(parts, axis=1)
                if s > 0:
                    a = a + acc[0]
                acc[0] = a
                hnd = pltpu.bitcast(a[:, 0:L], u32)
                for jb in range(1, 2 * FB):
                    hnd = hnd | pltpu.bitcast(a[:, jb * L:(jb + 1) * L], u32)
                return pltpu.bitcast(hnd, f32)

            def fin(jb):
                g = jnp.sum(acc[0][:, jb * L:(jb + 1) * L], axis=0, keepdims=True)
                u = jnp.sum(acc[0][:, (FB + jb) * L:(FB + jb + 1) * L], axis=0, keepdims=True)
                h = g * jax.nn.sigmoid(g) * u
                hb = jnp.broadcast_to(h, (L, L)).T
                hb_v[slot, jb * L:(jb + 1) * L, :] = hb
                return hb[0:8]

            return [functools.partial(sub, s) for s in range(NG)] + [functools.partial(fin, jb) for jb in range(FB)]

        gt0 = [] if order == 'same' else (g2_thunks(0, 0) if g2 else g_thunks(0, 0))
        nk = (len(gt0) * midsplit[0]) // sum(midsplit)
        gpk = split(gt0[:nk], NB)
        gpm = split(gt0[nk:], NB)
        kvbs = []

        def kv_dot(j):
            cs = slice(j * L, (j + 1) * L)
            wv = mk(lambda rs, k: wqkv_v[rs, 2 * D + j * L: 2 * D + (j + 1) * L], D, 1, gpk[j], tie2 and tieM)
            kv = _dg(pt_v[:, cs].astype(bf16), wv, 0, 0)
            kvbs.append(jnp.where(mask, kv, 0.0).astype(bf16))

        def m_dot(j):
            cs = slice(j * L, (j + 1) * L)
            wo = mk(lambda rs, k: wo_v[j * L + rs.start: j * L + rs.stop, k * L:(k + 1) * L], L, NB, gpm[j],
                    tie2 and tieM, list(range(NB)))
            m_v[cs, :] = _dot(kvbs[j], wo).astype(bf16)

        for j in range(NB + midskew):
            if j < NB:
                kv_dot(j)
            if j >= midskew:
                m_dot(j - midskew)

        def body2(i, _):
            b = lax.rem(iblk + 1 + i, NI)
            row0 = pl.multiple_of(b * R, R)
            rows = pl.ds(row0, R)
            cn = lax.rem(i + 1, NI)
            ridx = lax.broadcasted_iota(jnp.int32, (R, 1), 0) + row0
            HK = D // 2
            xnb = xn_v.at[rows]
            xblk = x_v.at[rows]
            oblk = out_v.at[rows]
            slot = lax.rem(i, 2)
            gt = g2_thunks(cn, 1 - slot) if g2 else g_thunks(cn, 1 - slot, (i // NI) * 8 if opq else None)
            dt = d_thunks(i, slot)
            if order == 'same':
                gt = g2_thunks(i, 0) if g2 else g_thunks(i, 0, (i // NI) * 8 if opq else None)
                dt = d_thunks(i, 0)
            if noffn:
                gt, dt = [], []
            if order == 'DH_GAC':
                na = len(gt) // 2
                qparts = split(gt[:na], NC)
                cparts = split(gt[na:], NC)
                hparts = split(dt, NC)
            elif order == 'DH_GQ':
                qparts = split(gt, NC)
                cparts = [[]] * NC
                hparts = split(dt, NC)
            elif order == 'same':
                qparts = split(gt, NC)
                nh = (len(dt) * samesplit[0]) // sum(samesplit)
                hparts = split(dt[:nh], NC)
                cparts = [dt[nh:]] + [[]] * (NC - 1)
            elif order == 'w':
                seq = {'GD': None, 'DG': dt + gt}[qw[0]]
                tot = sum(qw[1:])
                parts, a = [], 0
                for k, w in enumerate(qw[1:]):
                    e = len(seq) if k == len(qw) - 2 else a + (len(seq) * w) // tot
                    parts.append(seq[a:e]); a = e
                qparts, hparts, cparts = parts[0:4], parts[4:8], parts[8:12]
            xn = xnb[...]

            def Q(c):
                cs = slice(c * CW, (c + 1) * CW)
                rhs = mk(lambda rs, k: xn[rs, k * L:(k + 1) * L], R, NB, qparts[c], tie2, kkQ)
                qT = _dg(wqkv_v[:, cs], rhs, 0, 1)
                pq = _phi(qT)
                zc = zc_v[cs, :]
                nh = CW // DH
                for t in range(R // L):
                    p = pq[:, t * L:(t + 1) * L]
                    den = jnp.sum((p * zc).reshape(nh, DH, L), axis=1, keepdims=True) + 1e-6
                    o = (p.reshape(nh, DH, L) * rcp(den)).reshape(CW, L).astype(bf16)
                    o_v[t * L:(t + 1) * L, cs] = o.T

            def load_o(half):
                return lambda rs, k: o_v[rs, half * HK + k * L: half * HK + (k + 1) * L]

            def Hh(n):
                cs = slice(n * CW, (n + 1) * CW)
                if wtie:
                    rhs = mk(lambda rs, k: m_v[rs, n * CW + k * L: n * CW + (k + 1) * L], HK, CW // L, hparts[n], tie2, [0, 1])
                    acc_v[:, cs] = _dot(o_v[:, 0:HK], rhs)
                else:
                    lhs = mk(load_o(0), R, NB // 2, hparts[n], tie2, kkH)
                    acc_v[:, cs] = _dot(lhs, m_v[0:HK, cs])

            def C(n):
                cs = slice(n * CW, (n + 1) * CW)
                if wtie:
                    rhs = mk(lambda rs, k: m_v[HK + rs.start: HK + rs.stop, n * CW + k * L: n * CW + (k + 1) * L], HK, CW // L, cparts[n], tie2, [0, 1])
                    a = acc_v[:, cs] + _dot(o_v[:, HK:D], rhs)
                else:
                    a = acc_v[:, cs] + _dot(mk(load_o(1), R, NB // 2, cparts[n], tie2, kkH), m_v[HK:D, cs])
                y = jnp.sum(y_v[:, cs], axis=0, keepdims=True) * gate
                res = xblk[:, cs].astype(f32) + xnb[:, cs].astype(f32) + a + jnp.where(ridx == idx, y, 0.0)
                oblk[:, cs] = res.astype(bf16)
                o_dma(b, n).start()

            for c in range(NC):
                Q(c)
            for n in range(NC):
                Hh(n)
            for n in range(NC):
                C(n)
            return None

        with sc("wait_ffn"):
            if order == 'same':
                wg_dma(0).wait()
                wu_dma(0).wait()
            for c in range(1, NI):
                wg_dma(c).wait()
                wu_dma(c).wait()
            for c in range(NI):
                wd_dma(c).wait()
        with sc("p2_loop"):
            lax.fori_loop(0, NI, body2, None)
        with sc("wait_out"):
            for b in range(NI):
                for n in range(NC):
                    o_dma(b, n).wait()

    def fn(A_x, A_wqkv, A_wo, B_x, B_w_r, B_w_gate, B_w_up, B_w_down):
        anyspec = pl.BlockSpec(memory_space=pl.ANY)
        out = pl.pallas_call(
            kernel,
            out_shape=jax.ShapeDtypeStruct((S, D), bf16),
            in_specs=[anyspec] * 7,
            out_specs=anyspec,
            scratch_shapes=[
                pltpu.VMEM((S, D), bf16), pltpu.VMEM((S, D), bf16), pltpu.VMEM((D, 3 * D), bf16),
                pltpu.VMEM((D, D), bf16), pltpu.VMEM((D,), bf16),
                pltpu.VMEM((NI, D, FC), bf16), pltpu.VMEM((NI, D, FC), bf16), pltpu.VMEM((NI, FC, D), bf16),
                pltpu.VMEM((S, D), bf16), pltpu.VMEM((D, D), f32), pltpu.VMEM((D, L), f32),
                pltpu.VMEM((D, D), bf16), pltpu.VMEM((D + 8 * 128, L), f32),
                pltpu.VMEM((R, D), bf16), pltpu.VMEM((R, D), f32),
                pltpu.VMEM((2, FC, L), f32), pltpu.VMEM((8, D), f32),
                pltpu.SemaphoreType.DMA((NSEM,)),
            ],
            compiler_params=pltpu.CompilerParams(vmem_limit_bytes=100 * 1024 * 1024, flags=flags,
                                                 disable_semaphore_checks=nosemchk),
        )(A_x.reshape(S, D), A_wqkv, A_wo, B_w_r, B_w_gate, B_w_up, B_w_down)
        return out.reshape(1, S, D)
    return fn


_IMPL = make(**dict(order='w',qw=('DG',2,2,2,2,2,2,2,2,2,2,2,2),g2=True,GR=16,DS=16,wtie=True,tieM=False,flags={'XLA_TPU_EVENLY_DISTRIBUTE_CRITICAL_NODES':True}))


@jax.jit
def pallas_parallel_sum__linear_attn_block__moe_arch_mod__prompt_kernel(
    A_x: jax.Array,
    A_wqkv: jax.Array,
    A_wo: jax.Array,
    B_x: jax.Array,
    B_w_r: jax.Array,
    B_w_gate: jax.Array,
    B_w_up: jax.Array,
    B_w_down: jax.Array,
):
    return _IMPL(A_x, A_wqkv, A_wo, B_x, B_w_r, B_w_gate, B_w_up, B_w_down)
```

```python
import functools, contextlib
import numpy as np
import jax
import jax.numpy as jnp
from jax import lax
import jax.experimental.pallas as pl
import jax.experimental.pallas.tpu as pltpu

S, D, H, DH, F = 2048, 1024, 32, 32, 3584
L = 128
NB = D // L
f32, bf16, u32 = jnp.float32, jnp.bfloat16, jnp.uint32


def _phi(t):
    return jnp.where(t > 0, t + 1.0, jnp.exp(t)) + 1e-6


def _dot(a, b):
    return jnp.dot(a, b, preferred_element_type=f32)


def _dg(a, b, ca, cb):
    return lax.dot_general(a, b, (((ca,), (cb,)), ((), ())), preferred_element_type=f32)


def _zero(v):
    b = pltpu.bitcast(v, u32)
    return lax.shift_right_logical(lax.shift_right_logical(b, jnp.uint32(31)), jnp.uint32(1))


def _tie(xv, z):
    return pltpu.bitcast(pltpu.bitcast(xv, u32) | z, bf16)


def tied_lhs(load, nrows, nslab, thunks, kk=None):
    n = len(thunks)
    if n == 0:
        return jnp.concatenate([load(slice(0, nrows), k) for k in range(nslab)], axis=1)
    if kk is None:
        kk = [k for k in range(0, nslab, 2)]
    per = -(-n // len(kk))
    npos = 1
    while npos < per * len(kk) and npos < nrows // 16:
        npos *= 2
    step = nrows // npos
    slabs = []
    order = {}
    for p in range(n):
        m, q = divmod(p, per)
        r = (q * npos) // per + (m * npos) // (per * len(kk))
        order.setdefault((kk[m], min(r, npos - 1)), []).append(p)
    zs = {}
    for p in range(n):
        v = thunks[p]()
        zs[p] = None if v is None else _zero(v)
    for k in range(nslab):
        if k not in kk:
            slabs.append(load(slice(0, nrows), k))
            continue
        parts = []
        for r in range(npos):
            ps = [zs[p] for p in order.get((k, r), []) if zs[p] is not None]
            if not ps:
                parts.append(load(slice(r * step, (r + 1) * step), k))
            else:
                z = ps[0]
                for z2 in ps[1:]:
                    z = z | z2
                parts.append(_tie(load(slice(r * step, r * step + 16), k), z))
                if step > 16:
                    parts.append(load(slice(r * step + 16, (r + 1) * step), k))
        slabs.append(jnp.concatenate(parts, axis=0))
    return jnp.concatenate(slabs, axis=1)


def split(lst, n):
    k = -(-len(lst) // n) if lst else 0
    return [lst[a * k:(a + 1) * k] for a in range(n)]


def make(R=512, scopes=False, recip="nr", flags=None, tie2=True, tieM=True, LNS=4, GS=8, DS=32,
         kkQ=None, kkH=None, order='DH_GAC', x0parts=4, finlate=4, nosemchk=False,
         lnpos=(2, 3, 4, 5), lnpos0=(3, 4, 5, 6), opq=True, qw=None, noffn=False, ksplit=True, g2=False, GR=16, wtie=False, lnk=(0, 0, 0, 0), lnp=(0, 0, 0, 0), midsplit=(1, 1), midskew=8, samesplit=(1, 0), resH=True, ypatch=True, defer=False, fint='first', kkQ0=None, wqt=None):
    sc = (lambda n: jax.named_scope(n)) if scopes else (lambda n: contextlib.nullcontext())
    NI = S // R
    CW = 256
    NC = D // CW
    FC = F // NI
    FB = FC // L

    def rcp(x):
        if recip == "approx":
            return pl.reciprocal(x, approx=True)
        if recip == "nr":
            r = pl.reciprocal(x, approx=True)
            return r * (2.0 - x * r)
        return pl.reciprocal(x, approx=False)

    NX0 = x0parts
    SX0, SWR, SWK = 0, NX0, NX0 + 1
    SX = SWK + 4
    SW = SX + NI - 1
    SF = SW + 1
    SO = SF + 2
    NSEM = SO + 1

    def kernel(x_hbm, wqkv_hbm, wo_hbm, wr_hbm, wg_hbm, wu_hbm, wd_hbm, out_hbm,
               x_v, xn_v, wqkv_v, wo_v, wr_v, wg_v, wu_v, wd_v, out_v, pt_v, zc_v, m_v, xb_v, o_v, acc_v, hb_v, y_v, gu_v, wqt_v,
               sems):
        XR = R // NX0

        def x0_dma(h):
            return pltpu.make_async_copy(x_hbm.at[pl.ds(h * XR, XR)], x_v.at[pl.ds(h * XR, XR)], sems.at[SX0 + h])

        wr_dma = pltpu.make_async_copy(wr_hbm, wr_v, sems.at[SWR])
        wk_cols = [(0, L), (L, L), (CW, CW), (2 * CW, 2 * CW)]

        def wk_dma(g):
            cs = pl.ds(D + wk_cols[g][0], wk_cols[g][1])
            return pltpu.make_async_copy(wqkv_hbm.at[:, cs], wqkv_v.at[:, cs], sems.at[SWK + g])

        def x_dma(i):
            return pltpu.make_async_copy(x_hbm.at[pl.ds(i * R, R)], x_v.at[pl.ds(i * R, R)], sems.at[SX + i - 1])

        wq_dma = pltpu.make_async_copy(wqkv_hbm.at[:, pl.ds(0, D)], wqkv_v.at[:, pl.ds(0, D)], sems.at[SW])
        wv_dma = pltpu.make_async_copy(wqkv_hbm.at[:, pl.ds(2 * D, D)], wqkv_v.at[:, pl.ds(2 * D, D)], sems.at[SW])
        wo_dma = pltpu.make_async_copy(wo_hbm, wo_v, sems.at[SW])

        def wg_dma(c):
            return pltpu.make_async_copy(wg_hbm.at[:, pl.ds(c * FC, FC)], wg_v.at[c], sems.at[SF + (c > 0)])

        def wu_dma(c):
            return pltpu.make_async_copy(wu_hbm.at[:, pl.ds(c * FC, FC)], wu_v.at[c], sems.at[SF + (c > 0)])

        def wd_dma(c):
            return pltpu.make_async_copy(wd_hbm.at[pl.ds(c * FC, FC)], wd_v.at[c], sems.at[SF + 1])

        def o_dma(b, n):
            rows = pl.ds(pl.multiple_of(b * R, R), R)
            cs = pl.ds(n * CW, CW)
            return pltpu.make_async_copy(out_v.at[rows, cs], out_hbm.at[rows, cs], sems.at[SO])

        for h in range(NX0):
            x0_dma(h).start()
            if h == 0:
                wr_dma.start()
        for g in range(4):
            wk_dma(g).start()
        for i in range(1, NI):
            x_dma(i).start()
        wq_dma.start()
        wv_dma.start()
        wo_dma.start()
        for c in range(NI):
            wg_dma(c).start()
            wu_dma(c).start()
        for c in range(NI):
            wd_dma(c).start()

        def ln(row0, n, st, wr):
            best, bidx = st
            rows = pl.ds(row0, n)
            x = x_v[rows, :].astype(f32)
            m = jnp.mean(x, axis=-1, keepdims=True)
            d = x - m
            v = jnp.mean(d * d, axis=-1, keepdims=True)
            xn = d * lax.rsqrt(v + 1e-5)
            xn_v[rows, :] = xn.astype(bf16)
            r = jnp.broadcast_to(jnp.sum(xn * wr, axis=-1, keepdims=True), (n, L))
            sub_iota = lax.broadcasted_iota(jnp.int32, (8, L), 0) + row0
            for g in range(n // 8):
                rg = r[8 * g:8 * g + 8]
                better = rg > best
                best = jnp.where(better, rg, best)
                bidx = jnp.where(better, sub_iota + 8 * g, bidx)
            st[0], st[1] = best, bidx
            hnd = pltpu.bitcast(best, u32)
            for g in range(n // 8):
                hnd = hnd | pltpu.bitcast(xn[8 * g:8 * g + 8, D - L:D], u32)
            return pltpu.bitcast(hnd, f32)

        st = [jnp.full((8, L), -jnp.inf, f32), jnp.full((8, L), S, jnp.int32)]
        for h in range(NX0):
            with sc("wait_x0"):
                x0_dma(h).wait()
                if h == 0:
                    wr_dma.wait()
            if h == 0:
                wr0 = wr_v[...].astype(f32).reshape(1, D)
            ln(h * XR, XR, st, wr0)
        best, bidx = st

        def p1_iter(i, zacc, best, bidx, first):
            row0 = 0 if first else pl.multiple_of(i * R, R)
            rows = pl.ds(row0, R)
            nxt = R if first else pl.multiple_of(lax.rem(i + 1, NI) * R, R)
            st = [best, bidx]
            wr = wr_v[...].astype(f32).reshape(1, D)
            if first:
                wk_dma(0).wait()
            xn = xn_v[rows, :]
            pks, zs = [], []
            sub = R // LNS
            slot = [0]

            def lnth(n):
                out = []
                for _ in range(n):
                    out.append(LN)
                return out

            def K(c):
                if first and c == 0:
                    k0 = _dot(xn, wqkv_v[:, D: D + L])
                    wk_dma(1).wait()
                    k1 = _dot(xn, wqkv_v[:, D + L: D + 2 * L])
                    pk = _phi(jnp.concatenate([k0, k1], axis=1))
                    zs.append(jnp.sum(pk.reshape(R // 8, 8, CW), axis=0))
                    pks.append(pk.astype(bf16))
                    return
                if first and c in (1, 2):
                    wk_dma(c + 1).wait()
                    if c == 2:
                        x_dma(1).wait()
                nl = lnk[c]
                if nl:
                    w = tied_lhs(lambda rs, k: wqkv_v[rs, D + c * CW + k * L: D + c * CW + (k + 1) * L], D, CW // L,
                                 lnth(nl), [0, 1])
                else:
                    w = wqkv_v[:, D + c * CW: D + (c + 1) * CW]
                k = _dot(xn, w)
                pk = _phi(k)
                zs.append(jnp.sum(pk.reshape(R // 8, 8, CW), axis=0))
                pks.append(pk.astype(bf16))

            def PT(c):
                cs = slice(c * CW, (c + 1) * CW)
                nl = lnp[c]
                if nl:
                    rhs = tied_lhs(lambda rs, k: pks[c][rs, k * L:(k + 1) * L], R, CW // L, lnth(nl), [0, 1])
                else:
                    rhs = pks[c]
                r = _dg(xn, rhs, 0, 0)
                if first:
                    pt_v[:, cs] = r
                else:
                    pt_v[:, cs] += r

            def LN():
                p = slot[0]
                slot[0] += 1
                return ln(nxt + p * sub, sub, st, wr)

            seq = [lambda: K(0), lambda: K(1), lambda: PT(0), lambda: K(2), lambda: PT(1), lambda: K(3),
                   lambda: PT(2), lambda: PT(3)]
            for pos, f in enumerate(seq):
                f()
                for _ in range((lnpos0 if first else lnpos).count(pos)):
                    LN()
            assert slot[0] == LNS
            zacc = zacc + jnp.concatenate(zs, axis=1)
            return zacc, st[0], st[1]

        zacc = jnp.zeros((8, D), f32)
        with sc("p1_it0"):
            zacc, best, bidx = p1_iter(0, zacc, best, bidx, True)

        def body1(i, carry):
            zacc, best, bidx = carry

            @pl.when(i < NI - 1)
            def _():
                x_dma(jnp.minimum(i + 1, NI - 1)).wait()

            @pl.when(i == NI - 1)
            def _():
                wq_dma.wait()
                wv_dma.wait()
                wo_dma.wait()
                if order != 'same':
                    wg_dma(0).wait()
                    wu_dma(0).wait()

            return p1_iter(i, zacc, best, bidx, False)

        with sc("p1_loop"):
            zacc, best, bidx = lax.fori_loop(1, NI, body1, (zacc, best, bidx))

        z = jnp.sum(zacc, axis=0, keepdims=True)
        zc_v[...] = jnp.broadcast_to(z, (L, D)).T
        ri = lax.broadcasted_iota(jnp.int32, (L, L), 0) // DH
        ci = lax.broadcasted_iota(jnp.int32, (L, L), 1) // DH
        mask = ri == ci
        bmax = jnp.max(best, axis=0, keepdims=True)
        idx = jnp.clip(jnp.min(jnp.where(best == bmax, bidx, S)), 0, S - 1)
        g0 = pl.multiple_of((idx // 16) * 16, 16)
        xg = xn_v[pl.ds(g0, 16), :]
        gate = jax.nn.sigmoid(bmax[:, 0:1])
        rr = lax.broadcasted_iota(jnp.int32, (16, 1), 0)
        xsel = jnp.sum(jnp.where(rr == idx - g0, xg.astype(f32), 0.0), axis=0, keepdims=True)
        xb_v[0:D, :] = jnp.broadcast_to(xsel, (L, D)).T
        y_v[...] = jnp.zeros((8, D), f32)
        iblk = idx // R

        def mk(load, nrows, nslab, th, on, kk=None):
            if on:
                return tied_lhs(load, nrows, nslab, th, kk)
            for t in th:
                t()
            return tied_lhs(load, nrows, nslab, [])

        def g_thunks(c, slot, zz=None):
            gu = {}
            wg = wg_v.at[c]
            wu = wu_v.at[c]

            def g_sub(jb, s):
                n = D // GS
                rs = slice(s * n, (s + 1) * n)
                cs = slice(jb * L, (jb + 1) * L)
                if zz is None:
                    xb = xb_v[rs, :]
                else:
                    xb = xb_v[pl.ds(pl.multiple_of((zz | (zz << jb)) + rs.start, 8), n), :]
                g = jnp.sum((wg[rs, cs].astype(f32) * xb).reshape(n // 8, 8, L), axis=0)
                u = jnp.sum((wu[rs, cs].astype(f32) * xb).reshape(n // 8, 8, L), axis=0)
                if s > 0:
                    g = g + gu[jb][0]
                    u = u + gu[jb][1]
                gu[jb] = (g, u)
                return pltpu.bitcast(pltpu.bitcast(g, u32) | pltpu.bitcast(u, u32), f32)

            def g_fin(jb):
                g, u = gu[jb]
                g = jnp.sum(g, axis=0, keepdims=True)
                u = jnp.sum(u, axis=0, keepdims=True)
                h = g * jax.nn.sigmoid(g) * u
                hb = jnp.broadcast_to(h, (L, L)).T
                hb_v[slot, jb * L:(jb + 1) * L, :] = hb
                return hb[0:8]

            th = []
            pend = []
            for jb in range(FB):
                for s in range(GS):
                    th.append(functools.partial(g_sub, jb, s))
                    if pend and s == finlate - 1:
                        th.append(pend.pop(0))
                pend.append(functools.partial(g_fin, jb))
                if finlate == 0:
                    th.append(pend.pop(0))
            th.extend(pend)
            return th

        def d_thunks(c, slot):
            ya = [None]
            NDS = FC // DS
            wd = wd_v.at[c]

            def d_sub(s):
                rs = slice(s * DS, (s + 1) * DS)
                hb = hb_v[slot, rs, :]
                w = wd[rs, :].astype(f32)
                parts = []
                for jb in range(NB):
                    parts.append(jnp.sum((w[:, jb * L:(jb + 1) * L] * hb).reshape(DS // 8, 8, L), axis=0))
                yy = jnp.concatenate(parts, axis=1)
                yy = yy + (ya[0] if s > 0 else y_v[...])
                ya[0] = yy
                if s == NDS - 1:
                    y_v[...] = yy
                hnd = pltpu.bitcast(yy[:, 0:L], u32)
                for jb in range(1, NB):
                    hnd = hnd | pltpu.bitcast(yy[:, jb * L:(jb + 1) * L], u32)
                return pltpu.bitcast(hnd, f32)

            return [functools.partial(d_sub, s) for s in range(NDS)]

        def g2_thunks(c, slot, fins_sep=False, defer=False):
            acc = [None]
            wg = wg_v.at[c]
            wu = wu_v.at[c]
            NG = D // GR

            def sub(s):
                rs = slice(s * GR, (s + 1) * GR)
                xb = xb_v[rs, :]
                parts = []
                for w in (wg, wu):
                    wf = w[rs, :].astype(f32)
                    for jb in range(FB):
                        parts.append(jnp.sum((wf[:, jb * L:(jb + 1) * L] * xb).reshape(GR // 8, 8, L), axis=0))
                a = jnp.concatenate(parts, axis=1)
                if s > 0:
                    a = a + acc[0]
                acc[0] = a
                if defer and s == NG - 1:
                    gu_v[...] = a
                hnd = pltpu.bitcast(a[:, 0:L], u32)
                for jb in range(1, 2 * FB):
                    hnd = hnd | pltpu.bitcast(a[:, jb * L:(jb + 1) * L], u32)
                return pltpu.bitcast(hnd, f32)

            subs = [functools.partial(sub, s) for s in range(NG)]
            if defer:
                return subs
            return subs + fin_thunks(slot, lambda cs: acc[0][:, cs])

        def fin_thunks(slot, get):
            def fin(jb):
                g = jnp.sum(get(slice(jb * L, (jb + 1) * L)), axis=0, keepdims=True)
                u = jnp.sum(get(slice((FB + jb) * L, (FB + jb + 1) * L)), axis=0, keepdims=True)
                h = g * jax.nn.sigmoid(g) * u
                hb = jnp.broadcast_to(h, (L, L)).T
                hb_v[slot, jb * L:(jb + 1) * L, :] = hb
                return hb[0:8]
            return [functools.partial(fin, jb) for jb in range(FB)]

        if wqt == 'mid':
            for c in range(NC):
                wqt_v[c * CW:(c + 1) * CW, :] = wqkv_v[:, c * CW:(c + 1) * CW].T
        gt0 = [] if order == 'same' else (g2_thunks(0, 0, defer=defer) if g2 else g_thunks(0, 0))
        nk = (len(gt0) * midsplit[0]) // sum(midsplit)
        gpk = split(gt0[:nk], NB)
        gpm = split(gt0[nk:], NB)
        kvbs = []

        def kv_dot(j):
            cs = slice(j * L, (j + 1) * L)
            wv = mk(lambda rs, k: wqkv_v[rs, 2 * D + j * L: 2 * D + (j + 1) * L], D, 1, gpk[j], tie2 and tieM)
            kv = _dg(pt_v[:, cs].astype(bf16), wv, 0, 0)
            kvbs.append(jnp.where(mask, kv, 0.0).astype(bf16))

        def m_dot(j):
            cs = slice(j * L, (j + 1) * L)
            wo = mk(lambda rs, k: wo_v[j * L + rs.start: j * L + rs.stop, k * L:(k + 1) * L], L, NB, gpm[j],
                    tie2 and tieM, list(range(NB)))
            m_v[cs, :] = _dot(kvbs[j], wo).astype(bf16)

        for j in range(NB + midskew):
            if j < NB:
                kv_dot(j)
            if j >= midskew:
                m_dot(j - midskew)

        def body2(i, _):
            b = lax.rem(iblk + 1 + i, NI)
            row0 = pl.multiple_of(b * R, R)
            rows = pl.ds(row0, R)
            cn = lax.rem(i + 1, NI)
            ridx = lax.broadcasted_iota(jnp.int32, (R, 1), 0) + row0
            HK = D // 2
            xnb = xn_v.at[rows]
            xblk = x_v.at[rows]
            oblk = out_v.at[rows]
            slot = lax.rem(i, 2)
            if defer:
                slot = 0
                gt = g2_thunks(cn, 0, defer=True)
                ft = fin_thunks(0, lambda cs: gu_v[:, cs])
                dt = d_thunks(i, 0)
                if fint == 'first':
                    dt = ft + dt
                else:
                    seq_, nf = [], 0
                    for s_ in range(len(dt)):
                        need = min(FB, ((s_ + 1) * DS + L - 1) // L + fint)
                        while nf < need:
                            seq_.append(ft[nf]); nf += 1
                        seq_.append(dt[s_])
                    dt = seq_
            else:
                gt = g2_thunks(cn, 1 - slot) if g2 else g_thunks(cn, 1 - slot, (i // NI) * 8 if opq else None)
                dt = d_thunks(i, slot)
            if order == 'same':
                gt = g2_thunks(i, 0) if g2 else g_thunks(i, 0, (i // NI) * 8 if opq else None)
                dt = d_thunks(i, 0)
            if noffn:
                gt, dt = [], []
            if order == 'DH_GAC':
                na = len(gt) // 2
                qparts = split(gt[:na], NC)
                cparts = split(gt[na:], NC)
                hparts = split(dt, NC)
            elif order == 'DH_GQ':
                qparts = split(gt, NC)
                cparts = [[]] * NC
                hparts = split(dt, NC)
            elif order == 'same':
                qparts = split(gt, NC)
                nh = (len(dt) * samesplit[0]) // sum(samesplit)
                hparts = split(dt[:nh], NC)
                cparts = [dt[nh:]] + [[]] * (NC - 1)
            elif order == 'w':
                seq = {'GD': None, 'DG': dt + gt}[qw[0]]
                tot = sum(qw[1:])
                parts, a = [], 0
                for k, w in enumerate(qw[1:]):
                    e = len(seq) if k == len(qw) - 2 else a + (len(seq) * w) // tot
                    parts.append(seq[a:e]); a = e
                qparts, hparts, cparts = parts[0:4], parts[4:8], parts[8:12]
            xn = xnb[...]

            def Q(c):
                cs = slice(c * CW, (c + 1) * CW)
                rhs = mk(lambda rs, k: xn[rs, k * L:(k + 1) * L], R, NB, qparts[c], tie2, (kkQ0 if (c == 0 and kkQ0) else kkQ))
                if wqt:
                    qT = _dg(wqt_v[cs, :], rhs, 1, 1)
                else:
                    qT = _dg(wqkv_v[:, cs], rhs, 0, 1)
                pq = _phi(qT)
                zc = zc_v[cs, :]
                nh = CW // DH
                for t in range(R // L):
                    p = pq[:, t * L:(t + 1) * L]
                    den = jnp.sum((p * zc).reshape(nh, DH, L), axis=1, keepdims=True) + 1e-6
                    o = (p.reshape(nh, DH, L) * rcp(den)).reshape(CW, L).astype(bf16)
                    o_v[t * L:(t + 1) * L, cs] = o.T

            def load_o(half):
                return lambda rs, k: o_v[rs, half * HK + k * L: half * HK + (k + 1) * L]

            def Hh(n):
                cs = slice(n * CW, (n + 1) * CW)
                if wtie:
                    rhs = mk(lambda rs, k: m_v[rs, n * CW + k * L: n * CW + (k + 1) * L], HK, CW // L, hparts[n], tie2, [0, 1])
                    a = _dot(o_v[:, 0:HK], rhs)
                else:
                    lhs = mk(load_o(0), R, NB // 2, hparts[n], tie2, kkH)
                    a = _dot(lhs, m_v[0:HK, cs])
                if resH:
                    a = a + (xblk[:, cs].astype(f32) + xnb[:, cs].astype(f32))
                acc_v[:, cs] = a

            def patch():
                loc = idx - row0
                gl = pl.multiple_of(jnp.clip((loc // 8) * 8, 0, R - 8), 8)
                y = jnp.sum(y_v[...], axis=0, keepdims=True) * gate
                r8 = lax.broadcasted_iota(jnp.int32, (8, 1), 0) + gl
                acc_v[pl.ds(gl, 8), :] += jnp.where(r8 == loc, y, 0.0)

            def C(n):
                cs = slice(n * CW, (n + 1) * CW)
                if wtie:
                    rhs = mk(lambda rs, k: m_v[HK + rs.start: HK + rs.stop, n * CW + k * L: n * CW + (k + 1) * L], HK, CW // L, cparts[n], tie2, [0, 1])
                    a = acc_v[:, cs] + _dot(o_v[:, HK:D], rhs)
                else:
                    a = acc_v[:, cs] + _dot(mk(load_o(1), R, NB // 2, cparts[n], tie2, kkH), m_v[HK:D, cs])
                if not resH:
                    a = a + (xblk[:, cs].astype(f32) + xnb[:, cs].astype(f32))
                if not ypatch:
                    y = jnp.sum(y_v[:, cs], axis=0, keepdims=True) * gate
                    a = a + jnp.where(ridx == idx, y, 0.0)
                oblk[:, cs] = a.astype(bf16)
                o_dma(b, n).start()

            for c in range(NC):
                Q(c)
            for n in range(NC):
                Hh(n)
            if ypatch:
                patch()
            for n in range(NC):
                C(n)
            return None

        with sc("wait_ffn"):
            if order == 'same':
                wg_dma(0).wait()
                wu_dma(0).wait()
            for c in range(1, NI):
                wg_dma(c).wait()
                wu_dma(c).wait()
            for c in range(NI):
                wd_dma(c).wait()
        with sc("p2_loop"):
            lax.fori_loop(0, NI, body2, None)
        with sc("wait_out"):
            for b in range(NI):
                for n in range(NC):
                    o_dma(b, n).wait()

    def fn(A_x, A_wqkv, A_wo, B_x, B_w_r, B_w_gate, B_w_up, B_w_down):
        anyspec = pl.BlockSpec(memory_space=pl.ANY)
        out = pl.pallas_call(
            kernel,
            out_shape=jax.ShapeDtypeStruct((S, D), bf16),
            in_specs=[anyspec] * 7,
            out_specs=anyspec,
            scratch_shapes=[
                pltpu.VMEM((S, D), bf16), pltpu.VMEM((S, D), bf16), pltpu.VMEM((D, 3 * D), bf16),
                pltpu.VMEM((D, D), bf16), pltpu.VMEM((D,), bf16),
                pltpu.VMEM((NI, D, FC), bf16), pltpu.VMEM((NI, D, FC), bf16), pltpu.VMEM((NI, FC, D), bf16),
                pltpu.VMEM((S, D), bf16), pltpu.VMEM((D, D), f32), pltpu.VMEM((D, L), f32),
                pltpu.VMEM((D, D), bf16), pltpu.VMEM((D + 8 * 128, L), f32),
                pltpu.VMEM((R, D), bf16), pltpu.VMEM((R, D), f32),
                pltpu.VMEM((2, FC, L), f32), pltpu.VMEM((8, D), f32), pltpu.VMEM((8, 2 * FC), f32), pltpu.VMEM((D, D), bf16),
                pltpu.SemaphoreType.DMA((NSEM,)),
            ],
            compiler_params=pltpu.CompilerParams(vmem_limit_bytes=100 * 1024 * 1024, flags=flags,
                                                 disable_semaphore_checks=nosemchk),
        )(A_x.reshape(S, D), A_wqkv, A_wo, B_w_r, B_w_gate, B_w_up, B_w_down)
        return out.reshape(1, S, D)
    return fn


_IMPL = make(**dict(order='w',g2=True,GR=16,DS=16,wtie=True,tieM=False,qw=('DG',2,2,2,2,2,2,2,2,2,2,2,2),wqt='mid',flags={'XLA_TPU_EVENLY_DISTRIBUTE_CRITICAL_NODES':True}))


@jax.jit
def pallas_parallel_sum__linear_attn_block__moe_arch_mod__prompt_kernel(
    A_x: jax.Array,
    A_wqkv: jax.Array,
    A_wo: jax.Array,
    B_x: jax.Array,
    B_w_r: jax.Array,
    B_w_gate: jax.Array,
    B_w_up: jax.Array,
    B_w_down: jax.Array,
):
    return _IMPL(A_x, A_wqkv, A_wo, B_x, B_w_r, B_w_gate, B_w_up, B_w_down)
```

```python
import functools, contextlib
import numpy as np
import jax
import jax.numpy as jnp
from jax import lax
import jax.experimental.pallas as pl
import jax.experimental.pallas.tpu as pltpu

S, D, H, DH, F = 2048, 1024, 32, 32, 3584
L = 128
NB = D // L
f32, bf16, u32 = jnp.float32, jnp.bfloat16, jnp.uint32


def _phi(t):
    return jnp.where(t > 0, t + 1.0, jnp.exp(t)) + 1e-6


def _dot(a, b):
    return jnp.dot(a, b, preferred_element_type=f32)


def _dg(a, b, ca, cb):
    return lax.dot_general(a, b, (((ca,), (cb,)), ((), ())), preferred_element_type=f32)


def _zero(v):
    b = pltpu.bitcast(v, u32)
    return lax.shift_right_logical(lax.shift_right_logical(b, jnp.uint32(31)), jnp.uint32(1))


def _tie(xv, z):
    return pltpu.bitcast(pltpu.bitcast(xv, u32) | z, bf16)


def tied_lhs(load, nrows, nslab, thunks, kk=None):
    n = len(thunks)
    if n == 0:
        return jnp.concatenate([load(slice(0, nrows), k) for k in range(nslab)], axis=1)
    if kk is None:
        kk = [k for k in range(0, nslab, 2)]
    per = -(-n // len(kk))
    npos = 1
    while npos < per * len(kk) and npos < nrows // 16:
        npos *= 2
    step = nrows // npos
    slabs = []
    order = {}
    for p in range(n):
        m, q = divmod(p, per)
        r = (q * npos) // per + (m * npos) // (per * len(kk))
        order.setdefault((kk[m], min(r, npos - 1)), []).append(p)
    zs = {}
    for p in range(n):
        v = thunks[p]()
        zs[p] = None if v is None else _zero(v)
    for k in range(nslab):
        if k not in kk:
            slabs.append(load(slice(0, nrows), k))
            continue
        parts = []
        for r in range(npos):
            ps = [zs[p] for p in order.get((k, r), []) if zs[p] is not None]
            if not ps:
                parts.append(load(slice(r * step, (r + 1) * step), k))
            else:
                z = ps[0]
                for z2 in ps[1:]:
                    z = z | z2
                parts.append(_tie(load(slice(r * step, r * step + 16), k), z))
                if step > 16:
                    parts.append(load(slice(r * step + 16, (r + 1) * step), k))
        slabs.append(jnp.concatenate(parts, axis=0))
    return jnp.concatenate(slabs, axis=1)


def split(lst, n):
    k = -(-len(lst) // n) if lst else 0
    return [lst[a * k:(a + 1) * k] for a in range(n)]


def make(R=512, scopes=False, recip="nr", flags=None, tie2=True, tieM=True, LNS=4, GS=8, DS=32,
         kkQ=None, kkH=None, order='DH_GAC', x0parts=4, finlate=4, nosemchk=False,
         lnpos=(2, 3, 4, 5), lnpos0=(3, 4, 5, 6), opq=True, qw=None, noffn=False, ksplit=True, g2=False, GR=16, wtie=False, lnk=(0, 0, 0, 0), lnp=(0, 0, 0, 0), midsplit=(1,) * 16, midskew=8, samesplit=(1, 0), resH=True, ypatch=True, defer=False, fint='first', kkQ0=None, wqt=None, trf32=False, wqtf32=False):
    sc = (lambda n: jax.named_scope(n)) if scopes else (lambda n: contextlib.nullcontext())
    NI = S // R
    CW = 256
    NC = D // CW
    FC = F // NI
    FB = FC // L

    def rcp(x):
        if recip == "approx":
            return pl.reciprocal(x, approx=True)
        if recip == "nr":
            r = pl.reciprocal(x, approx=True)
            return r * (2.0 - x * r)
        return pl.reciprocal(x, approx=False)

    NX0 = x0parts
    SX0, SWR, SWK = 0, NX0, NX0 + 1
    SX = SWK + 4
    SW = SX + NI - 1
    SF = SW + 1
    SO = SF + 2
    NSEM = SO + 1

    def kernel(x_hbm, wqkv_hbm, wo_hbm, wr_hbm, wg_hbm, wu_hbm, wd_hbm, out_hbm,
               x_v, xn_v, wqkv_v, wo_v, wr_v, wg_v, wu_v, wd_v, out_v, pt_v, zc_v, m_v, xb_v, o_v, acc_v, hb_v, y_v, gu_v, wqt_v,
               sems):
        XR = R // NX0

        def x0_dma(h):
            return pltpu.make_async_copy(x_hbm.at[pl.ds(h * XR, XR)], x_v.at[pl.ds(h * XR, XR)], sems.at[SX0 + h])

        wr_dma = pltpu.make_async_copy(wr_hbm, wr_v, sems.at[SWR])
        wk_cols = [(0, L), (L, L), (CW, CW), (2 * CW, 2 * CW)]

        def wk_dma(g):
            cs = pl.ds(D + wk_cols[g][0], wk_cols[g][1])
            return pltpu.make_async_copy(wqkv_hbm.at[:, cs], wqkv_v.at[:, cs], sems.at[SWK + g])

        def x_dma(i):
            return pltpu.make_async_copy(x_hbm.at[pl.ds(i * R, R)], x_v.at[pl.ds(i * R, R)], sems.at[SX + i - 1])

        wq_dma = pltpu.make_async_copy(wqkv_hbm.at[:, pl.ds(0, D)], wqkv_v.at[:, pl.ds(0, D)], sems.at[SW])
        wv_dma = pltpu.make_async_copy(wqkv_hbm.at[:, pl.ds(2 * D, D)], wqkv_v.at[:, pl.ds(2 * D, D)], sems.at[SW])
        wo_dma = pltpu.make_async_copy(wo_hbm, wo_v, sems.at[SW])

        def wg_dma(c):
            return pltpu.make_async_copy(wg_hbm.at[:, pl.ds(c * FC, FC)], wg_v.at[c], sems.at[SF + (c > 0)])

        def wu_dma(c):
            return pltpu.make_async_copy(wu_hbm.at[:, pl.ds(c * FC, FC)], wu_v.at[c], sems.at[SF + (c > 0)])

        def wd_dma(c):
            return pltpu.make_async_copy(wd_hbm.at[pl.ds(c * FC, FC)], wd_v.at[c], sems.at[SF + 1])

        def o_dma(b, n):
            rows = pl.ds(pl.multiple_of(b * R, R), R)
            cs = pl.ds(n * CW, CW)
            return pltpu.make_async_copy(out_v.at[rows, cs], out_hbm.at[rows, cs], sems.at[SO])

        for h in range(NX0):
            x0_dma(h).start()
            if h == 0:
                wr_dma.start()
        for g in range(4):
            wk_dma(g).start()
        for i in range(1, NI):
            x_dma(i).start()
        wq_dma.start()
        wv_dma.start()
        wo_dma.start()
        for c in range(NI):
            wg_dma(c).start()
            wu_dma(c).start()
        for c in range(NI):
            wd_dma(c).start()

        def ln(row0, n, st, wr):
            best, bidx = st
            rows = pl.ds(row0, n)
            x = x_v[rows, :].astype(f32)
            m = jnp.mean(x, axis=-1, keepdims=True)
            d = x - m
            v = jnp.mean(d * d, axis=-1, keepdims=True)
            xn = d * lax.rsqrt(v + 1e-5)
            xn_v[rows, :] = xn.astype(bf16)
            r = jnp.broadcast_to(jnp.sum(xn * wr, axis=-1, keepdims=True), (n, L))
            sub_iota = lax.broadcasted_iota(jnp.int32, (8, L), 0) + row0
            for g in range(n // 8):
                rg = r[8 * g:8 * g + 8]
                better = rg > best
                best = jnp.where(better, rg, best)
                bidx = jnp.where(better, sub_iota + 8 * g, bidx)
            st[0], st[1] = best, bidx
            hnd = pltpu.bitcast(best, u32)
            for g in range(n // 8):
                hnd = hnd | pltpu.bitcast(xn[8 * g:8 * g + 8, D - L:D], u32)
            return pltpu.bitcast(hnd, f32)

        st = [jnp.full((8, L), -jnp.inf, f32), jnp.full((8, L), S, jnp.int32)]
        for h in range(NX0):
            with sc("wait_x0"):
                x0_dma(h).wait()
                if h == 0:
                    wr_dma.wait()
            if h == 0:
                wr0 = wr_v[...].astype(f32).reshape(1, D)
            ln(h * XR, XR, st, wr0)
        best, bidx = st

        def p1_iter(i, zacc, best, bidx, first):
            row0 = 0 if first else pl.multiple_of(i * R, R)
            rows = pl.ds(row0, R)
            nxt = R if first else pl.multiple_of(lax.rem(i + 1, NI) * R, R)
            st = [best, bidx]
            wr = wr_v[...].astype(f32).reshape(1, D)
            if first:
                wk_dma(0).wait()
            xn = xn_v[rows, :]
            pks, zs = [], []
            sub = R // LNS
            slot = [0]

            def lnth(n):
                out = []
                for _ in range(n):
                    out.append(LN)
                return out

            def K(c):
                if first and c == 0:
                    k0 = _dot(xn, wqkv_v[:, D: D + L])
                    wk_dma(1).wait()
                    k1 = _dot(xn, wqkv_v[:, D + L: D + 2 * L])
                    pk = _phi(jnp.concatenate([k0, k1], axis=1))
                    zs.append(jnp.sum(pk.reshape(R // 8, 8, CW), axis=0))
                    pks.append(pk.astype(bf16))
                    return
                if first and c in (1, 2):
                    wk_dma(c + 1).wait()
                    if c == 2:
                        x_dma(1).wait()
                nl = lnk[c]
                if nl:
                    w = tied_lhs(lambda rs, k: wqkv_v[rs, D + c * CW + k * L: D + c * CW + (k + 1) * L], D, CW // L,
                                 lnth(nl), [0, 1])
                else:
                    w = wqkv_v[:, D + c * CW: D + (c + 1) * CW]
                k = _dot(xn, w)
                pk = _phi(k)
                zs.append(jnp.sum(pk.reshape(R // 8, 8, CW), axis=0))
                pks.append(pk.astype(bf16))

            def PT(c):
                cs = slice(c * CW, (c + 1) * CW)
                nl = lnp[c]
                if nl:
                    rhs = tied_lhs(lambda rs, k: pks[c][rs, k * L:(k + 1) * L], R, CW // L, lnth(nl), [0, 1])
                else:
                    rhs = pks[c]
                r = _dg(xn, rhs, 0, 0)
                if first:
                    pt_v[:, cs] = r
                else:
                    pt_v[:, cs] += r

            def LN():
                p = slot[0]
                slot[0] += 1
                return ln(nxt + p * sub, sub, st, wr)

            seq = [lambda: K(0), lambda: K(1), lambda: PT(0), lambda: K(2), lambda: PT(1), lambda: K(3),
                   lambda: PT(2), lambda: PT(3)]
            for pos, f in enumerate(seq):
                f()
                for _ in range((lnpos0 if first else lnpos).count(pos)):
                    LN()
            assert slot[0] == LNS
            zacc = zacc + jnp.concatenate(zs, axis=1)
            return zacc, st[0], st[1]

        zacc = jnp.zeros((8, D), f32)
        with sc("p1_it0"):
            zacc, best, bidx = p1_iter(0, zacc, best, bidx, True)

        def body1(i, carry):
            zacc, best, bidx = carry

            @pl.when(i < NI - 1)
            def _():
                x_dma(jnp.minimum(i + 1, NI - 1)).wait()

            @pl.when(i == NI - 1)
            def _():
                wq_dma.wait()
                wv_dma.wait()
                wo_dma.wait()
                if order != 'same':
                    wg_dma(0).wait()
                    wu_dma(0).wait()

            return p1_iter(i, zacc, best, bidx, False)

        with sc("p1_loop"):
            zacc, best, bidx = lax.fori_loop(1, NI, body1, (zacc, best, bidx))

        z = jnp.sum(zacc, axis=0, keepdims=True)
        zc_v[...] = jnp.broadcast_to(z, (L, D)).T
        ri = lax.broadcasted_iota(jnp.int32, (L, L), 0) // DH
        ci = lax.broadcasted_iota(jnp.int32, (L, L), 1) // DH
        mask = ri == ci
        bmax = jnp.max(best, axis=0, keepdims=True)
        idx = jnp.clip(jnp.min(jnp.where(best == bmax, bidx, S)), 0, S - 1)
        g0 = pl.multiple_of((idx // 16) * 16, 16)
        xg = xn_v[pl.ds(g0, 16), :]
        gate = jax.nn.sigmoid(bmax[:, 0:1])
        rr = lax.broadcasted_iota(jnp.int32, (16, 1), 0)
        xsel = jnp.sum(jnp.where(rr == idx - g0, xg.astype(f32), 0.0), axis=0, keepdims=True)
        xb_v[0:D, :] = jnp.broadcast_to(xsel, (L, D)).T
        y_v[...] = jnp.zeros((8, D), f32)
        iblk = idx // R

        def mk(load, nrows, nslab, th, on, kk=None):
            if on:
                return tied_lhs(load, nrows, nslab, th, kk)
            for t in th:
                t()
            return tied_lhs(load, nrows, nslab, [])

        def g_thunks(c, slot, zz=None):
            gu = {}
            wg = wg_v.at[c]
            wu = wu_v.at[c]

            def g_sub(jb, s):
                n = D // GS
                rs = slice(s * n, (s + 1) * n)
                cs = slice(jb * L, (jb + 1) * L)
                if zz is None:
                    xb = xb_v[rs, :]
                else:
                    xb = xb_v[pl.ds(pl.multiple_of((zz | (zz << jb)) + rs.start, 8), n), :]
                g = jnp.sum((wg[rs, cs].astype(f32) * xb).reshape(n // 8, 8, L), axis=0)
                u = jnp.sum((wu[rs, cs].astype(f32) * xb).reshape(n // 8, 8, L), axis=0)
                if s > 0:
                    g = g + gu[jb][0]
                    u = u + gu[jb][1]
                gu[jb] = (g, u)
                return pltpu.bitcast(pltpu.bitcast(g, u32) | pltpu.bitcast(u, u32), f32)

            def g_fin(jb):
                g, u = gu[jb]
                g = jnp.sum(g, axis=0, keepdims=True)
                u = jnp.sum(u, axis=0, keepdims=True)
                h = g * jax.nn.sigmoid(g) * u
                hb = jnp.broadcast_to(h, (L, L)).T
                hb_v[slot, jb * L:(jb + 1) * L, :] = hb
                return hb[0:8]

            th = []
            pend = []
            for jb in range(FB):
                for s in range(GS):
                    th.append(functools.partial(g_sub, jb, s))
                    if pend and s == finlate - 1:
                        th.append(pend.pop(0))
                pend.append(functools.partial(g_fin, jb))
                if finlate == 0:
                    th.append(pend.pop(0))
            th.extend(pend)
            return th

        def d_thunks(c, slot):
            ya = [None]
            NDS = FC // DS
            wd = wd_v.at[c]

            def d_sub(s):
                rs = slice(s * DS, (s + 1) * DS)
                hb = hb_v[slot, rs, :]
                w = wd[rs, :].astype(f32)
                parts = []
                for jb in range(NB):
                    parts.append(jnp.sum((w[:, jb * L:(jb + 1) * L] * hb).reshape(DS // 8, 8, L), axis=0))
                yy = jnp.concatenate(parts, axis=1)
                yy = yy + (ya[0] if s > 0 else y_v[...])
                ya[0] = yy
                if s == NDS - 1:
                    y_v[...] = yy
                hnd = pltpu.bitcast(yy[:, 0:L], u32)
                for jb in range(1, NB):
                    hnd = hnd | pltpu.bitcast(yy[:, jb * L:(jb + 1) * L], u32)
                return pltpu.bitcast(hnd, f32)

            return [functools.partial(d_sub, s) for s in range(NDS)]

        def g2_thunks(c, slot, fins_sep=False, defer=False):
            acc = [None]
            wg = wg_v.at[c]
            wu = wu_v.at[c]
            NG = D // GR

            def sub(s):
                rs = slice(s * GR, (s + 1) * GR)
                xb = xb_v[rs, :]
                parts = []
                for w in (wg, wu):
                    wf = w[rs, :].astype(f32)
                    for jb in range(FB):
                        parts.append(jnp.sum((wf[:, jb * L:(jb + 1) * L] * xb).reshape(GR // 8, 8, L), axis=0))
                a = jnp.concatenate(parts, axis=1)
                if s > 0:
                    a = a + acc[0]
                acc[0] = a
                if defer and s == NG - 1:
                    gu_v[...] = a
                hnd = pltpu.bitcast(a[:, 0:L], u32)
                for jb in range(1, 2 * FB):
                    hnd = hnd | pltpu.bitcast(a[:, jb * L:(jb + 1) * L], u32)
                return pltpu.bitcast(hnd, f32)

            subs = [functools.partial(sub, s) for s in range(NG)]
            if defer:
                return subs
            return subs + fin_thunks(slot, lambda cs: acc[0][:, cs])

        def fin_thunks(slot, get):
            def fin(jb):
                g = jnp.sum(get(slice(jb * L, (jb + 1) * L)), axis=0, keepdims=True)
                u = jnp.sum(get(slice((FB + jb) * L, (FB + jb + 1) * L)), axis=0, keepdims=True)
                h = g * jax.nn.sigmoid(g) * u
                hb = jnp.broadcast_to(h, (L, L)).T
                hb_v[slot, jb * L:(jb + 1) * L, :] = hb
                return hb[0:8]
            return [functools.partial(fin, jb) for jb in range(FB)]

        if wqt == 'mid':
            for c in range(NC):
                wqt_v[c * CW:(c + 1) * CW, :] = (wqkv_v[:, c * CW:(c + 1) * CW].astype(f32).T.astype(bf16) if wqtf32
                                                  else wqkv_v[:, c * CW:(c + 1) * CW].T)
        gt0 = [] if order == 'same' else (g2_thunks(0, 0, defer=defer) if g2 else g_thunks(0, 0))
        tot = sum(midsplit)
        gparts0, a0 = [], 0
        for k_, w_ in enumerate(midsplit):
            e0 = a0 + (len(gt0) * w_) // tot if tot else a0
            gparts0.append(gt0[a0:e0]); a0 = e0
        lastnz = max([k_ for k_, w_ in enumerate(midsplit) if w_] or [0])
        gparts0[lastnz] = gparts0[lastnz] + gt0[a0:]
        gpk, gpm = gparts0[:NB], gparts0[NB:]
        kvbs = []

        def kv_dot(j):
            cs = slice(j * L, (j + 1) * L)
            wv = mk(lambda rs, k: wqkv_v[rs, 2 * D + j * L: 2 * D + (j + 1) * L], D, 1, gpk[j], tie2 and tieM)
            kv = _dg(pt_v[:, cs].astype(bf16), wv, 0, 0)
            kvbs.append(jnp.where(mask, kv, 0.0).astype(bf16))

        def m_dot(j):
            cs = slice(j * L, (j + 1) * L)
            wo = mk(lambda rs, k: wo_v[j * L + rs.start: j * L + rs.stop, k * L:(k + 1) * L], L, NB, gpm[j],
                    tie2 and tieM, list(range(NB)))
            m_v[cs, :] = _dot(kvbs[j], wo).astype(bf16)

        for j in range(NB + midskew):
            if j < NB:
                kv_dot(j)
            if j >= midskew:
                m_dot(j - midskew)

        def body2(i, _):
            b = lax.rem(iblk + 1 + i, NI)
            row0 = pl.multiple_of(b * R, R)
            rows = pl.ds(row0, R)
            cn = lax.rem(i + 1, NI)
            ridx = lax.broadcasted_iota(jnp.int32, (R, 1), 0) + row0
            HK = D // 2
            xnb = xn_v.at[rows]
            xblk = x_v.at[rows]
            oblk = out_v.at[rows]
            slot = lax.rem(i, 2)
            if defer:
                slot = 0
                gt = g2_thunks(cn, 0, defer=True)
                ft = fin_thunks(0, lambda cs: gu_v[:, cs])
                dt = d_thunks(i, 0)
                if fint == 'first':
                    dt = ft + dt
                else:
                    seq_, nf = [], 0
                    for s_ in range(len(dt)):
                        need = min(FB, ((s_ + 1) * DS + L - 1) // L + fint)
                        while nf < need:
                            seq_.append(ft[nf]); nf += 1
                        seq_.append(dt[s_])
                    dt = seq_
            else:
                gt = g2_thunks(cn, 1 - slot) if g2 else g_thunks(cn, 1 - slot, (i // NI) * 8 if opq else None)
                dt = d_thunks(i, slot)
            if order == 'same':
                gt = g2_thunks(i, 0) if g2 else g_thunks(i, 0, (i // NI) * 8 if opq else None)
                dt = d_thunks(i, 0)
            if noffn:
                gt, dt = [], []
            if order == 'DH_GAC':
                na = len(gt) // 2
                qparts = split(gt[:na], NC)
                cparts = split(gt[na:], NC)
                hparts = split(dt, NC)
            elif order == 'DH_GQ':
                qparts = split(gt, NC)
                cparts = [[]] * NC
                hparts = split(dt, NC)
            elif order == 'same':
                qparts = split(gt, NC)
                nh = (len(dt) * samesplit[0]) // sum(samesplit)
                hparts = split(dt[:nh], NC)
                cparts = [dt[nh:]] + [[]] * (NC - 1)
            elif order == 'w':
                seq = {'GD': None, 'DG': dt + gt}[qw[0]]
                tot = sum(qw[1:])
                parts, a = [], 0
                for k, w in enumerate(qw[1:]):
                    e = len(seq) if k == len(qw) - 2 else a + (len(seq) * w) // tot
                    parts.append(seq[a:e]); a = e
                qparts, hparts, cparts = parts[0:4], parts[4:8], parts[8:12]
            xn = xnb[...]

            def Q(c):
                cs = slice(c * CW, (c + 1) * CW)
                rhs = mk(lambda rs, k: xn[rs, k * L:(k + 1) * L], R, NB, qparts[c], tie2, (kkQ0 if (c == 0 and kkQ0) else kkQ))
                if wqt:
                    qT = _dg(wqt_v[cs, :], rhs, 1, 1)
                else:
                    qT = _dg(wqkv_v[:, cs], rhs, 0, 1)
                pq = _phi(qT)
                zc = zc_v[cs, :]
                nh = CW // DH
                for t in range(R // L):
                    p = pq[:, t * L:(t + 1) * L]
                    den = jnp.sum((p * zc).reshape(nh, DH, L), axis=1, keepdims=True) + 1e-6
                    o = (p.reshape(nh, DH, L) * rcp(den)).reshape(CW, L)
                    if trf32:
                        o_v[t * L:(t + 1) * L, cs] = o.T.astype(bf16)
                    else:
                        o_v[t * L:(t + 1) * L, cs] = o.astype(bf16).T

            def load_o(half):
                return lambda rs, k: o_v[rs, half * HK + k * L: half * HK + (k + 1) * L]

            def Hh(n):
                cs = slice(n * CW, (n + 1) * CW)
                if wtie:
                    rhs = mk(lambda rs, k: m_v[rs, n * CW + k * L: n * CW + (k + 1) * L], HK, CW // L, hparts[n], tie2, [0, 1])
                    a = _dot(o_v[:, 0:HK], rhs)
                else:
                    lhs = mk(load_o(0), R, NB // 2, hparts[n], tie2, kkH)
                    a = _dot(lhs, m_v[0:HK, cs])
                if resH:
                    a = a + (xblk[:, cs].astype(f32) + xnb[:, cs].astype(f32))
                acc_v[:, cs] = a

            def patch():
                loc = idx - row0
                gl = pl.multiple_of(jnp.clip((loc // 8) * 8, 0, R - 8), 8)
                y = jnp.sum(y_v[...], axis=0, keepdims=True) * gate
                r8 = lax.broadcasted_iota(jnp.int32, (8, 1), 0) + gl
                acc_v[pl.ds(gl, 8), :] += jnp.where(r8 == loc, y, 0.0)

            def C(n):
                cs = slice(n * CW, (n + 1) * CW)
                if wtie:
                    rhs = mk(lambda rs, k: m_v[HK + rs.start: HK + rs.stop, n * CW + k * L: n * CW + (k + 1) * L], HK, CW // L, cparts[n], tie2, [0, 1])
                    a = acc_v[:, cs] + _dot(o_v[:, HK:D], rhs)
                else:
                    a = acc_v[:, cs] + _dot(mk(load_o(1), R, NB // 2, cparts[n], tie2, kkH), m_v[HK:D, cs])
                if not resH:
                    a = a + (xblk[:, cs].astype(f32) + xnb[:, cs].astype(f32))
                if not ypatch:
                    y = jnp.sum(y_v[:, cs], axis=0, keepdims=True) * gate
                    a = a + jnp.where(ridx == idx, y, 0.0)
                oblk[:, cs] = a.astype(bf16)
                o_dma(b, n).start()

            for c in range(NC):
                Q(c)
            for n in range(NC):
                Hh(n)
            if ypatch:
                patch()
            for n in range(NC):
                C(n)
            return None

        with sc("wait_ffn"):
            if order == 'same':
                wg_dma(0).wait()
                wu_dma(0).wait()
            for c in range(1, NI):
                wg_dma(c).wait()
                wu_dma(c).wait()
            for c in range(NI):
                wd_dma(c).wait()
        with sc("p2_loop"):
            lax.fori_loop(0, NI, body2, None)
        with sc("wait_out"):
            for b in range(NI):
                for n in range(NC):
                    o_dma(b, n).wait()

    def fn(A_x, A_wqkv, A_wo, B_x, B_w_r, B_w_gate, B_w_up, B_w_down):
        anyspec = pl.BlockSpec(memory_space=pl.ANY)
        out = pl.pallas_call(
            kernel,
            out_shape=jax.ShapeDtypeStruct((S, D), bf16),
            in_specs=[anyspec] * 7,
            out_specs=anyspec,
            scratch_shapes=[
                pltpu.VMEM((S, D), bf16), pltpu.VMEM((S, D), bf16), pltpu.VMEM((D, 3 * D), bf16),
                pltpu.VMEM((D, D), bf16), pltpu.VMEM((D,), bf16),
                pltpu.VMEM((NI, D, FC), bf16), pltpu.VMEM((NI, D, FC), bf16), pltpu.VMEM((NI, FC, D), bf16),
                pltpu.VMEM((S, D), bf16), pltpu.VMEM((D, D), f32), pltpu.VMEM((D, L), f32),
                pltpu.VMEM((D, D), bf16), pltpu.VMEM((D + 8 * 128, L), f32),
                pltpu.VMEM((R, D), bf16), pltpu.VMEM((R, D), f32),
                pltpu.VMEM((2, FC, L), f32), pltpu.VMEM((8, D), f32), pltpu.VMEM((8, 2 * FC), f32), pltpu.VMEM((D, D), bf16),
                pltpu.SemaphoreType.DMA((NSEM,)),
            ],
            compiler_params=pltpu.CompilerParams(vmem_limit_bytes=100 * 1024 * 1024, flags=flags,
                                                 disable_semaphore_checks=nosemchk),
        )(A_x.reshape(S, D), A_wqkv, A_wo, B_w_r, B_w_gate, B_w_up, B_w_down)
        return out.reshape(1, S, D)
    return fn


_IMPL = make(**dict(order='w',g2=True,GR=16,DS=16,wtie=True,wqt='mid',qw=('DG',2,2,2,2,2,2,2,2,2,2,2,2),kkQ=[4,6],tieM=True,midsplit=(0,0,1,1,1,1,1,1,1,1,1,1,1,1,1,1),midskew=4,flags={'XLA_TPU_EVENLY_DISTRIBUTE_CRITICAL_NODES':True}))


@jax.jit
def pallas_parallel_sum__linear_attn_block__moe_arch_mod__prompt_kernel(
    A_x: jax.Array,
    A_wqkv: jax.Array,
    A_wo: jax.Array,
    B_x: jax.Array,
    B_w_r: jax.Array,
    B_w_gate: jax.Array,
    B_w_up: jax.Array,
    B_w_down: jax.Array,
):
    return _IMPL(A_x, A_wqkv, A_wo, B_x, B_w_r, B_w_gate, B_w_up, B_w_down)
```

```python
import contextlib
import functools

import jax
import jax.numpy as jnp
from jax import lax
import jax.experimental.pallas as pl
import jax.experimental.pallas.tpu as pltpu

S, D, DH, F = 2048, 1024, 32, 3584
L = 128
NB = D // L
f32, bf16, u32 = jnp.float32, jnp.bfloat16, jnp.uint32


def _phi(t):
    return jnp.where(t > 0, t + 1.0, jnp.exp(t)) + 1e-6


def _dot(a, b):
    return jnp.dot(a, b, preferred_element_type=f32)


def _dg(a, b, ca, cb):
    return lax.dot_general(a, b, (((ca,), (cb,)), ((), ())), preferred_element_type=f32)


def _rcp(x):
    r = pl.reciprocal(x, approx=True)
    return r * (2.0 - x * r)


def _zero(v):
    b = pltpu.bitcast(v, u32)
    return lax.shift_right_logical(lax.shift_right_logical(b, jnp.uint32(31)), jnp.uint32(1))


def _any(x):
    h = pltpu.bitcast(x[:, 0:L], u32)
    for j in range(1, x.shape[1] // L):
        h = h | pltpu.bitcast(x[:, j * L:(j + 1) * L], u32)
    return pltpu.bitcast(h, f32)


def _paced(load, nrows, nslab, thunks, kk=None):
    n = len(thunks)
    if n == 0:
        return jnp.concatenate([load(slice(0, nrows), k) for k in range(nslab)], axis=1)
    kk = list(range(0, nslab, 2)) if kk is None else kk
    per = -(-n // len(kk))
    npos = 1
    while npos < per * len(kk) and npos < nrows // 16:
        npos *= 2
    step = nrows // npos
    where = {}
    for p in range(n):
        m, q = divmod(p, per)
        r = (q * npos) // per + (m * npos) // (per * len(kk))
        where.setdefault((kk[m], min(r, npos - 1)), []).append(p)
    zs = [_zero(t()) for t in thunks]
    slabs = []
    for k in range(nslab):
        if k not in kk:
            slabs.append(load(slice(0, nrows), k))
            continue
        parts = []
        for r in range(npos):
            ps = where.get((k, r))
            if not ps:
                parts.append(load(slice(r * step, (r + 1) * step), k))
                continue
            z = zs[ps[0]]
            for p in ps[1:]:
                z = z | zs[p]
            tile = load(slice(r * step, r * step + 16), k)
            parts.append(pltpu.bitcast(pltpu.bitcast(tile, u32) | z, bf16))
            if step > 16:
                parts.append(load(slice(r * step + 16, (r + 1) * step), k))
        slabs.append(jnp.concatenate(parts, axis=0))
    return jnp.concatenate(slabs, axis=1)


def _share(seq, weights):
    tot, out, a = sum(weights), [], 0
    last = max(i for i, w in enumerate(weights) if w)
    for i, w in enumerate(weights):
        e = len(seq) if i == last else a + (len(seq) * w) // tot
        out.append(seq[a:e])
        a = e
    return out


def make(R1=512, R2=512, x0rows=(0, 128, 256, 384, 512), LNS=4, lnpos=(2, 3, 4, 5), lnpos0=(3, 4, 5, 6),
         rpos=0, rpos0=3, GR=16, DS=16, qw=(2,) * 12, kkQ=(4, 6), ccols=(0, 256, 512, 768, 1024),
         midsplit=(0, 0) + (1,) * 14, midskew=4, scopes=False,
         flags=(("XLA_TPU_EVENLY_DISTRIBUTE_CRITICAL_NODES", True),)):
    sc = (lambda n: jax.named_scope(n)) if scopes else (lambda n: contextlib.nullcontext())
    N1, N2 = S // R1, S // R2
    CW = 256
    NC = D // CW
    FC = F // N2
    FB = FC // L
    HK = D // 2
    NX0 = len(x0rows) - 1
    wk_cols = [(0, L), (L, L), (CW, CW), (2 * CW, 2 * CW)]
    SX0, SWR, SWK = 0, NX0, NX0 + 1
    SX = SWK + len(wk_cols)
    SW = SX + N1 - 1
    SF = SW + 1
    SO = SF + 2
    NSEM = SO + 1

    def kernel(x_hbm, wqkv_hbm, wo_hbm, wr_hbm, wg_hbm, wu_hbm, wd_hbm, out_hbm,
               x_v, xn_v, wqkv_v, wo_v, wr_v, wg_v, wu_v, wd_v, out_v, pt_v, zc_v, m_v, xb_v, o_v, acc_v,
               hb_v, y_v, wqt_v, sems):
        def x0_dma(h):
            rs = pl.ds(x0rows[h], x0rows[h + 1] - x0rows[h])
            return pltpu.make_async_copy(x_hbm.at[rs], x_v.at[rs], sems.at[SX0 + h])

        def x_dma(i):
            rs = pl.ds(i * R1, R1)
            return pltpu.make_async_copy(x_hbm.at[rs], x_v.at[rs], sems.at[SX + i - 1])

        def wcols_dma(c0, n, sem):
            cs = pl.ds(c0, n)
            return pltpu.make_async_copy(wqkv_hbm.at[:, cs], wqkv_v.at[:, cs], sems.at[sem])

        def wk_dma(g):
            return wcols_dma(D + wk_cols[g][0], wk_cols[g][1], SWK + g)

        def wg_dma(c):
            return pltpu.make_async_copy(wg_hbm.at[:, pl.ds(c * FC, FC)], wg_v.at[c], sems.at[SF + (c > 0)])

        def wu_dma(c):
            return pltpu.make_async_copy(wu_hbm.at[:, pl.ds(c * FC, FC)], wu_v.at[c], sems.at[SF + (c > 0)])

        def wd_dma(c):
            return pltpu.make_async_copy(wd_hbm.at[pl.ds(c * FC, FC)], wd_v.at[c], sems.at[SF + 1])

        def o_dma(b, n):
            rows = pl.ds(pl.multiple_of(b * R2, R2), R2)
            cs = pl.ds(ccols[n], ccols[n + 1] - ccols[n])
            return pltpu.make_async_copy(out_v.at[rows, cs], out_hbm.at[rows, cs], sems.at[SO])

        wr_dma = pltpu.make_async_copy(wr_hbm, wr_v, sems.at[SWR])
        wq_dma = wcols_dma(0, D, SW)
        wv_dma = wcols_dma(2 * D, D, SW)
        wo_dma = pltpu.make_async_copy(wo_hbm, wo_v, sems.at[SW])

        for h in range(NX0):
            x0_dma(h).start()
        for g in range(len(wk_cols)):
            wk_dma(g).start()
            if g == 0:
                wr_dma.start()
        for i in range(1, N1):
            x_dma(i).start()
        wq_dma.start()
        wv_dma.start()
        wo_dma.start()
        for c in range(N2):
            wg_dma(c).start()
            wu_dma(c).start()
        for c in range(N2):
            wd_dma(c).start()

        def ln(row0, n):
            rows = pl.ds(row0, n)
            x = x_v[rows, :].astype(f32)
            m = jnp.mean(x, axis=-1, keepdims=True)
            d = x - m
            v = jnp.mean(d * d, axis=-1, keepdims=True)
            xn_v[rows, :] = (d * lax.rsqrt(v + 1e-5)).astype(bf16)

        def router(xn, row0, best, bidx):
            n = xn.shape[0]
            wr = wr_v[...].astype(f32).reshape(1, D)
            r = jnp.broadcast_to(jnp.sum(xn.astype(f32) * wr, axis=-1, keepdims=True), (n, L))
            rid = lax.broadcasted_iota(jnp.int32, (8, L), 0) + row0
            for g in range(n // 8):
                rg = r[8 * g:8 * g + 8]
                better = rg > best
                best = jnp.where(better, rg, best)
                bidx = jnp.where(better, rid + 8 * g, bidx)
            return best, bidx

        def p1_block(i, zacc, best, bidx, first):
            row0 = 0 if first else pl.multiple_of(i * R1, R1)
            nxt = R1 if first else pl.multiple_of(lax.rem(i + 1, N1) * R1, R1)
            if first:
                with sc("w_c0"):
                    wk_dma(0).wait()
                    wr_dma.wait()
            xn = xn_v[pl.ds(row0, R1), :]
            pks, zs, raw = [], [], []

            def fin_k(k):
                pk = _phi(k)
                zs.append(jnp.sum(pk.reshape(R1 // 8, 8, CW), axis=0))
                pks.append(pk.astype(bf16))

            def K(c):
                if first and c == 0:
                    k0 = _dot(xn, wqkv_v[:, D:D + L])
                    wk_dma(1).wait()
                    k1 = _dot(xn, wqkv_v[:, D + L:D + 2 * L])
                    raw.append(jnp.concatenate([k0, k1], axis=1))
                    return
                if first and c in (1, 2):
                    wk_dma(c + 1).wait()
                    if c == 2:
                        x_dma(1).wait()
                if raw:
                    fin_k(raw.pop())
                fin_k(_dot(xn, wqkv_v[:, D + c * CW:D + (c + 1) * CW]))

            def PT(c):
                cs = slice(c * CW, (c + 1) * CW)
                r = _dg(xn, pks[c], 0, 0)
                if first:
                    pt_v[:, cs] = r
                else:
                    pt_v[:, cs] += r

            seq = [(K, 0), (K, 1), (PT, 0), (K, 2), (PT, 1), (K, 3), (PT, 2), (PT, 3)]
            sub, done = R1 // LNS, 0
            for pos, (f, c) in enumerate(seq):
                if pos == (rpos0 if first else rpos):
                    best, bidx = router(xn, row0, best, bidx)
                f(c)
                for _ in range((lnpos0 if first else lnpos).count(pos)):
                    ln(nxt + done * sub, sub)
                    done += 1
            assert done == LNS
            return zacc + jnp.concatenate(zs, axis=1), best, bidx

        for h in range(NX0):
            with sc("wait_x0"):
                x0_dma(h).wait()
            ln(x0rows[h], x0rows[h + 1] - x0rows[h])

        best = jnp.full((8, L), -jnp.inf, f32)
        bidx = jnp.full((8, L), S, jnp.int32)
        with sc("p1_it0"):
            zacc, best, bidx = p1_block(0, jnp.zeros((8, D), f32), best, bidx, True)

        def body1(i, carry):
            @pl.when(i < N1 - 1)
            def _():
                x_dma(jnp.minimum(i + 1, N1 - 1)).wait()

            @pl.when(i == N1 - 1)
            def _():
                wq_dma.wait()
                wv_dma.wait()
                wo_dma.wait()
                wg_dma(0).wait()
                wu_dma(0).wait()

            return p1_block(i, *carry, False)

        with sc("p1_loop"):
            zacc, best, bidx = lax.fori_loop(1, N1, body1, (zacc, best, bidx))

        z = jnp.sum(zacc, axis=0, keepdims=True)
        zc_v[...] = jnp.broadcast_to(z, (L, D)).T
        bmax = jnp.max(best, axis=0, keepdims=True)
        idx = jnp.clip(jnp.min(jnp.where(best == bmax, bidx, S)), 0, S - 1)
        gate = jax.nn.sigmoid(bmax[:, 0:1])
        g0 = pl.multiple_of((idx // 16) * 16, 16)
        rr = lax.broadcasted_iota(jnp.int32, (16, 1), 0)
        xsel = jnp.sum(jnp.where(rr == idx - g0, xn_v[pl.ds(g0, 16), :].astype(f32), 0.0), axis=0, keepdims=True)
        xb_v[...] = jnp.broadcast_to(xsel, (L, D)).T
        y_v[...] = jnp.zeros((8, D), f32)
        iblk = idx // R2
        for c in range(NC):
            wqt_v[c * CW:(c + 1) * CW, :] = wqkv_v[:, c * CW:(c + 1) * CW].T

        def gate_up_thunks(c, slot):
            acc = [None]
            wg, wu = wg_v.at[c], wu_v.at[c]

            def sub(s):
                rs = slice(s * GR, (s + 1) * GR)
                xb = xb_v[rs, :]
                parts = []
                for w in (wg, wu):
                    wf = w[rs, :].astype(f32)
                    for jb in range(FB):
                        parts.append(jnp.sum((wf[:, jb * L:(jb + 1) * L] * xb).reshape(GR // 8, 8, L), axis=0))
                a = jnp.concatenate(parts, axis=1)
                acc[0] = a if s == 0 else a + acc[0]
                return _any(acc[0])

            def fin(jb):
                g = jnp.sum(acc[0][:, jb * L:(jb + 1) * L], axis=0, keepdims=True)
                u = jnp.sum(acc[0][:, (FB + jb) * L:(FB + jb + 1) * L], axis=0, keepdims=True)
                hb = jnp.broadcast_to(g * jax.nn.sigmoid(g) * u, (L, L)).T
                hb_v[slot, jb * L:(jb + 1) * L, :] = hb
                return hb[0:8]

            return ([functools.partial(sub, s) for s in range(D // GR)]
                    + [functools.partial(fin, jb) for jb in range(FB)])

        def down_thunks(c, slot):
            acc = [None]
            wd = wd_v.at[c]
            n = FC // DS

            def sub(s):
                rs = slice(s * DS, (s + 1) * DS)
                hb = hb_v[slot, rs, :]
                w = wd[rs, :].astype(f32)
                yy = jnp.concatenate(
                    [jnp.sum((w[:, jb * L:(jb + 1) * L] * hb).reshape(DS // 8, 8, L), axis=0) for jb in range(NB)],
                    axis=1)
                acc[0] = yy + (acc[0] if s > 0 else y_v[...])
                if s == n - 1:
                    y_v[...] = acc[0]
                return _any(acc[0])

            return [functools.partial(sub, s) for s in range(n)]

        ri = lax.broadcasted_iota(jnp.int32, (L, L), 0) // DH
        ci = lax.broadcasted_iota(jnp.int32, (L, L), 1) // DH
        parts0 = _share(gate_up_thunks(0, 0), midsplit)
        kvs = []
        for j in range(NB + midskew):
            if j < NB:
                wv = _paced(lambda rs, k: wqkv_v[rs, 2 * D + j * L:2 * D + (j + 1) * L], D, 1, parts0[j])
                kv = _dg(pt_v[:, j * L:(j + 1) * L].astype(bf16), wv, 0, 0)
                kvs.append(jnp.where(ri == ci, kv, 0.0).astype(bf16))
            if j >= midskew:
                jj = j - midskew
                wo = _paced(lambda rs, k: wo_v[jj * L + rs.start:jj * L + rs.stop, k * L:(k + 1) * L], L, NB,
                            parts0[NB + jj], list(range(NB)))
                m_v[jj * L:(jj + 1) * L, :] = _dot(kvs[jj], wo).astype(bf16)

        with sc("wait_ffn"):
            for c in range(1, N2):
                wg_dma(c).wait()
                wu_dma(c).wait()
            for c in range(N2):
                wd_dma(c).wait()

        def body2(i, _):
            b = lax.rem(iblk + 1 + i, N2)
            row0 = pl.multiple_of(b * R2, R2)
            rows = pl.ds(row0, R2)
            xnb, xblk, oblk = xn_v.at[rows], x_v.at[rows], out_v.at[rows]
            slot = lax.rem(i, 2)
            parts = _share(down_thunks(i, slot) + gate_up_thunks(lax.rem(i + 1, N2), 1 - slot), qw)
            xn = xnb[...]

            def Q(c):
                cs = slice(c * CW, (c + 1) * CW)
                rhs = _paced(lambda rs, k: xn[rs, k * L:(k + 1) * L], R2, NB, parts[c], list(kkQ))
                pq = _phi(_dg(wqt_v[cs, :], rhs, 1, 1))
                zc = zc_v[cs, :]
                nh = CW // DH
                for t in range(R2 // L):
                    p = pq[:, t * L:(t + 1) * L]
                    den = jnp.sum((p * zc).reshape(nh, DH, L), axis=1, keepdims=True) + 1e-6
                    o = (p.reshape(nh, DH, L) * _rcp(den)).reshape(CW, L)
                    o_v[t * L:(t + 1) * L, cs] = o.astype(bf16).T

            def H(n):
                cs = slice(n * CW, (n + 1) * CW)
                rhs = _paced(lambda rs, k: m_v[rs, n * CW + k * L:n * CW + (k + 1) * L], HK, CW // L,
                             parts[NC + n], [0, 1])
                acc_v[:, cs] = _dot(o_v[:, 0:HK], rhs) + (xblk[:, cs].astype(f32) + xnb[:, cs].astype(f32))

            def C(n):
                c0, nsl = ccols[n], (ccols[n + 1] - ccols[n]) // L
                cs = slice(c0, ccols[n + 1])
                rhs = _paced(lambda rs, k: m_v[HK + rs.start:HK + rs.stop, c0 + k * L:c0 + (k + 1) * L], HK, nsl,
                             parts[2 * NC + n], list(range(nsl)))
                oblk[:, cs] = (acc_v[:, cs] + _dot(o_v[:, HK:D], rhs)).astype(bf16)
                o_dma(b, n).start()

            for c in range(NC):
                Q(c)
            for n in range(NC):
                H(n)
            loc = idx - row0
            gl = pl.multiple_of(jnp.clip((loc // 8) * 8, 0, R2 - 8), 8)
            y = jnp.sum(y_v[...], axis=0, keepdims=True) * gate
            r8 = lax.broadcasted_iota(jnp.int32, (8, 1), 0) + gl
            acc_v[pl.ds(gl, 8), :] += jnp.where(r8 == loc, y, 0.0)
            for n in range(len(ccols) - 1):
                C(n)

        with sc("p2_loop"):
            lax.fori_loop(0, N2, body2, None)
        with sc("wait_out"):
            for b in range(N2):
                for n in range(len(ccols) - 1):
                    o_dma(b, n).wait()

    def fn(A_x, A_wqkv, A_wo, B_x, B_w_r, B_w_gate, B_w_up, B_w_down):
        anyspec = pl.BlockSpec(memory_space=pl.ANY)
        out = pl.pallas_call(
            kernel,
            out_shape=jax.ShapeDtypeStruct((S, D), bf16),
            in_specs=[anyspec] * 7,
            out_specs=anyspec,
            scratch_shapes=[
                pltpu.VMEM((S, D), bf16), pltpu.VMEM((S, D), bf16), pltpu.VMEM((D, 3 * D), bf16),
                pltpu.VMEM((D, D), bf16), pltpu.VMEM((D,), bf16),
                pltpu.VMEM((N2, D, FC), bf16), pltpu.VMEM((N2, D, FC), bf16), pltpu.VMEM((N2, FC, D), bf16),
                pltpu.VMEM((S, D), bf16), pltpu.VMEM((D, D), f32), pltpu.VMEM((D, L), f32),
                pltpu.VMEM((D, D), bf16), pltpu.VMEM((D, L), f32),
                pltpu.VMEM((R2, D), bf16), pltpu.VMEM((R2, D), f32),
                pltpu.VMEM((2, FC, L), f32), pltpu.VMEM((8, D), f32), pltpu.VMEM((D, D), bf16),
                pltpu.SemaphoreType.DMA((NSEM,)),
            ],
            compiler_params=pltpu.CompilerParams(vmem_limit_bytes=100 * 1024 * 1024,
                                                 flags=dict(flags) if flags else None),
        )(A_x.reshape(S, D), A_wqkv, A_wo, B_w_r, B_w_gate, B_w_up, B_w_down)
        return out.reshape(1, S, D)
    return fn


_IMPL = make(**dict())


@jax.jit
def pallas_parallel_sum__linear_attn_block__moe_arch_mod__prompt_kernel(
    A_x: jax.Array,
    A_wqkv: jax.Array,
    A_wo: jax.Array,
    B_x: jax.Array,
    B_w_r: jax.Array,
    B_w_gate: jax.Array,
    B_w_up: jax.Array,
    B_w_down: jax.Array,
):
    return _IMPL(A_x, A_wqkv, A_wo, B_x, B_w_r, B_w_gate, B_w_up, B_w_down)
```

```python
import contextlib
import functools

import jax
import jax.numpy as jnp
from jax import lax
import jax.experimental.pallas as pl
import jax.experimental.pallas.tpu as pltpu

S, D, DH, F = 2048, 1024, 32, 3584
L = 128
NB = D // L
f32, bf16, u32 = jnp.float32, jnp.bfloat16, jnp.uint32


def _phi(t, mm=False):
    if mm:
        return (jnp.maximum(t, 0.0) + 1e-6) + jnp.exp(jnp.minimum(t, 0.0))
    return jnp.where(t > 0, t + 1.0, jnp.exp(t)) + 1e-6


def _dot(a, b):
    return jnp.dot(a, b, preferred_element_type=f32)


def _dg(a, b, ca, cb):
    return lax.dot_general(a, b, (((ca,), (cb,)), ((), ())), preferred_element_type=f32)


def _rcp(x):
    r = pl.reciprocal(x, approx=True)
    return r * (2.0 - x * r)


def _zero(v):
    b = pltpu.bitcast(v, u32)
    return lax.shift_right_logical(lax.shift_right_logical(b, jnp.uint32(31)), jnp.uint32(1))


def _any(x):
    h = pltpu.bitcast(x[:, 0:L], u32)
    for j in range(1, x.shape[1] // L):
        h = h | pltpu.bitcast(x[:, j * L:(j + 1) * L], u32)
    return pltpu.bitcast(h, f32)


def _paced(load, nrows, nslab, thunks, kk=None):
    n = len(thunks)
    if n == 0:
        return jnp.concatenate([load(slice(0, nrows), k) for k in range(nslab)], axis=1)
    kk = list(range(0, nslab, 2)) if kk is None else kk
    per = -(-n // len(kk))
    npos = 1
    while npos < per * len(kk) and npos < nrows // 16:
        npos *= 2
    step = nrows // npos
    where = {}
    for p in range(n):
        m, q = divmod(p, per)
        r = (q * npos) // per + (m * npos) // (per * len(kk))
        where.setdefault((kk[m], min(r, npos - 1)), []).append(p)
    zs = [_zero(t()) for t in thunks]
    slabs = []
    for k in range(nslab):
        if k not in kk:
            slabs.append(load(slice(0, nrows), k))
            continue
        parts = []
        for r in range(npos):
            ps = where.get((k, r))
            if not ps:
                parts.append(load(slice(r * step, (r + 1) * step), k))
                continue
            z = zs[ps[0]]
            for p in ps[1:]:
                z = z | zs[p]
            tile = load(slice(r * step, r * step + 16), k)
            parts.append(pltpu.bitcast(pltpu.bitcast(tile, u32) | z, bf16))
            if step > 16:
                parts.append(load(slice(r * step + 16, (r + 1) * step), k))
        slabs.append(jnp.concatenate(parts, axis=0))
    return jnp.concatenate(slabs, axis=1)


def _share(seq, weights):
    tot, out, a = sum(weights), [], 0
    last = max(i for i, w in enumerate(weights) if w)
    for i, w in enumerate(weights):
        e = len(seq) if i == last else a + (len(seq) * w) // tot
        out.append(seq[a:e])
        a = e
    return out


def make(R1=512, R2=512, x0rows=(0, 128, 256, 384, 512), LNS=4, lnpos=(2, 3, 4, 5), lnpos0=(3, 4, 5, 6),
         rpos=0, rpos0=3, GR=16, DS=16, qw=(2,) * 12, kkQ=(4, 6), ccols=(0, 256, 512, 768, 1024),
         midsplit=(0,) + (1,) * 15, midskew=4, scopes=False, CW1=256, early=True, dbg=None, trf32=False, phimm=False, ggroups=((0, 4), (4, 7)), GRs=(32, 32), glags=(2, 1), porder='H0 H1 H2 P0 P1 P2 H3 P3 C0 C1 C2 C3',
         flags=(("XLA_TPU_EVENLY_DISTRIBUTE_CRITICAL_NODES", True),)):
    sc = (lambda n: jax.named_scope(n)) if scopes else (lambda n: contextlib.nullcontext())
    N1, N2 = S // R1, S // R2
    if ggroups is None:
        ggroups, GRs, glags = ((0, F // (S // R2) // L),), (GR,), (1,)
    CW = 256
    NC = D // CW
    FC = F // N2
    FB = FC // L
    HK = D // 2
    NX0 = len(x0rows) - 1
    wk_cols = [(0, L), (L, L), (CW, CW), (2 * CW, 2 * CW)]
    SX0, SWR, SWK = 0, NX0, NX0 + 1
    SX = SWK + len(wk_cols)
    SW = SX + N1 - 1
    SF = SW + 1
    SO = SF + 2
    NSEM = SO + 1

    def kernel(x_hbm, wqkv_hbm, wo_hbm, wr_hbm, wg_hbm, wu_hbm, wd_hbm, out_hbm,
               x_v, xn_v, wqkv_v, wo_v, wr_v, wg_v, wu_v, wd_v, out_v, pt_v, zc_v, m_v, xb_v, o_v, acc_v,
               hb_v, y_v, wqt_v, sems):
        def x0_dma(h):
            rs = pl.ds(x0rows[h], x0rows[h + 1] - x0rows[h])
            return pltpu.make_async_copy(x_hbm.at[rs], x_v.at[rs], sems.at[SX0 + h])

        def x_dma(i):
            rs = pl.ds(i * R1, R1)
            return pltpu.make_async_copy(x_hbm.at[rs], x_v.at[rs], sems.at[SX + i - 1])

        def wcols_dma(c0, n, sem):
            cs = pl.ds(c0, n)
            return pltpu.make_async_copy(wqkv_hbm.at[:, cs], wqkv_v.at[:, cs], sems.at[sem])

        def wk_dma(g):
            return wcols_dma(D + wk_cols[g][0], wk_cols[g][1], SWK + g)

        def wg_dma(c):
            return pltpu.make_async_copy(wg_hbm.at[:, pl.ds(c * FC, FC)], wg_v.at[c], sems.at[SF + (c > 0)])

        def wu_dma(c):
            return pltpu.make_async_copy(wu_hbm.at[:, pl.ds(c * FC, FC)], wu_v.at[c], sems.at[SF + (c > 0)])

        def wd_dma(c):
            return pltpu.make_async_copy(wd_hbm.at[pl.ds(c * FC, FC)], wd_v.at[c], sems.at[SF + 1])

        def o_dma(b, n):
            rows = pl.ds(pl.multiple_of(b * R2, R2), R2)
            cs = pl.ds(ccols[n], ccols[n + 1] - ccols[n])
            return pltpu.make_async_copy(out_v.at[rows, cs], out_hbm.at[rows, cs], sems.at[SO])

        wr_dma = pltpu.make_async_copy(wr_hbm, wr_v, sems.at[SWR])
        wq_dma = wcols_dma(0, D, SW)
        wv_dma = wcols_dma(2 * D, D, SW)
        wo_dma = pltpu.make_async_copy(wo_hbm, wo_v, sems.at[SW])

        for h in range(NX0):
            x0_dma(h).start()
        for g in range(len(wk_cols)):
            wk_dma(g).start()
            if g == 0:
                wr_dma.start()
        for i in range(1, N1):
            x_dma(i).start()
        wq_dma.start()
        wv_dma.start()
        wo_dma.start()
        for c in range(N2):
            wg_dma(c).start()
            wu_dma(c).start()
        for c in range(N2):
            wd_dma(c).start()

        def ln(row0, n):
            rows = pl.ds(row0, n)
            x = x_v[rows, :].astype(f32)
            m = jnp.mean(x, axis=-1, keepdims=True)
            d = x - m
            v = jnp.mean(d * d, axis=-1, keepdims=True)
            xn_v[rows, :] = (d * lax.rsqrt(v + 1e-5)).astype(bf16)

        def router(xn, row0, best, bidx):
            n = xn.shape[0]
            wr = wr_v[...].astype(f32).reshape(1, D)
            r = jnp.broadcast_to(jnp.sum(xn.astype(f32) * wr, axis=-1, keepdims=True), (n, L))
            rid = lax.broadcasted_iota(jnp.int32, (8, L), 0) + row0
            for g in range(n // 8):
                rg = r[8 * g:8 * g + 8]
                better = rg > best
                best = jnp.where(better, rg, best)
                bidx = jnp.where(better, rid + 8 * g, bidx)
            return best, bidx

        def p1_block(i, zacc, best, bidx, first):
            row0 = 0 if first else pl.multiple_of(i * R1, R1)
            nxt = R1 if first else pl.multiple_of(lax.rem(i + 1, N1) * R1, R1)
            if first:
                with sc("w_c0"):
                    wk_dma(0).wait()
                    wr_dma.wait()
            xn = xn_v[pl.ds(row0, R1), :]
            pks, zs, raw = [], [], []

            def fin_k(k):
                pk = _phi(k, phimm)
                zs.append(jnp.sum(pk.reshape(R1 // 8, 8, CW1), axis=0))
                pks.append(pk.astype(bf16))

            def kdot(c0, n):
                return _dot(xn, wqkv_v[:, D + c0:D + c0 + n])

            def K(c):
                if first and c == 0:
                    ks = [kdot(0, L)]
                    wk_dma(1).wait()
                    ks.append(kdot(L, L))
                    if CW1 == 512:
                        wk_dma(2).wait()
                        ks.append(kdot(2 * L, 2 * L))
                    raw.append(jnp.concatenate(ks, axis=1))
                    return
                if first and CW1 == 256 and c in (1, 2):
                    wk_dma(c + 1).wait()
                    if c == 2:
                        x_dma(1).wait()
                if first and CW1 == 512 and c == 1:
                    wk_dma(3).wait()
                    x_dma(1).wait()
                if raw:
                    fin_k(raw.pop())
                fin_k(kdot(c * CW1, CW1))

            def PT(c):
                cs = slice(c * CW1, (c + 1) * CW1)
                r = _dg(xn, pks[c], 0, 0)
                if first:
                    pt_v[:, cs] = r
                else:
                    pt_v[:, cs] += r

            if CW1 == 256:
                seq = [(K, 0), (K, 1), (PT, 0), (K, 2), (PT, 1), (K, 3), (PT, 2), (PT, 3)]
            else:
                seq = [(K, 0), (K, 1), (PT, 0), (PT, 1)]
            sub, done = R1 // LNS, 0
            for pos, (f, c) in enumerate(seq):
                if pos == (rpos0 if first else rpos):
                    best, bidx = router(xn, row0, best, bidx)
                f(c)
                for _ in range((lnpos0 if first else lnpos).count(pos)):
                    ln(nxt + done * sub, sub)
                    done += 1
            assert done == LNS
            return zacc + jnp.concatenate(zs, axis=1), best, bidx

        for h in range(NX0):
            with sc("wait_x0"):
                x0_dma(h).wait()
            ln(x0rows[h], x0rows[h + 1] - x0rows[h])

        best = jnp.full((8, L), -jnp.inf, f32)
        bidx = jnp.full((8, L), S, jnp.int32)
        with sc("p1_it0"):
            zacc, best, bidx = p1_block(0, jnp.zeros((8, D), f32), best, bidx, True)

        with sc("wait_x"):
            for i in range(2, N1):
                x_dma(i).wait()

        def body1(i, carry):
            return p1_block(i, *carry, False)

        with sc("p1_loop"):
            zacc, best, bidx = lax.fori_loop(1, N1, body1, (zacc, best, bidx))
        with sc("wait_w"):
            wq_dma.wait()
            wv_dma.wait()
            wo_dma.wait()
            wg_dma(0).wait()
            wu_dma(0).wait()
            if early:
                for c in range(1, N2):
                    wg_dma(c).wait()
                    wu_dma(c).wait()
                for c in range(N2):
                    wd_dma(c).wait()

        z = jnp.sum(zacc, axis=0, keepdims=True)
        zc_v[...] = jnp.broadcast_to(z, (L, D)).T
        bmax = jnp.max(best, axis=0, keepdims=True)
        idx = jnp.clip(jnp.min(jnp.where(best == bmax, bidx, S)), 0, S - 1)
        gate = jax.nn.sigmoid(bmax[:, 0:1])
        g0 = pl.multiple_of((idx // 16) * 16, 16)
        rr = lax.broadcasted_iota(jnp.int32, (16, 1), 0)
        xsel = jnp.sum(jnp.where(rr == idx - g0, xn_v[pl.ds(g0, 16), :].astype(f32), 0.0), axis=0, keepdims=True)
        xb_v[...] = jnp.broadcast_to(xsel, (L, D)).T
        y_v[...] = jnp.zeros((8, D), f32)
        iblk = idx // R2
        for c in range(NC):
            wqt_v[c * CW:(c + 1) * CW, :] = wqkv_v[:, c * CW:(c + 1) * CW].T

        def gate_up_thunks(c, slot):
            wg, wu = wg_v.at[c], wu_v.at[c]
            out = []
            for (j0, j1), gr, lag in zip(ggroups, GRs, glags):
                acc = [None]
                nb = j1 - j0

                def sub(s, acc=acc, j0=j0, j1=j1, gr=gr):
                    rs = slice(s * gr, (s + 1) * gr)
                    xb = xb_v[rs, :]
                    parts = []
                    for w in (wg, wu):
                        wf = w[rs, j0 * L:j1 * L].astype(f32)
                        for jb in range(j1 - j0):
                            parts.append(jnp.sum((wf[:, jb * L:(jb + 1) * L] * xb).reshape(gr // 8, 8, L), axis=0))
                    a = jnp.concatenate(parts, axis=1)
                    acc[0] = a if s == 0 else a + acc[0]
                    return _any(acc[0])

                def fin(jb, acc=acc, j0=j0, nb=nb):
                    g = jnp.sum(acc[0][:, jb * L:(jb + 1) * L], axis=0, keepdims=True)
                    u = jnp.sum(acc[0][:, (nb + jb) * L:(nb + jb + 1) * L], axis=0, keepdims=True)
                    hb = jnp.broadcast_to(g * jax.nn.sigmoid(g) * u, (L, L)).T
                    hb_v[slot, (j0 + jb) * L:(j0 + jb + 1) * L, :] = hb
                    return hb[0:8]

                out.append([functools.partial(sub, s) for s in range(D // gr)])
                out.append([functools.partial(fin, jb) for jb in range(nb)])
            seq = list(out[0])
            for gi in range(1, len(out) // 2):
                fins, subs = out[2 * gi - 1], out[2 * gi]
                lag = glags[gi - 1]
                for k, sb in enumerate(subs):
                    seq.append(sb)
                    if k % lag == lag - 1 and fins:
                        seq.append(fins.pop(0))
                seq.extend(fins)
            seq.extend(out[-1])
            return seq

        def down_thunks(c, slot):
            acc = [None]
            wd = wd_v.at[c]
            n = FC // DS

            def sub(s):
                rs = slice(s * DS, (s + 1) * DS)
                hb = hb_v[slot, rs, :]
                w = wd[rs, :].astype(f32)
                yy = jnp.concatenate(
                    [jnp.sum((w[:, jb * L:(jb + 1) * L] * hb).reshape(DS // 8, 8, L), axis=0) for jb in range(NB)],
                    axis=1)
                acc[0] = yy + (acc[0] if s > 0 else y_v[...])
                if s == n - 1:
                    y_v[...] = acc[0]
                return _any(acc[0])

            return [functools.partial(sub, s) for s in range(n)]

        ri = lax.broadcasted_iota(jnp.int32, (L, L), 0) // DH
        ci = lax.broadcasted_iota(jnp.int32, (L, L), 1) // DH
        order0 = [t for j in range(NB + midskew) for t in ([j] if j < NB else []) + ([NB + j - midskew] if j >= midskew else [])]
        parts0 = dict(zip(order0, _share(gate_up_thunks(0, 0), midsplit)))
        kvs = []
        for j in range(NB + midskew):
            if j < NB:
                wv = _paced(lambda rs, k: wqkv_v[rs, 2 * D + j * L:2 * D + (j + 1) * L], D, 1, parts0[j])
                kv = _dg(pt_v[:, j * L:(j + 1) * L].astype(bf16), wv, 0, 0)
                kvs.append(jnp.where(ri == ci, kv, 0.0).astype(bf16))
            if j >= midskew:
                jj = j - midskew
                wo = _paced(lambda rs, k: wo_v[jj * L + rs.start:jj * L + rs.stop, k * L:(k + 1) * L], L, NB,
                            parts0[NB + jj], list(range(NB)))
                m_v[jj * L:(jj + 1) * L, :] = _dot(kvs[jj], wo).astype(bf16)

        if not early:
            with sc("wait_ffn"):
                for c in range(1, N2):
                    wg_dma(c).wait()
                    wu_dma(c).wait()
                for c in range(N2):
                    wd_dma(c).wait()

        def body2(i, _):
            b = lax.rem(iblk + 1 + i, N2)
            row0 = pl.multiple_of(b * R2, R2)
            rows = pl.ds(row0, R2)
            xnb, xblk, oblk = xn_v.at[rows], x_v.at[rows], out_v.at[rows]
            slot = lax.rem(i, 2)
            parts = _share(down_thunks(i, slot) + gate_up_thunks(lax.rem(i + 1, N2), 1 - slot), qw)
            if dbg == 'noffn':
                parts = [[] for _ in qw]
                for t_ in down_thunks(i, slot)[:1]:
                    if False: t_()
            xn = xnb[...]

            def Q(c):
                cs = slice(c * CW, (c + 1) * CW)
                rhs = _paced(lambda rs, k: xn[rs, k * L:(k + 1) * L], R2, NB, parts[c], list(kkQ))
                pq = _phi(_dg(wqt_v[cs, :], rhs, 1, 1), phimm)
                zc = zc_v[cs, :]
                nh = CW // DH
                for t in range(R2 // L):
                    p = pq[:, t * L:(t + 1) * L]
                    den = jnp.sum((p * zc).reshape(nh, DH, L), axis=1, keepdims=True) + 1e-6
                    o = (p.reshape(nh, DH, L) * _rcp(den)).reshape(CW, L)
                    o_v[t * L:(t + 1) * L, cs] = o.T.astype(bf16) if trf32 else o.astype(bf16).T

            def H(n):
                cs = slice(n * CW, (n + 1) * CW)
                rhs = _paced(lambda rs, k: m_v[rs, n * CW + k * L:n * CW + (k + 1) * L], HK, CW // L,
                             parts[NC + n], [0, 1])
                acc_v[:, cs] = _dot(o_v[:, 0:HK], rhs) + (xblk[:, cs].astype(f32) + xnb[:, cs].astype(f32))

            def C(n):
                c0, nsl = ccols[n], (ccols[n + 1] - ccols[n]) // L
                cs = slice(c0, ccols[n + 1])
                rhs = _paced(lambda rs, k: m_v[HK + rs.start:HK + rs.stop, c0 + k * L:c0 + (k + 1) * L], HK, nsl,
                             parts[2 * NC + n], list(range(nsl)))
                oblk[:, cs] = (acc_v[:, cs] + _dot(o_v[:, HK:D], rhs)).astype(bf16)
                o_dma(b, n).start()

            loc = idx - row0
            gl = pl.multiple_of(jnp.clip((loc // 8) * 8, 0, R2 - 8), 8)
            r8 = lax.broadcasted_iota(jnp.int32, (8, 1), 0) + gl

            def patch(c0, c1):
                cs = slice(c0, c1)
                y = jnp.sum(y_v[:, cs], axis=0, keepdims=True) * gate
                acc_v[pl.ds(gl, 8), cs] += jnp.where(r8 == loc, y, 0.0)

            for c in range(NC):
                Q(c)
            for tok in porder.split():
                if tok[0] == 'H':
                    H(int(tok[1:]))
                elif tok[0] == 'C':
                    C(int(tok[1:]))
                elif tok == 'P':
                    patch(0, D)
                else:
                    n_ = int(tok[1:])
                    patch(n_ * CW, (n_ + 1) * CW)

        with sc("p2_loop"):
            lax.fori_loop(0, N2, body2, None)
        with sc("wait_out"):
            for b in range(N2):
                for n in range(len(ccols) - 1):
                    o_dma(b, n).wait()

    def fn(A_x, A_wqkv, A_wo, B_x, B_w_r, B_w_gate, B_w_up, B_w_down):
        anyspec = pl.BlockSpec(memory_space=pl.ANY)
        out = pl.pallas_call(
            kernel,
            out_shape=jax.ShapeDtypeStruct((S, D), bf16),
            in_specs=[anyspec] * 7,
            out_specs=anyspec,
            scratch_shapes=[
                pltpu.VMEM((S, D), bf16), pltpu.VMEM((S, D), bf16), pltpu.VMEM((D, 3 * D), bf16),
                pltpu.VMEM((D, D), bf16), pltpu.VMEM((D,), bf16),
                pltpu.VMEM((N2, D, FC), bf16), pltpu.VMEM((N2, D, FC), bf16), pltpu.VMEM((N2, FC, D), bf16),
                pltpu.VMEM((S, D), bf16), pltpu.VMEM((D, D), f32), pltpu.VMEM((D, L), f32),
                pltpu.VMEM((D, D), bf16), pltpu.VMEM((D, L), f32),
                pltpu.VMEM((R2, D), bf16), pltpu.VMEM((R2, D), f32),
                pltpu.VMEM((2, FC, L), f32), pltpu.VMEM((8, D), f32), pltpu.VMEM((D, D), bf16),
                pltpu.SemaphoreType.DMA((NSEM,)),
            ],
            compiler_params=pltpu.CompilerParams(vmem_limit_bytes=100 * 1024 * 1024,
                                                 flags=dict(flags) if flags else None),
        )(A_x.reshape(S, D), A_wqkv, A_wo, B_w_r, B_w_gate, B_w_up, B_w_down)
        return out.reshape(1, S, D)
    return fn


_IMPL = make(**dict())


@jax.jit
def pallas_parallel_sum__linear_attn_block__moe_arch_mod__prompt_kernel(
    A_x: jax.Array,
    A_wqkv: jax.Array,
    A_wo: jax.Array,
    B_x: jax.Array,
    B_w_r: jax.Array,
    B_w_gate: jax.Array,
    B_w_up: jax.Array,
    B_w_down: jax.Array,
):
    return _IMPL(A_x, A_wqkv, A_wo, B_x, B_w_r, B_w_gate, B_w_up, B_w_down)
```

```python
import functools

import jax
import jax.numpy as jnp
from jax import lax
import jax.experimental.pallas as pl
import jax.experimental.pallas.tpu as pltpu

S, D, DH, F = 2048, 1024, 32, 3584
L = 128
NB = D // L
R = 512
NI = S // R
CW = 256
NC = D // CW
HK = D // 2
FC = F // NI
X0 = (0, 128, 256, 384, 512)
WK = ((0, L), (L, L), (CW, CW), (2 * CW, 2 * CW))
G_GROUPS, G_ROWS, G_LAG = ((0, 4), (4, 7)), 32, 2
D_ROWS = 16
MID_SKEW = 4
P2_ORDER = "H0 H1 H2 P0 P1 P2 H3 P3 C0 C1 C2 C3"

SEM_X0 = 0
SEM_WR = SEM_X0 + len(X0) - 1
SEM_WK = SEM_WR + 1
SEM_X = SEM_WK + len(WK)
SEM_W = SEM_X + NI - 1
SEM_F = SEM_W + 1
SEM_O = SEM_F + 1
NSEM = SEM_O + 1

f32, bf16, u32 = jnp.float32, jnp.bfloat16, jnp.uint32


def _phi(t):
    return jnp.where(t > 0, t + 1.0, jnp.exp(t)) + 1e-6


def _dot(a, b):
    return jnp.dot(a, b, preferred_element_type=f32)


def _dg(a, b, ca, cb):
    return lax.dot_general(a, b, (((ca,), (cb,)), ((), ())), preferred_element_type=f32)


def _rcp(x):
    r = pl.reciprocal(x, approx=True)
    return r * (2.0 - x * r)


def _zero(v):
    b = pltpu.bitcast(v, u32)
    return lax.shift_right_logical(lax.shift_right_logical(b, jnp.uint32(31)), jnp.uint32(1))


def _any(x):
    h = pltpu.bitcast(x[:, 0:L], u32)
    for j in range(1, x.shape[1] // L):
        h = h | pltpu.bitcast(x[:, j * L:(j + 1) * L], u32)
    return pltpu.bitcast(h, f32)


def _paced(load, nrows, nslab, thunks, kk):
    n = len(thunks)
    if n == 0:
        return jnp.concatenate([load(slice(0, nrows), k) for k in range(nslab)], axis=1)
    per = -(-n // len(kk))
    npos = 1
    while npos < per * len(kk) and npos < nrows // 16:
        npos *= 2
    step = nrows // npos
    where = {}
    for p in range(n):
        m, q = divmod(p, per)
        r = (q * npos) // per + (m * npos) // (per * len(kk))
        where.setdefault((kk[m], min(r, npos - 1)), []).append(p)
    zs = [_zero(t()) for t in thunks]
    slabs = []
    for k in range(nslab):
        if k not in kk:
            slabs.append(load(slice(0, nrows), k))
            continue
        parts = []
        for r in range(npos):
            ps = where.get((k, r))
            if not ps:
                parts.append(load(slice(r * step, (r + 1) * step), k))
                continue
            z = zs[ps[0]]
            for p in ps[1:]:
                z = z | zs[p]
            tile = load(slice(r * step, r * step + 16), k)
            parts.append(pltpu.bitcast(pltpu.bitcast(tile, u32) | z, bf16))
            if step > 16:
                parts.append(load(slice(r * step + 16, (r + 1) * step), k))
        slabs.append(jnp.concatenate(parts, axis=0))
    return jnp.concatenate(slabs, axis=1)


def _share(seq, n, skip=0):
    m = n - skip
    k = len(seq) // m
    return [[] for _ in range(skip)] + [seq[a * k:(a + 1) * k if a < m - 1 else len(seq)] for a in range(m)]


def _kernel(x_hbm, wqkv_hbm, wo_hbm, wr_hbm, wg_hbm, wu_hbm, wd_hbm, out_hbm,
            x_v, xn_v, wqkv_v, wo_v, wr_v, wg_v, wu_v, wd_v, out_v, pt_v, zc_v, m_v, xb_v, o_v, acc_v,
            hb_v, y_v, wqt_v, sems):
    def x0_dma(h):
        rs = pl.ds(X0[h], X0[h + 1] - X0[h])
        return pltpu.make_async_copy(x_hbm.at[rs], x_v.at[rs], sems.at[SEM_X0 + h])

    def x_dma(i):
        rs = pl.ds(i * R, R)
        return pltpu.make_async_copy(x_hbm.at[rs], x_v.at[rs], sems.at[SEM_X + i - 1])

    def wcols_dma(c0, n, sem):
        cs = pl.ds(c0, n)
        return pltpu.make_async_copy(wqkv_hbm.at[:, cs], wqkv_v.at[:, cs], sems.at[sem])

    def wk_dma(g):
        return wcols_dma(D + WK[g][0], WK[g][1], SEM_WK + g)

    def ffn_dmas():
        out = []
        for c in range(NI):
            cs = pl.ds(c * FC, FC)
            out.append(pltpu.make_async_copy(wg_hbm.at[:, cs], wg_v.at[c], sems.at[SEM_F]))
            out.append(pltpu.make_async_copy(wu_hbm.at[:, cs], wu_v.at[c], sems.at[SEM_F]))
        for c in range(NI):
            out.append(pltpu.make_async_copy(wd_hbm.at[pl.ds(c * FC, FC)], wd_v.at[c], sems.at[SEM_F]))
        return out

    def w_dmas():
        return [wcols_dma(0, D, SEM_W), wcols_dma(2 * D, D, SEM_W), pltpu.make_async_copy(wo_hbm, wo_v, sems.at[SEM_W])]

    def o_dma(b, n):
        rows = pl.ds(pl.multiple_of(b * R, R), R)
        cs = pl.ds(n * CW, CW)
        return pltpu.make_async_copy(out_v.at[rows, cs], out_hbm.at[rows, cs], sems.at[SEM_O])

    wr_dma = pltpu.make_async_copy(wr_hbm, wr_v, sems.at[SEM_WR])
    for h in range(len(X0) - 1):
        x0_dma(h).start()
    for g in range(len(WK)):
        wk_dma(g).start()
        if g == 0:
            wr_dma.start()
    for i in range(1, NI):
        x_dma(i).start()
    for cp in w_dmas() + ffn_dmas():
        cp.start()

    def ln(row0, n):
        rows = pl.ds(row0, n)
        x = x_v[rows, :].astype(f32)
        m = jnp.mean(x, axis=-1, keepdims=True)
        d = x - m
        v = jnp.mean(d * d, axis=-1, keepdims=True)
        xn_v[rows, :] = (d * lax.rsqrt(v + 1e-5)).astype(bf16)

    def router(xn, row0, best, bidx):
        n = xn.shape[0]
        wr = wr_v[...].astype(f32).reshape(1, D)
        r = jnp.broadcast_to(jnp.sum(xn.astype(f32) * wr, axis=-1, keepdims=True), (n, L))
        rid = lax.broadcasted_iota(jnp.int32, (8, L), 0) + row0
        for g in range(n // 8):
            rg = r[8 * g:8 * g + 8]
            better = rg > best
            best = jnp.where(better, rg, best)
            bidx = jnp.where(better, rid + 8 * g, bidx)
        return best, bidx

    def p1_block(i, zacc, best, bidx, first):
        row0 = 0 if first else pl.multiple_of(i * R, R)
        nxt = R if first else pl.multiple_of(lax.rem(i + 1, NI) * R, R)
        if first:
            wk_dma(0).wait()
            wr_dma.wait()
        xn = xn_v[pl.ds(row0, R), :]
        pks, zs, raw = [], [], []

        def kdot(c0, n):
            return _dot(xn, wqkv_v[:, D + c0:D + c0 + n])

        def fin_k(k):
            pk = _phi(k)
            zs.append(jnp.sum(pk.reshape(R // 8, 8, CW), axis=0))
            pks.append(pk.astype(bf16))

        def K(c):
            if first and c == 0:
                k0 = kdot(0, L)
                wk_dma(1).wait()
                raw.append(jnp.concatenate([k0, kdot(L, L)], axis=1))
                return
            if first and c in (1, 2):
                wk_dma(c + 1).wait()
                if c == 2:
                    x_dma(1).wait()
            if raw:
                fin_k(raw.pop())
            fin_k(kdot(c * CW, CW))

        def PT(c):
            cs = slice(c * CW, (c + 1) * CW)
            r = _dg(xn, pks[c], 0, 0)
            if first:
                pt_v[:, cs] = r
            else:
                pt_v[:, cs] += r

        seq = [(K, 0), (K, 1), (PT, 0), (K, 2), (PT, 1), (K, 3), (PT, 2), (PT, 3)]
        done = 0
        for pos, (f, c) in enumerate(seq):
            if pos == (3 if first else 0):
                best, bidx = router(xn, row0, best, bidx)
            f(c)
            if (3 <= pos <= 6) if first else (2 <= pos <= 5):
                ln(nxt + done * (R // 4), R // 4)
                done += 1
        return zacc + jnp.concatenate(zs, axis=1), best, bidx

    for h in range(len(X0) - 1):
        x0_dma(h).wait()
        ln(X0[h], X0[h + 1] - X0[h])
    zacc, best, bidx = p1_block(0, jnp.zeros((8, D), f32), jnp.full((8, L), -jnp.inf, f32),
                                jnp.full((8, L), S, jnp.int32), True)
    for i in range(2, NI):
        x_dma(i).wait()
    zacc, best, bidx = lax.fori_loop(1, NI, lambda i, c: p1_block(i, *c, False), (zacc, best, bidx))
    for cp in w_dmas() + ffn_dmas():
        cp.wait()

    z = jnp.sum(zacc, axis=0, keepdims=True)
    zc_v[...] = jnp.broadcast_to(z, (L, D)).T
    bmax = jnp.max(best, axis=0, keepdims=True)
    idx = jnp.clip(jnp.min(jnp.where(best == bmax, bidx, S)), 0, S - 1)
    gate = jax.nn.sigmoid(bmax[:, 0:1])
    g0 = pl.multiple_of((idx // 16) * 16, 16)
    rr = lax.broadcasted_iota(jnp.int32, (16, 1), 0)
    xsel = jnp.sum(jnp.where(rr == idx - g0, xn_v[pl.ds(g0, 16), :].astype(f32), 0.0), axis=0, keepdims=True)
    xb_v[...] = jnp.broadcast_to(xsel, (L, D)).T
    y_v[...] = jnp.zeros((8, D), f32)
    iblk = idx // R
    for c in range(NC):
        wqt_v[c * CW:(c + 1) * CW, :] = wqkv_v[:, c * CW:(c + 1) * CW].T

    def gate_up_thunks(c, slot):
        wg, wu = wg_v.at[c], wu_v.at[c]
        subs, fins = [], []
        for j0, j1 in G_GROUPS:
            acc = [None]
            nb = j1 - j0

            def sub(s, acc=acc, j0=j0, j1=j1):
                rs = slice(s * G_ROWS, (s + 1) * G_ROWS)
                xb = xb_v[rs, :]
                parts = []
                for w in (wg, wu):
                    wf = w[rs, j0 * L:j1 * L].astype(f32)
                    for jb in range(j1 - j0):
                        parts.append(jnp.sum((wf[:, jb * L:(jb + 1) * L] * xb).reshape(G_ROWS // 8, 8, L), axis=0))
                a = jnp.concatenate(parts, axis=1)
                acc[0] = a if s == 0 else a + acc[0]
                return _any(acc[0])

            def fin(jb, acc=acc, j0=j0, nb=nb):
                g = jnp.sum(acc[0][:, jb * L:(jb + 1) * L], axis=0, keepdims=True)
                u = jnp.sum(acc[0][:, (nb + jb) * L:(nb + jb + 1) * L], axis=0, keepdims=True)
                hb = jnp.broadcast_to(g * jax.nn.sigmoid(g) * u, (L, L)).T
                hb_v[slot, (j0 + jb) * L:(j0 + jb + 1) * L, :] = hb
                return hb[0:8]

            subs.append([functools.partial(sub, s) for s in range(D // G_ROWS)])
            fins.append([functools.partial(fin, jb) for jb in range(nb)])
        seq = list(subs[0])
        for gi in range(1, len(subs)):
            pend = fins[gi - 1]
            for k, sb in enumerate(subs[gi]):
                seq.append(sb)
                if k % G_LAG == G_LAG - 1 and pend:
                    seq.append(pend.pop(0))
            seq.extend(pend)
        return seq + fins[-1]

    def down_thunks(c, slot):
        acc = [None]
        wd = wd_v.at[c]
        n = FC // D_ROWS

        def sub(s):
            rs = slice(s * D_ROWS, (s + 1) * D_ROWS)
            hb = hb_v[slot, rs, :]
            w = wd[rs, :].astype(f32)
            yy = jnp.concatenate(
                [jnp.sum((w[:, jb * L:(jb + 1) * L] * hb).reshape(D_ROWS // 8, 8, L), axis=0) for jb in range(NB)],
                axis=1)
            acc[0] = yy + (acc[0] if s > 0 else y_v[...])
            if s == n - 1:
                y_v[...] = acc[0]
            return _any(acc[0])

        return [functools.partial(sub, s) for s in range(n)]

    ri = lax.broadcasted_iota(jnp.int32, (L, L), 0) // DH
    ci = lax.broadcasted_iota(jnp.int32, (L, L), 1) // DH
    parts0 = _share(gate_up_thunks(0, 0), 2 * NB, skip=1)
    kvs = []
    for j in range(NB + MID_SKEW):
        if j < NB:
            wv = _paced(lambda rs, k: wqkv_v[rs, 2 * D + j * L:2 * D + (j + 1) * L], D, 1, parts0.pop(0), [0])
            kv = _dg(pt_v[:, j * L:(j + 1) * L].astype(bf16), wv, 0, 0)
            kvs.append(jnp.where(ri == ci, kv, 0.0).astype(bf16))
        if j >= MID_SKEW:
            jj = j - MID_SKEW
            wo = _paced(lambda rs, k: wo_v[jj * L + rs.start:jj * L + rs.stop, k * L:(k + 1) * L], L, NB,
                        parts0.pop(0), list(range(NB)))
            m_v[jj * L:(jj + 1) * L, :] = _dot(kvs[jj], wo).astype(bf16)

    def body2(i, _):
        b = lax.rem(iblk + 1 + i, NI)
        row0 = pl.multiple_of(b * R, R)
        rows = pl.ds(row0, R)
        xnb, xblk, oblk = xn_v.at[rows], x_v.at[rows], out_v.at[rows]
        slot = lax.rem(i, 2)
        parts = _share(down_thunks(i, slot) + gate_up_thunks(lax.rem(i + 1, NI), 1 - slot), 3 * NC)
        xn = xnb[...]

        def Q(c):
            cs = slice(c * CW, (c + 1) * CW)
            rhs = _paced(lambda rs, k: xn[rs, k * L:(k + 1) * L], R, NB, parts[c], [4, 6])
            pq = _phi(_dg(wqt_v[cs, :], rhs, 1, 1))
            zc = zc_v[cs, :]
            nh = CW // DH
            for t in range(R // L):
                p = pq[:, t * L:(t + 1) * L]
                den = jnp.sum((p * zc).reshape(nh, DH, L), axis=1, keepdims=True) + 1e-6
                o = (p.reshape(nh, DH, L) * _rcp(den)).reshape(CW, L)
                o_v[t * L:(t + 1) * L, cs] = o.astype(bf16).T

        def H(n):
            cs = slice(n * CW, (n + 1) * CW)
            rhs = _paced(lambda rs, k: m_v[rs, n * CW + k * L:n * CW + (k + 1) * L], HK, CW // L,
                         parts[NC + n], [0, 1])
            acc_v[:, cs] = _dot(o_v[:, 0:HK], rhs) + (xblk[:, cs].astype(f32) + xnb[:, cs].astype(f32))

        loc = idx - row0
        gl = pl.multiple_of(jnp.clip((loc // 8) * 8, 0, R - 8), 8)
        r8 = lax.broadcasted_iota(jnp.int32, (8, 1), 0) + gl

        def P(n):
            cs = slice(n * CW, (n + 1) * CW)
            y = jnp.sum(y_v[:, cs], axis=0, keepdims=True) * gate
            acc_v[pl.ds(gl, 8), cs] += jnp.where(r8 == loc, y, 0.0)

        def C(n):
            cs = slice(n * CW, (n + 1) * CW)
            rhs = _paced(lambda rs, k: m_v[HK + rs.start:HK + rs.stop, n * CW + k * L:n * CW + (k + 1) * L], HK,
                         CW // L, parts[2 * NC + n], [0, 1])
            oblk[:, cs] = (acc_v[:, cs] + _dot(o_v[:, HK:D], rhs)).astype(bf16)
            o_dma(b, n).start()

        for c in range(NC):
            Q(c)
        for tok in P2_ORDER.split():
            {"H": H, "P": P, "C": C}[tok[0]](int(tok[1]))

    lax.fori_loop(0, NI, body2, None)
    for b in range(NI):
        for n in range(NC):
            o_dma(b, n).wait()


@jax.jit
def pallas_parallel_sum__linear_attn_block__moe_arch_mod__prompt_kernel(
    A_x: jax.Array,
    A_wqkv: jax.Array,
    A_wo: jax.Array,
    B_x: jax.Array,
    B_w_r: jax.Array,
    B_w_gate: jax.Array,
    B_w_up: jax.Array,
    B_w_down: jax.Array,
):
    del B_x
    anyspec = pl.BlockSpec(memory_space=pl.ANY)
    out = pl.pallas_call(
        _kernel,
        out_shape=jax.ShapeDtypeStruct((S, D), bf16),
        in_specs=[anyspec] * 7,
        out_specs=anyspec,
        scratch_shapes=[
            pltpu.VMEM((S, D), bf16),
            pltpu.VMEM((S, D), bf16),
            pltpu.VMEM((D, 3 * D), bf16),
            pltpu.VMEM((D, D), bf16),
            pltpu.VMEM((D,), bf16),
            pltpu.VMEM((NI, D, FC), bf16),
            pltpu.VMEM((NI, D, FC), bf16),
            pltpu.VMEM((NI, FC, D), bf16),
            pltpu.VMEM((S, D), bf16),
            pltpu.VMEM((D, D), f32),
            pltpu.VMEM((D, L), f32),
            pltpu.VMEM((D, D), bf16),
            pltpu.VMEM((D, L), f32),
            pltpu.VMEM((R, D), bf16),
            pltpu.VMEM((R, D), f32),
            pltpu.VMEM((2, FC, L), f32),
            pltpu.VMEM((8, D), f32),
            pltpu.VMEM((D, D), bf16),
            pltpu.SemaphoreType.DMA((NSEM,)),
        ],
        compiler_params=pltpu.CompilerParams(
            vmem_limit_bytes=100 * 1024 * 1024,
            flags={"XLA_TPU_EVENLY_DISTRIBUTE_CRITICAL_NODES": True},
        ),
    )(A_x.reshape(S, D), A_wqkv, A_wo, B_w_r, B_w_gate, B_w_up, B_w_down)
    return out.reshape(1, S, D)
```

```python
import functools

import jax
import jax.numpy as jnp
from jax import lax
import jax.experimental.pallas as pl
import jax.experimental.pallas.tpu as pltpu

S, D, DH, F = 2048, 1024, 32, 3584
L = 128
NB = D // L
R = 512
NI = S // R
CW = 256
NC = D // CW
HK = D // 2
FC = F // NI
X0 = (0, 128, 256, 384, 512)
WK = ((0, L), (L, L), (CW, CW), (2 * CW, 2 * CW))
G_GROUPS, G_ROWS, G_LAG, G_LATE = ((0, 4), (4, 7)), 32, 5, 12
D_ROWS = 16
MID_SKEW = 4
P2_ORDER = "H0 H1 H2 P0 P1 P2 H3 P3 C0 C1 C2 C3"

SEM_X0 = 0
SEM_WR = SEM_X0 + len(X0) - 1
SEM_WK = SEM_WR + 1
SEM_X = SEM_WK + len(WK)
SEM_W = SEM_X + NI - 1
SEM_F = SEM_W + 1
SEM_O = SEM_F + 1
NSEM = SEM_O + 1

f32, bf16, u32 = jnp.float32, jnp.bfloat16, jnp.uint32


def _phi(t):
    return jnp.where(t > 0, t + 1.0, jnp.exp(t)) + 1e-6


def _dot(a, b):
    return jnp.dot(a, b, preferred_element_type=f32)


def _dg(a, b, ca, cb):
    return lax.dot_general(a, b, (((ca,), (cb,)), ((), ())), preferred_element_type=f32)


def _rcp(x):
    r = pl.reciprocal(x, approx=True)
    return r * (2.0 - x * r)


def _zero(v):
    b = pltpu.bitcast(v, u32)
    return lax.shift_right_logical(lax.shift_right_logical(b, jnp.uint32(31)), jnp.uint32(1))


def _any(x):
    h = pltpu.bitcast(x[:, 0:L], u32)
    for j in range(1, x.shape[1] // L):
        h = h | pltpu.bitcast(x[:, j * L:(j + 1) * L], u32)
    return pltpu.bitcast(h, f32)


def _paced(load, nrows, nslab, thunks, kk):
    n = len(thunks)
    if n == 0:
        return jnp.concatenate([load(slice(0, nrows), k) for k in range(nslab)], axis=1)
    per = -(-n // len(kk))
    npos = 1
    while npos < per * len(kk) and npos < nrows // 16:
        npos *= 2
    step = nrows // npos
    where = {}
    for p in range(n):
        m, q = divmod(p, per)
        r = (q * npos) // per + (m * npos) // (per * len(kk))
        where.setdefault((kk[m], min(r, npos - 1)), []).append(p)
    zs = [_zero(t()) for t in thunks]
    slabs = []
    for k in range(nslab):
        if k not in kk:
            slabs.append(load(slice(0, nrows), k))
            continue
        parts = []
        for r in range(npos):
            ps = where.get((k, r))
            if not ps:
                parts.append(load(slice(r * step, (r + 1) * step), k))
                continue
            z = zs[ps[0]]
            for p in ps[1:]:
                z = z | zs[p]
            tile = load(slice(r * step, r * step + 16), k)
            parts.append(pltpu.bitcast(pltpu.bitcast(tile, u32) | z, bf16))
            if step > 16:
                parts.append(load(slice(r * step + 16, (r + 1) * step), k))
        slabs.append(jnp.concatenate(parts, axis=0))
    return jnp.concatenate(slabs, axis=1)


def _share(seq, n, skip=0):
    m = n - skip
    k = len(seq) // m
    return [[] for _ in range(skip)] + [seq[a * k:(a + 1) * k if a < m - 1 else len(seq)] for a in range(m)]


def _kernel(x_hbm, wqkv_hbm, wo_hbm, wr_hbm, wg_hbm, wu_hbm, wd_hbm, out_hbm,
            x_v, xn_v, wqkv_v, wo_v, wr_v, wg_v, wu_v, wd_v, out_v, pt_v, zc_v, m_v, xb_v, o_v, acc_v,
            hb_v, y_v, wqt_v, gu_v, sems):
    def x0_dma(h):
        rs = pl.ds(X0[h], X0[h + 1] - X0[h])
        return pltpu.make_async_copy(x_hbm.at[rs], x_v.at[rs], sems.at[SEM_X0 + h])

    def x_dma(i):
        rs = pl.ds(i * R, R)
        return pltpu.make_async_copy(x_hbm.at[rs], x_v.at[rs], sems.at[SEM_X + i - 1])

    def wcols_dma(c0, n, sem):
        cs = pl.ds(c0, n)
        return pltpu.make_async_copy(wqkv_hbm.at[:, cs], wqkv_v.at[:, cs], sems.at[sem])

    def wk_dma(g):
        return wcols_dma(D + WK[g][0], WK[g][1], SEM_WK + g)

    def ffn_dmas():
        out = []
        for c in range(NI):
            cs = pl.ds(c * FC, FC)
            out.append(pltpu.make_async_copy(wg_hbm.at[:, cs], wg_v.at[c], sems.at[SEM_F]))
            out.append(pltpu.make_async_copy(wu_hbm.at[:, cs], wu_v.at[c], sems.at[SEM_F]))
        for c in range(NI):
            out.append(pltpu.make_async_copy(wd_hbm.at[pl.ds(c * FC, FC)], wd_v.at[c], sems.at[SEM_F]))
        return out

    def w_dmas():
        return [wcols_dma(0, D, SEM_W), wcols_dma(2 * D, D, SEM_W), pltpu.make_async_copy(wo_hbm, wo_v, sems.at[SEM_W])]

    def o_dma(b, n):
        rows = pl.ds(pl.multiple_of(b * R, R), R)
        cs = pl.ds(n * CW, CW)
        return pltpu.make_async_copy(out_v.at[rows, cs], out_hbm.at[rows, cs], sems.at[SEM_O])

    wr_dma = pltpu.make_async_copy(wr_hbm, wr_v, sems.at[SEM_WR])
    for h in range(len(X0) - 1):
        x0_dma(h).start()
    for g in range(len(WK)):
        wk_dma(g).start()
        if g == 0:
            wr_dma.start()
    for i in range(1, NI):
        x_dma(i).start()
    for cp in w_dmas() + ffn_dmas():
        cp.start()

    def ln(row0, n):
        rows = pl.ds(row0, n)
        x = x_v[rows, :].astype(f32)
        m = jnp.mean(x, axis=-1, keepdims=True)
        d = x - m
        v = jnp.mean(d * d, axis=-1, keepdims=True)
        xn_v[rows, :] = (d * lax.rsqrt(v + 1e-5)).astype(bf16)

    def router(xn, row0, best, bidx):
        n = xn.shape[0]
        wr = wr_v[...].astype(f32).reshape(1, D)
        r = jnp.broadcast_to(jnp.sum(xn.astype(f32) * wr, axis=-1, keepdims=True), (n, L))
        rid = lax.broadcasted_iota(jnp.int32, (8, L), 0) + row0
        for g in range(n // 8):
            rg = r[8 * g:8 * g + 8]
            better = rg > best
            best = jnp.where(better, rg, best)
            bidx = jnp.where(better, rid + 8 * g, bidx)
        return best, bidx

    def p1_block(i, zacc, best, bidx, first):
        row0 = 0 if first else pl.multiple_of(i * R, R)
        nxt = R if first else pl.multiple_of(lax.rem(i + 1, NI) * R, R)
        if first:
            wk_dma(0).wait()
            wr_dma.wait()
        xn = xn_v[pl.ds(row0, R), :]
        pks, zs, raw = [], [], []

        def kdot(c0, n):
            return _dot(xn, wqkv_v[:, D + c0:D + c0 + n])

        def fin_k(k):
            pk = _phi(k)
            zs.append(jnp.sum(pk.reshape(R // 8, 8, CW), axis=0))
            pks.append(pk.astype(bf16))

        def K(c):
            if first and c == 0:
                k0 = kdot(0, L)
                wk_dma(1).wait()
                raw.append(jnp.concatenate([k0, kdot(L, L)], axis=1))
                return
            if first and c in (1, 2):
                wk_dma(c + 1).wait()
                if c == 2:
                    x_dma(1).wait()
            if raw:
                fin_k(raw.pop())
            fin_k(kdot(c * CW, CW))

        def PT(c):
            cs = slice(c * CW, (c + 1) * CW)
            r = _dg(xn, pks[c], 0, 0)
            if first:
                pt_v[:, cs] = r
            else:
                pt_v[:, cs] += r

        seq = [(K, 0), (K, 1), (PT, 0), (K, 2), (PT, 1), (K, 3), (PT, 2), (PT, 3)]
        done = 0
        for pos, (f, c) in enumerate(seq):
            if pos == (3 if first else 0):
                best, bidx = router(xn, row0, best, bidx)
            f(c)
            if (3 <= pos <= 6) if first else (2 <= pos <= 5):
                ln(nxt + done * (R // 4), R // 4)
                done += 1
        return zacc + jnp.concatenate(zs, axis=1), best, bidx

    for h in range(len(X0) - 1):
        x0_dma(h).wait()
        ln(X0[h], X0[h + 1] - X0[h])
    zacc, best, bidx = p1_block(0, jnp.zeros((8, D), f32), jnp.full((8, L), -jnp.inf, f32),
                                jnp.full((8, L), S, jnp.int32), True)
    for i in range(2, NI):
        x_dma(i).wait()
    zacc, best, bidx = lax.fori_loop(1, NI, lambda i, c: p1_block(i, *c, False), (zacc, best, bidx))
    for cp in w_dmas() + ffn_dmas():
        cp.wait()

    z = jnp.sum(zacc, axis=0, keepdims=True)
    zc_v[...] = jnp.broadcast_to(z, (L, D)).T
    bmax = jnp.max(best, axis=0, keepdims=True)
    idx = jnp.clip(jnp.min(jnp.where(best == bmax, bidx, S)), 0, S - 1)
    gate = jax.nn.sigmoid(bmax[:, 0:1])
    g0 = pl.multiple_of((idx // 16) * 16, 16)
    rr = lax.broadcasted_iota(jnp.int32, (16, 1), 0)
    xsel = jnp.sum(jnp.where(rr == idx - g0, xn_v[pl.ds(g0, 16), :].astype(f32), 0.0), axis=0, keepdims=True)
    xb_v[...] = jnp.broadcast_to(xsel, (L, D)).T
    y_v[...] = jnp.zeros((8, D), f32)
    iblk = idx // R
    for c in range(NC):
        wqt_v[c * CW:(c + 1) * CW, :] = wqkv_v[:, c * CW:(c + 1) * CW].T

    def finish_h(get, j0, nb, jb, slot):
        g = jnp.sum(get(slice(jb * L, (jb + 1) * L)), axis=0, keepdims=True)
        u = jnp.sum(get(slice((nb + jb) * L, (nb + jb + 1) * L)), axis=0, keepdims=True)
        hb = jnp.broadcast_to(g * jax.nn.sigmoid(g) * u, (L, L)).T
        hb_v[slot, (j0 + jb) * L:(j0 + jb + 1) * L, :] = hb
        return hb[0:8]

    def gate_up_thunks(c, slot):
        wg, wu = wg_v.at[c], wu_v.at[c]
        subs, fins = [], []
        for j0, j1 in G_GROUPS:
            acc = [None]
            nb = j1 - j0

            def sub(s, acc=acc, j0=j0, j1=j1):
                rs = slice(s * G_ROWS, (s + 1) * G_ROWS)
                xb = xb_v[rs, :]
                parts = []
                for w in (wg, wu):
                    wf = w[rs, j0 * L:j1 * L].astype(f32)
                    for jb in range(j1 - j0):
                        parts.append(jnp.sum((wf[:, jb * L:(jb + 1) * L] * xb).reshape(G_ROWS // 8, 8, L), axis=0))
                a = jnp.concatenate(parts, axis=1)
                acc[0] = a if s == 0 else a + acc[0]
                if (j0, j1) == G_GROUPS[-1] and s == D // G_ROWS - 1:
                    gu_v[...] = acc[0]
                return _any(acc[0])

            subs.append([functools.partial(sub, s) for s in range(D // G_ROWS)])
            fins.append([functools.partial(finish_h, lambda cs, acc=acc: acc[0][:, cs], j0, nb, jb, slot)
                         for jb in range(nb)])
        seq = list(subs[0])
        for gi in range(1, len(subs)):
            pend = fins[gi - 1]
            for k, sb in enumerate(subs[gi]):
                seq.append(sb)
                if k % G_LAG == G_LAG - 1 and pend:
                    seq.append(pend.pop(0))
            seq.extend(pend)
        return seq

    def late_thunks(slot):
        j0, j1 = G_GROUPS[-1]
        return [functools.partial(finish_h, lambda cs: gu_v[:, cs], j0, j1 - j0, jb, slot) for jb in range(j1 - j0)]

    def down_thunks(c, slot):
        acc = [None]
        wd = wd_v.at[c]
        n = FC // D_ROWS

        def sub(s):
            rs = slice(s * D_ROWS, (s + 1) * D_ROWS)
            hb = hb_v[slot, rs, :]
            w = wd[rs, :].astype(f32)
            yy = jnp.concatenate(
                [jnp.sum((w[:, jb * L:(jb + 1) * L] * hb).reshape(D_ROWS // 8, 8, L), axis=0) for jb in range(NB)],
                axis=1)
            acc[0] = yy + (acc[0] if s > 0 else y_v[...])
            if s == n - 1:
                y_v[...] = acc[0]
            return _any(acc[0])

        return [functools.partial(sub, s) for s in range(n)]

    ri = lax.broadcasted_iota(jnp.int32, (L, L), 0) // DH
    ci = lax.broadcasted_iota(jnp.int32, (L, L), 1) // DH
    parts0 = _share(gate_up_thunks(0, 0), 2 * NB, skip=1)
    kvs = []
    for j in range(NB + MID_SKEW):
        if j < NB:
            wv = _paced(lambda rs, k: wqkv_v[rs, 2 * D + j * L:2 * D + (j + 1) * L], D, 1, parts0.pop(0), [0])
            kv = _dg(pt_v[:, j * L:(j + 1) * L].astype(bf16), wv, 0, 0)
            kvs.append(jnp.where(ri == ci, kv, 0.0).astype(bf16))
        if j >= MID_SKEW:
            jj = j - MID_SKEW
            wo = _paced(lambda rs, k: wo_v[jj * L + rs.start:jj * L + rs.stop, k * L:(k + 1) * L], L, NB,
                        parts0.pop(0), list(range(NB)))
            m_v[jj * L:(jj + 1) * L, :] = _dot(kvs[jj], wo).astype(bf16)

    def body2(i, _):
        b = lax.rem(iblk + 1 + i, NI)
        row0 = pl.multiple_of(b * R, R)
        rows = pl.ds(row0, R)
        xnb, xblk, oblk = xn_v.at[rows], x_v.at[rows], out_v.at[rows]
        slot = lax.rem(i, 2)
        down = down_thunks(i, slot)
        parts = _share(down[:G_LATE] + late_thunks(slot) + down[G_LATE:]
                       + gate_up_thunks(lax.rem(i + 1, NI), 1 - slot), 3 * NC)
        xn = xnb[...]

        def Q(c):
            cs = slice(c * CW, (c + 1) * CW)
            rhs = _paced(lambda rs, k: xn[rs, k * L:(k + 1) * L], R, NB, parts[c], [6])
            pq = _phi(_dg(wqt_v[cs, :], rhs, 1, 1))
            zc = zc_v[cs, :]
            nh = CW // DH
            for t in range(R // L):
                p = pq[:, t * L:(t + 1) * L]
                den = jnp.sum((p * zc).reshape(nh, DH, L), axis=1, keepdims=True) + 1e-6
                o = (p.reshape(nh, DH, L) * _rcp(den)).reshape(CW, L)
                o_v[t * L:(t + 1) * L, cs] = o.astype(bf16).T

        def H(n):
            cs = slice(n * CW, (n + 1) * CW)
            rhs = _paced(lambda rs, k: m_v[rs, n * CW + k * L:n * CW + (k + 1) * L], HK, CW // L,
                         parts[NC + n], [0, 1])
            acc_v[:, cs] = _dot(o_v[:, 0:HK], rhs) + (xblk[:, cs].astype(f32) + xnb[:, cs].astype(f32))

        loc = idx - row0
        gl = pl.multiple_of(jnp.clip((loc // 8) * 8, 0, R - 8), 8)
        r8 = lax.broadcasted_iota(jnp.int32, (8, 1), 0) + gl

        def P(n):
            cs = slice(n * CW, (n + 1) * CW)
            y = jnp.sum(y_v[:, cs], axis=0, keepdims=True) * gate
            acc_v[pl.ds(gl, 8), cs] += jnp.where(r8 == loc, y, 0.0)

        def C(n):
            cs = slice(n * CW, (n + 1) * CW)
            rhs = _paced(lambda rs, k: m_v[HK + rs.start:HK + rs.stop, n * CW + k * L:n * CW + (k + 1) * L], HK,
                         CW // L, parts[2 * NC + n], [0, 1])
            oblk[:, cs] = (acc_v[:, cs] + _dot(o_v[:, HK:D], rhs)).astype(bf16)
            o_dma(b, n).start()

        for c in range(NC):
            Q(c)
        for tok in P2_ORDER.split():
            {"H": H, "P": P, "C": C}[tok[0]](int(tok[1]))

    lax.fori_loop(0, NI, body2, None)
    for b in range(NI):
        for n in range(NC):
            o_dma(b, n).wait()


@jax.jit
def pallas_parallel_sum__linear_attn_block__moe_arch_mod__prompt_kernel(
    A_x: jax.Array,
    A_wqkv: jax.Array,
    A_wo: jax.Array,
    B_x: jax.Array,
    B_w_r: jax.Array,
    B_w_gate: jax.Array,
    B_w_up: jax.Array,
    B_w_down: jax.Array,
):
    del B_x
    anyspec = pl.BlockSpec(memory_space=pl.ANY)
    out = pl.pallas_call(
        _kernel,
        out_shape=jax.ShapeDtypeStruct((S, D), bf16),
        in_specs=[anyspec] * 7,
        out_specs=anyspec,
        scratch_shapes=[
            pltpu.VMEM((S, D), bf16),
            pltpu.VMEM((S, D), bf16),
            pltpu.VMEM((D, 3 * D), bf16),
            pltpu.VMEM((D, D), bf16),
            pltpu.VMEM((D,), bf16),
            pltpu.VMEM((NI, D, FC), bf16),
            pltpu.VMEM((NI, D, FC), bf16),
            pltpu.VMEM((NI, FC, D), bf16),
            pltpu.VMEM((S, D), bf16),
            pltpu.VMEM((D, D), f32),
            pltpu.VMEM((D, L), f32),
            pltpu.VMEM((D, D), bf16),
            pltpu.VMEM((D, L), f32),
            pltpu.VMEM((R, D), bf16),
            pltpu.VMEM((R, D), f32),
            pltpu.VMEM((2, FC, L), f32),
            pltpu.VMEM((8, D), f32),
            pltpu.VMEM((D, D), bf16),
            pltpu.VMEM((8, 2 * (G_GROUPS[-1][1] - G_GROUPS[-1][0]) * L), f32),
            pltpu.SemaphoreType.DMA((NSEM,)),
        ],
        compiler_params=pltpu.CompilerParams(
            vmem_limit_bytes=100 * 1024 * 1024,
            flags={"XLA_TPU_EVENLY_DISTRIBUTE_CRITICAL_NODES": True},
        ),
    )(A_x.reshape(S, D), A_wqkv, A_wo, B_w_r, B_w_gate, B_w_up, B_w_down)
    return out.reshape(1, S, D)
```
